```python
import jax
import jax.numpy as jnp

def _softmax(x, axis=-1):
    return jax.nn.softmax(x, axis=axis)

def _gelu(x):
    return jax.nn.gelu(x, approximate=True)

def _silu(x):
    return jax.nn.silu(x)

def _sigmoid(x):
    return jax.nn.sigmoid(x)

def _layernorm(x, axis=-1, eps=1e-05):
    m = jnp.mean(x, axis=axis, keepdims=True)
    v = jnp.var(x, axis=axis, keepdims=True)
    return (x - m) / jnp.sqrt(v + eps)

def _scatter_add(tgt, idx, src, axis=0):
    return tgt.at[idx].add(src)

def _segment_sum(src, seg, n):
    return jax.ops.segment_sum(src, seg, n)

class _Rng:

    def __init__(self, key):
        self._k = key

    def _next(self):
        self._k, sub = jax.random.split(self._k)
        return sub

    def normal(self, shape):
        return jax.random.normal(self._next(), shape, dtype=jnp.bfloat16)

    def randint(self, lo, hi, shape):
        return jax.random.randint(self._next(), shape, lo, hi, dtype=jnp.int32)

    def uniform(self, shape, lo=0.0, hi=1.0):
        return jax.random.uniform(self._next(), shape, jnp.bfloat16, lo, hi)

    def permutation(self, n):
        return jax.random.permutation(self._next(), n)
kernel_name = 'interleave_layers__memory_aug_infini_attn__moe_arch_mod__prompt'

def setup_inputs():
    _rng = _Rng(jax.random.key(int.from_bytes(__import__("os").urandom(4), "little")))
    _w = lambda a: (lambda t: t.astype(jnp.bfloat16) if jnp.issubdtype(t.dtype, jnp.floating) else t)(jnp.asarray(a))

    def _A_setup():
        B, S, D, H = (1, 2048, 1024, 32)
        N = 4
        L = max(1, S // N)
        sc = D ** (-0.5)
        return {'x': _w((lambda *s: _rng.normal(s) * 0.05)(B, N * L, D)), 'wq': _w((lambda *s: _rng.normal(s) * 0.05)(D, D) * sc), 'wk': _w((lambda *s: _rng.normal(s) * 0.05)(D, D) * sc), 'wv': _w((lambda *s: _rng.normal(s) * 0.05)(D, D) * sc), 'wo': _w((lambda *s: _rng.normal(s) * 0.05)(D, D) * sc), 'beta': _w((lambda *s: _rng.normal(s) * 0.05)(H))}
    _A_in = _A_setup()

    def _B_setup():
        B, S, D, F, C = (1, 2048, 1024, 3584, 2)
        return {'x': _w((lambda *s: _rng.normal(s) * 0.05)(B, S, D)), 'w_r': _w((lambda *s: _rng.normal(s) * 0.05)(D)), 'w_gate': _w((lambda *s: _rng.normal(s) * 0.05)(D, F)), 'w_up': _w((lambda *s: _rng.normal(s) * 0.05)(D, F)), 'w_down': _w((lambda *s: _rng.normal(s) * 0.05)(F, D))}
    _B_in = _B_setup()
    return {'A_x': _A_in['x'], 'A_wq': _A_in['wq'], 'A_wk': _A_in['wk'], 'A_wv': _A_in['wv'], 'A_wo': _A_in['wo'], 'A_beta': _A_in['beta'], 'B_x': _B_in['x'], 'B_w_r': _B_in['w_r'], 'B_w_gate': _B_in['w_gate'], 'B_w_up': _B_in['w_up'], 'B_w_down': _B_in['w_down']}

def reference(A_x, A_wq, A_wk, A_wv, A_wo, A_beta, B_x, B_w_r, B_w_gate, B_w_up, B_w_down):

    def _A_ref(x, wq, wk, wv, wo, beta):
        B, S, D = x.shape
        H = 32
        Dh = D // H
        N = 4
        L = S // N
        q = (lambda x, *d: x.transpose(*d))((x @ wq).reshape(B, S, H, Dh), 0, 2, 1, 3).reshape(B, H, N, L, Dh)
        k = (lambda x, *d: x.transpose(*d))((x @ wk).reshape(B, S, H, Dh), 0, 2, 1, 3).reshape(B, H, N, L, Dh)
        v = (lambda x, *d: x.transpose(*d))((x @ wv).reshape(B, S, H, Dh), 0, 2, 1, 3).reshape(B, H, N, L, Dh)
        phi = lambda t: jnp.where(t > 0, t + 1.0, jnp.exp(t))
        scale = Dh ** (-0.5)
        ar = jnp.arange(L)
        mask = (lambda x, dt: x.astype(dt))(ar[:, None] < ar[None, :], x.dtype) * -1000000000.0
        g = _sigmoid(beta).reshape(1, H, 1, 1)
        M = jnp.einsum('bhd,bhe->bhde', q[:, :, 0, 0, :] * 0.0, q[:, :, 0, 0, :] * 0.0)
        z = q[:, :, 0, 0, :] * 0.0
        outs = []
        for s in range(N):
            qs, ks, vs = (q[:, :, s].copy(), k[:, :, s].copy(), v[:, :, s].copy())
            logits = jnp.einsum('bhqd,bhkd->bhqk', qs, ks) * scale + mask
            p = _softmax(logits, axis=-1)
            a_dot = jnp.einsum('bhqk,bhkd->bhqd', p, vs)
            pq = phi(qs)
            num = jnp.einsum('bhld,bhde->bhle', pq, M)
            den = jnp.einsum('bhld,bhd->bhl', pq, z)[..., None] + 1e-06
            a_mem = num / den
            o = g * a_mem + (1.0 - g) * a_dot
            outs.append(o)
            pk = phi(ks)
            M = M + jnp.einsum('bhld,bhle->bhde', pk, vs)
            z = z + jnp.einsum('bhld->bhd', pk)
        o = (lambda x, *d: x.transpose(*d))(jnp.stack(outs, 2).reshape(B, H, S, Dh), 0, 2, 1, 3).reshape(B, S, D)
        return o @ wo

    def _B_ref(x, w_r, w_gate, w_up, w_down):
        B, S, D = x.shape
        C = 2
        r = x @ w_r
        idx = jnp.argsort(-r, axis=-1)[:, :C]
        idx_e = jnp.repeat(idx.reshape(B, C, 1), D, axis=2)
        x_sel = jnp.take_along_axis(x, idx_e, axis=1)
        g = _silu(x_sel @ w_gate)
        u = x_sel @ w_up
        y = g * u @ w_down
        r_sel = _sigmoid(jnp.take_along_axis(r, idx, axis=1))
        y = y * r_sel.reshape(B, C, 1)
        b_off = (jnp.arange(B) * S).reshape(B, 1)
        flat_idx = (idx + b_off).reshape(B * C)
        zero = (x * 0.0).reshape(B * S, D)
        upd = _scatter_add(zero, flat_idx, y.reshape(B * C, D), axis=0)
        return x + upd.reshape(B, S, D)
    x = A_x
    x = x + _A_ref(_layernorm(x, axis=-1), A_wq, A_wk, A_wv, A_wo, A_beta)
    x = x + _B_ref(_layernorm(x, axis=-1), B_w_r, B_w_gate, B_w_up, B_w_down)
    x = x + _A_ref(_layernorm(x, axis=-1), A_wq, A_wk, A_wv, A_wo, A_beta)
    x = x + _B_ref(_layernorm(x, axis=-1), B_w_r, B_w_gate, B_w_up, B_w_down)
    return x
```

```python
import numpy as np
import jax
import jax.numpy as jnp
from jax import lax
import jax.experimental.pallas as pl
import jax.experimental.pallas.tpu as pltpu

F32 = jnp.float32
BF16 = jnp.bfloat16

S, D, H, NSEG, FF = 2048, 1024, 32, 4, 3584
DH = D // H
L = S // NSEG
NG = D // 128
HPG = 128 // DH
QB = 128
LOG2E = float(np.log2(np.e))
SCALE = float(np.asarray(DH ** -0.5, dtype=np.float32).astype(jnp.bfloat16).astype(np.float32))
QSCALE = SCALE * LOG2E
MASKV = -1e9 * LOG2E


def _phi(t):
    return jnp.where(t > 0, t + 1.0, jnp.exp(t))


def _ln(x):
    m = jnp.mean(x, axis=-1, keepdims=True)
    xc = x - m
    v = jnp.mean(xc * xc, axis=-1, keepdims=True)
    return xc * lax.rsqrt(v + 1e-5)


def _nt(a, b):
    return lax.dot_general(a, b, (((1,), (1,)), ((), ())), preferred_element_type=F32)


def _nn(a, b):
    return jnp.dot(a, b, preferred_element_type=F32)


def _kernel(x_hbm, wq_hbm, wk_hbm, wv_hbm, wo_hbm, beta_ref, wr_ref, wg_hbm, wu_hbm, wd_hbm,
            out_hbm,
            xin, xf, xn, wq, wk, wv, wo, wqT, wvT, wg, wu, wd,
            qT, pqT, vT, kk, pk, ob, zs, gs, rr, mT,
            sem_x, sem_w, sem_o):
    def x_copy(i):
        return pltpu.make_async_copy(x_hbm.at[0, pl.ds(i * L, L), :], xin.at[pl.ds(i * L, L), :], sem_x.at[i])

    def w_copy(j):
        src = (wk_hbm, wq_hbm, wv_hbm, wo_hbm, wg_hbm, wu_hbm, wd_hbm)[j]
        dst = (wk, wq, wv, wo, wg, wu, wd)[j]
        return pltpu.make_async_copy(src, dst, sem_w.at[j])

    x_copy(0).start()
    w_copy(0).start()
    w_copy(1).start()
    w_copy(2).start()
    for i in range(1, NSEG):
        x_copy(i).start()
    for j in range(3, 7):
        w_copy(j).start()

    b = beta_ref[...].astype(F32)
    sg = 1.0 / (1.0 + jnp.exp(-b))
    lane = lax.broadcasted_iota(jnp.int32, (1, H), 1)
    for h in range(H):
        gh = jnp.sum(jnp.where(lane == h, sg, 0.0), axis=1, keepdims=True)
        gs[pl.ds(h * DH, DH), :] = jnp.broadcast_to(gh, (DH, 128))

    krow = lax.broadcasted_iota(jnp.int32, (QB, QB), 0)
    qcol = lax.broadcasted_iota(jnp.int32, (QB, QB), 1)

    def ln0(i, c):
        x_copy(i).wait()
        r = pl.multiple_of(i * L, L)
        xv = xin[pl.ds(r, L), :].astype(F32)
        xf[pl.ds(r, L), :] = xv
        xn[pl.ds(r, L), :] = _ln(xv).astype(BF16)
        return c
    lax.fori_loop(0, NSEG, ln0, 0)

    w_copy(0).wait()
    w_copy(1).wait()

    def tr_body(src, dst):
        def body(i, c):
            r = pl.multiple_of(i * 128, 128)
            dst[:, pl.ds(r, 128)] = src[pl.ds(r, 128), :].T
            return c
        lax.fori_loop(0, D // 128, body, 0)
    tr_body(wq, wqT)
    w_copy(2).wait()
    tr_body(wv, wvT)

    def layer(li, carry):
        last = li == 1
        def proj(s, c):
            r = pl.multiple_of(s * L, L)
            xb = xn[pl.ds(r, L), :]
            kf = _nn(xb, wk[...])
            pf = _phi(kf)
            zs[pl.ds(s, 1), :] = jnp.sum(pf, axis=0, keepdims=True)
            kb16 = kf.astype(BF16)
            pb16 = pf.astype(BF16)
            for g in range(NG):
                kk[g, pl.ds(r, L), :] = kb16[:, g * 128:(g + 1) * 128]
                pk[g, pl.ds(r, L), :] = pb16[:, g * 128:(g + 1) * 128]
            qf = _nt(wqT[...], xb)
            qT[:, pl.ds(r, L)] = (qf * QSCALE).astype(BF16)
            pqT[:, pl.ds(r, L)] = _phi(qf).astype(BF16)
            vf = _nt(wvT[...], xb)
            vT[:, pl.ds(r, L)] = vf.astype(BF16)
            return c
        lax.fori_loop(0, NSEG, proj, 0)

        def attn(g, c):
            g0 = pl.multiple_of(g * 128, 128)
            gate = gs[pl.ds(g0, 128), :]
            maskT = jnp.where(krow > qcol, MASKV, 0.0).astype(F32)
            rh = lax.broadcasted_iota(jnp.int32, (128, 128), 0) // DH
            ch = lax.broadcasted_iota(jnp.int32, (128, 128), 1) // DH
            bd = rh == ch
            macc = None
            zacc = None
            for s in range(NSEG):
                t0 = s * L
                if s > 0:
                    zrow = jnp.broadcast_to(zacc, (8, 128))
                    lane_h = lax.broadcasted_iota(jnp.int32, (8, 128), 1) // DH
                    zl = [jnp.where(lane_h == h, zrow, 0.0) for h in range(HPG)]
                    lhs = jnp.concatenate([macc] + zl, axis=0).astype(BF16)
                    nd = _nn(lhs, pqT[pl.ds(g0, 128), pl.ds(t0, L)])
                cols = []
                for qb in range(L // QB):
                    nk = (qb + 1) * QB
                    q0 = t0 + qb * QB
                    rows = []
                    for h in range(HPG):
                        qt = qT[pl.ds(g0 + h * DH, DH), pl.ds(q0, QB)]
                        parts = []
                        if h > 0:
                            parts.append(jnp.zeros((h * DH, QB), BF16))
                        parts.append(qt)
                        if h < HPG - 1:
                            parts.append(jnp.zeros(((HPG - 1 - h) * DH, QB), BF16))
                        w = jnp.concatenate(parts, axis=0)
                        st = _nn(kk[g, pl.ds(t0, nk), :], w)
                        if qb > 0:
                            st = jnp.concatenate([st[:nk - QB], st[nk - QB:] + maskT], axis=0)
                        else:
                            st = st + maskT
                        m = jnp.max(st, axis=0, keepdims=True)
                        p = jnp.exp2(st - m)
                        l = jnp.sum(p, axis=0, keepdims=True)
                        vt = vT[pl.ds(g0 + h * DH, DH), pl.ds(t0, nk)]
                        ot = _nn(vt, p.astype(BF16))
                        adot = ot * (1.0 / l)
                        gt = gate[h * DH:(h + 1) * DH, :]
                        if s > 0:
                            num = nd[h * DH:(h + 1) * DH, qb * QB:(qb + 1) * QB]
                            den = nd[128 + 8 * h:128 + 8 * h + 1, qb * QB:(qb + 1) * QB] + 1e-6
                            o = gt * (num / den) + (1.0 - gt) * adot
                        else:
                            o = (1.0 - gt) * adot
                        rows.append(o)
                    oT = jnp.concatenate(rows, axis=0)
                    ob[pl.ds(q0, QB), pl.ds(g0, 128)] = oT.T.astype(BF16)
                if s < NSEG - 1:
                    upd = _nn(vT[pl.ds(g0, 128), pl.ds(t0, L)], pk[g, pl.ds(t0, L), :])
                    upd = jnp.where(bd, upd, 0.0)
                    zrow_new = zs[pl.ds(s, 1), pl.ds(g0, 128)]
                    if s == 0:
                        macc, zacc = upd, zrow_new
                    else:
                        macc, zacc = macc + upd, zacc + zrow_new
            return c
        lax.fori_loop(0, NG, attn, 0)

        @pl.when(li == 0)
        def _():
            w_copy(3).wait()

        def oproj(i, c):
            r = pl.multiple_of(i * L, L)
            t = _nn(ob[pl.ds(r, L), :], wo[...])
            x1 = xf[pl.ds(r, L), :] + t
            xl = _ln(x1)
            wr = wr_ref[...].astype(F32)
            rs = jnp.sum(xl * wr, axis=1, keepdims=True)
            rr[pl.ds(r, L), :] = jnp.broadcast_to(rs, (L, 128))
            x2 = x1 + xl
            xf[pl.ds(r, L), :] = x2
            ob[pl.ds(r, L), :] = xl.astype(BF16)
            xn[pl.ds(r, L), :] = jnp.where(last, x2, _ln(x2)).astype(BF16)
            return c
        lax.fori_loop(0, NSEG, oproj, 0)

        def out_copy(i):
            return pltpu.make_async_copy(xn.at[pl.ds(i * L, L), :], out_hbm.at[0, pl.ds(i * L, L), :], sem_o.at[i])

        @pl.when(last)
        def _():
            for i in range(NSEG):
                out_copy(i).start()

        @pl.when(li == 0)
        def _():
            w_copy(4).wait()
            w_copy(5).wait()
            w_copy(6).wait()

        rv = rr[...]
        idx = lax.broadcasted_iota(jnp.int32, (S, 128), 0)
        m1 = jnp.max(rv)
        i1 = jnp.clip(jnp.min(jnp.where(rv == m1, idx, S)), 0, S - 1)
        rv2 = jnp.where(idx == i1, -jnp.inf, rv)
        m2 = jnp.max(rv2)
        i2 = jnp.clip(jnp.min(jnp.where(rv2 == m2, idx, S)), 0, S - 1)
        sel = ((i1, m1), (i2, m2))
        g1 = pl.multiple_of((i1 // 16) * 16, 16)
        g2 = pl.multiple_of((i2 // 16) * 16, 16)
        xs = jnp.concatenate([ob[pl.ds(g1, 16), :], ob[pl.ds(g2, 16), :]], axis=0)
        gg = _nn(xs, wg[...])
        uu = _nn(xs, wu[...])
        hh = (gg * (1.0 / (1.0 + jnp.exp(-gg))) * uu).astype(BF16)
        yy = _nn(hh, wd[...])
        riota = lax.broadcasted_iota(jnp.int32, (16, D), 0)
        for j, ((ii, mm), gr) in enumerate(zip(sel, (g1, g2))):
            sig = 1.0 / (1.0 + jnp.exp(-jnp.full((16, D), mm, F32)))
            x2 = xf[pl.ds(gr, 16), :]
            x2 = jnp.where(riota == ii - gr, x2 + yy[16 * j:16 * (j + 1)] * sig, x2)
            xf[pl.ds(gr, 16), :] = x2
            xn[pl.ds(gr, 16), :] = jnp.where(last, x2, _ln(x2)).astype(BF16)

        @pl.when(last)
        def _():
            for i in range(NSEG):
                out_copy(i).wait()
            for gr in (g1, g2):
                cp = pltpu.make_async_copy(xn.at[pl.ds(gr, 16), :], out_hbm.at[0, pl.ds(gr, 16), :], sem_o.at[0])
                cp.start()
                cp.wait()
        return carry

    lax.fori_loop(0, 2, layer, 0)


@jax.jit
def pallas_interleave_layers__memory_aug_infini_attn__moe_arch_mod__prompt_kernel(
    A_x: jax.Array,
    A_wq: jax.Array,
    A_wk: jax.Array,
    A_wv: jax.Array,
    A_wo: jax.Array,
    A_beta: jax.Array,
    B_x: jax.Array,
    B_w_r: jax.Array,
    B_w_gate: jax.Array,
    B_w_up: jax.Array,
    B_w_down: jax.Array,
):
    del B_x
    any_spec = pl.BlockSpec(memory_space=pl.ANY)
    small = lambda shape: pl.BlockSpec(shape, lambda: (0,) * len(shape))
    vm = pltpu.VMEM
    scratch = [
        vm((S, D), BF16),
        vm((S, D), F32),
        vm((S, D), BF16),
        vm((D, D), BF16), vm((D, D), BF16), vm((D, D), BF16), vm((D, D), BF16),
        vm((D, D), BF16), vm((D, D), BF16),
        vm((D, FF), BF16), vm((D, FF), BF16), vm((FF, D), BF16),
        vm((D, S), BF16), vm((D, S), BF16), vm((D, S), BF16),
        vm((NG, S, 128), BF16), vm((NG, S, 128), BF16),
        vm((S, D), BF16),
        vm((8, D), F32),
        vm((D, 128), F32),
        vm((S, 128), F32),
        vm((128, 128), F32),
        pltpu.SemaphoreType.DMA((NSEG,)),
        pltpu.SemaphoreType.DMA((7,)),
        pltpu.SemaphoreType.DMA((NSEG,)),
    ]
    return pl.pallas_call(
        _kernel,
        out_shape=jax.ShapeDtypeStruct((1, S, D), BF16),
        in_specs=[any_spec, any_spec, any_spec, any_spec, any_spec,
                  small((1, H)), small((1, D)), any_spec, any_spec, any_spec],
        out_specs=any_spec,
        scratch_shapes=scratch,
        compiler_params=pltpu.CompilerParams(vmem_limit_bytes=110 * 1024 * 1024),
        name="infini_mod",
    )(A_x, A_wq, A_wk, A_wv, A_wo, A_beta.reshape(1, H), B_w_r.reshape(1, D), B_w_gate, B_w_up, B_w_down)
```

```python
import numpy as np
import jax
import jax.numpy as jnp
from jax import lax
import jax.experimental.pallas as pl
import jax.experimental.pallas.tpu as pltpu

F32 = jnp.float32
BF16 = jnp.bfloat16
U32 = jnp.uint32

S, D, H, NSEG, FF = 2048, 1024, 32, 4, 3584
DH = D // H
L = S // NSEG
NG = D // 128
HPG = 128 // DH
QB = 128
NSB = 16
LOG2E = float(np.log2(np.e))
SCALE = float(np.asarray(DH ** -0.5, dtype=np.float32).astype(jnp.bfloat16).astype(np.float32))
QSCALE = SCALE * LOG2E
MASKV = -1e9 * LOG2E


def _phi(t):
    return jnp.where(t > 0, t + 1.0, jnp.exp(t))


def _ln(x):
    m = jnp.mean(x, axis=-1, keepdims=True)
    xc = x - m
    v = jnp.mean(xc * xc, axis=-1, keepdims=True)
    return xc * lax.rsqrt(v + 1e-5)


def _nt(a, b):
    return lax.dot_general(a, b, (((1,), (1,)), ((), ())), preferred_element_type=F32)


def _nn(a, b):
    return jnp.dot(a, b, preferred_element_type=F32)


def _b16(x):
    return pltpu.bitcast(x, BF16)


def _p32(x):
    return pltpu.bitcast(x.astype(BF16), U32)


def _tree(op, xs):
    xs = list(xs)
    while len(xs) > 1:
        nx = [op(xs[i], xs[i + 1]) for i in range(0, len(xs) - 1, 2)]
        if len(xs) % 2:
            nx.append(xs[-1])
        xs = nx
    return xs[0]


def _vsplit(x):
    return [x[i * 8:(i + 1) * 8] for i in range(x.shape[0] // 8)]


class _Sub:
    def __init__(self, idx, s, qb, h):
        self.idx, self.s, self.qb, self.h = idx, s, qb, h
        self.n = qb + 1


def _attn_plan(order=(3, 2, 1, 0), off=10):
    subs = []
    for s in range(NSEG):
        for qb in order:
            for h in range(HPG):
                subs.append(_Sub(len(subs), s, qb, h))
    tiles = [(u, kt) for u in subs for kt in range(u.n)]
    n = len(tiles)
    first = {}
    for i, (u, kt) in enumerate(tiles):
        if kt == 0:
            first[u.idx] = i
    pos = [first[u.idx] + u.n - 1 + off for (u, kt) in tiles]
    deferred = set((u.s, u.qb) for i, (u, kt) in enumerate(tiles) if pos[i] >= n)
    now, prev = {}, {}
    for i, (u, kt) in enumerate(tiles):
        if (u.s, u.qb) in deferred:
            prev.setdefault(max(pos[i] - n, 0), []).append(i)
        else:
            now.setdefault(pos[i], []).append(i)
    return tiles, now, prev


_PLAN = _attn_plan()


class _Refs:
    pass


def _attn_body(R, g, gp, zero, do_qk=True):
    tiles, now, prev = _PLAN
    krow = lax.broadcasted_iota(jnp.int32, (QB, QB), 0)
    qcol = lax.broadcasted_iota(jnp.int32, (QB, QB), 1)
    maskT = jnp.where(krow > qcol, MASKV, 0.0).astype(F32)
    bd = (krow // DH) == (qcol // DH)
    laneh = lax.broadcasted_iota(jnp.int32, (8, QB), 1) // DH
    st, outs, mem = {}, {}, {}

    def qk(i):
        u, kt = tiles[i]
        t0 = u.s * L
        q0 = t0 + u.qb * QB
        qt = _b16(R.qT[pl.ds(pl.multiple_of(g * 64 + u.h * 16, 16), 16), pl.ds(q0, QB)])
        parts = []
        if u.h > 0:
            parts.append(jnp.zeros((u.h * DH, QB), BF16))
        parts.append(qt)
        if u.h < HPG - 1:
            parts.append(jnp.zeros(((HPG - 1 - u.h) * DH, QB), BF16))
        w = jnp.concatenate(parts, axis=0)
        x = _nn(_b16(R.kk[g, pl.ds((t0 + kt * QB) // 2, QB // 2), :]), w)
        if kt == u.qb:
            x = x + maskT
        buf = R.sb[u.idx % NSB]
        buf[pl.ds(kt * QB, QB), :] = x
        mx = _tree(jnp.maximum, _vsplit(x))
        key = ("m", u.idx)
        st[key] = mx if kt == 0 else jnp.maximum(st[key], mx)
        if kt == u.qb:
            buf[pl.ds(4 * QB, 8), :] = jnp.broadcast_to(jnp.max(st[key], axis=0, keepdims=True), (8, QB))

    def pv(i, gg, tag):
        u, kt = tiles[i]
        t0 = u.s * L
        q0 = t0 + u.qb * QB
        buf = R.sb[u.idx % NSB]
        km, kl, ko = ("mf", u.idx, tag), ("l", u.idx, tag), ("o", u.idx, tag)
        if kt == 0:
            st[km] = buf[pl.ds(pl.multiple_of(4 * QB + zero, 8), 8), :]
        m = st[km]
        x = buf[pl.ds(pl.multiple_of(kt * QB + zero, 8), QB), :]
        p = jnp.concatenate([jnp.exp2(v - m) for v in _vsplit(x)], axis=0)
        ls = _tree(jnp.add, _vsplit(p))
        st[kl] = ls if kt == 0 else st[kl] + ls
        vt = _b16(R.vT[pl.ds(pl.multiple_of(gg * 64 + u.h * 16, 16), 16), pl.ds(t0 + kt * QB, QB)])
        ot = _nn(vt, p.astype(BF16))
        st[ko] = ot if kt == 0 else st[ko] + ot
        if kt == u.qb:
            l = jnp.sum(st[kl], axis=0, keepdims=True)
            adot = st[ko] * (1.0 / l)
            gt = R.gs[pl.ds(pl.multiple_of(gg * 128 + u.h * DH, 8), 8), :]
            gt = jnp.concatenate([1.0 - gt] * 4, axis=0)
            o = gt * adot
            if u.s > 0:
                o = R.am[u.s % 2][pl.ds(pl.multiple_of(u.qb * QB + u.h * DH + zero, 8), DH), :] + o
            lst = outs.setdefault((u.s, u.qb, tag), [])
            lst.append(o)
            if len(lst) == HPG:
                oT = jnp.concatenate(lst, axis=0)
                R.ob[gg, pl.ds(q0 // 2, QB // 2), :] = _p32(oT.T)

    def upd(s):
        t0 = s * L
        lhs = _b16(R.vT[pl.ds(pl.multiple_of(g * 64, 64), 64), pl.ds(t0, L)])
        rhs = _b16(R.pk[g, pl.ds(t0 // 2, L // 2), :])
        u_ = jnp.where(bd, _nn(lhs, rhs), 0.0)
        zr = R.zs[pl.ds(pl.multiple_of(g * 8 * NSEG + s * 8, 8), 8), :]
        if s == 0:
            mem["M"], mem["z"] = u_, zr
        else:
            mem["M"], mem["z"] = mem["M"] + u_, mem["z"] + zr

    def nd(s):
        t0 = s * L
        zl = [jnp.where(laneh == h, mem["z"], 0.0) for h in range(HPG)]
        lhs = jnp.concatenate([mem["M"]] + zl, axis=0).astype(BF16)
        for qb in range(L // QB):
            r = _nn(lhs, _b16(R.pqT[pl.ds(pl.multiple_of(g * 64, 64), 64), pl.ds(t0 + qb * QB, QB)]))
            for h in range(HPG):
                den = r[128 + 8 * h:128 + 8 * h + 8] + 1e-6
                gt = R.gs[pl.ds(pl.multiple_of(g * 128 + h * DH, 8), 8), :] * (1.0 / den)
                R.am[s % 2][pl.ds(qb * QB + h * DH, DH), :] = (
                    r[h * DH:(h + 1) * DH] * jnp.concatenate([gt] * 4, axis=0))

    extra = {}
    if do_qk:
        for s in range(NSEG - 1):
            extra.setdefault(40 * s + 2, []).append(("upd", s))
            extra.setdefault(40 * s + 20, []).append(("nd", s + 1))
    for i in range(len(tiles)):
        if do_qk:
            qk(i)
        for kind, s in extra.get(i, []):
            (upd if kind == "upd" else nd)(s)
        for j in prev.get(i, []):
            pv(j, gp, 0)
        if do_qk:
            for j in now.get(i, []):
                pv(j, g, 1)


def _kernel(x_hbm, wq_hbm, wk_hbm, wv_hbm, wo_hbm, beta_ref, wr_ref, wg_hbm, wu_hbm, wd_hbm,
            out_hbm,
            xin, xf, xn, wq, wk, wv, wo, wqT, wvT, wg, wu, wd,
            qT, pqT, vT, kk, pk, ob, xb, zs, gs, rr, am0, am1, *rest):
    sb = rest[:NSB]
    sem_x, sem_w, sem_o = rest[NSB:]
    R = _Refs()
    R.qT, R.pqT, R.vT, R.kk, R.pk, R.ob, R.zs, R.gs = qT, pqT, vT, kk, pk, ob, zs, gs
    R.am, R.sb = (am0, am1), sb

    def x_copy(i):
        return pltpu.make_async_copy(x_hbm.at[0, pl.ds(i * L, L), :], xin.at[pl.ds(i * L, L), :], sem_x.at[i])

    def w_copy(j):
        src = (wk_hbm, wq_hbm, wv_hbm, wo_hbm, wg_hbm, wu_hbm, wd_hbm)[j]
        dst = (wk, wq, wv, wo, wg, wu, wd)[j]
        return pltpu.make_async_copy(src, dst, sem_w.at[j])

    x_copy(0).start()
    w_copy(0).start()
    w_copy(1).start()
    w_copy(2).start()
    for i in range(1, NSEG):
        x_copy(i).start()
    for j in range(3, 7):
        w_copy(j).start()

    b = beta_ref[...].astype(F32)
    sg = 1.0 / (1.0 + jnp.exp(-b))
    lane = lax.broadcasted_iota(jnp.int32, (1, H), 1)
    for h in range(H):
        gh = jnp.sum(jnp.where(lane == h, sg, 0.0), axis=1, keepdims=True)
        gs[pl.ds(h * DH, DH), :] = jnp.broadcast_to(gh, (DH, 128))
    for buf in sb:
        buf[...] = jnp.zeros(buf.shape, F32)
    am0[...] = jnp.zeros(am0.shape, F32)
    am1[...] = jnp.zeros(am1.shape, F32)

    def ln0(i, c):
        x_copy(i).wait()
        r = pl.multiple_of(i * L, L)
        xv = xin[pl.ds(r, L), :].astype(F32)
        xf[pl.ds(r, L), :] = xv
        xn[pl.ds(r, L), :] = _ln(xv).astype(BF16)
        return c
    lax.fori_loop(0, NSEG, ln0, 0)

    w_copy(0).wait()
    w_copy(1).wait()

    def tr_body(src, dst):
        def body(i, c):
            r = pl.multiple_of(i * 128, 128)
            dst[:, pl.ds(r, 128)] = src[pl.ds(r, 128), :].T
            return c
        lax.fori_loop(0, D // 128, body, 0)
    tr_body(wq, wqT)
    w_copy(2).wait()
    tr_body(wv, wvT)

    def layer(li, carry):
        last = li == 1

        def proj(s, c):
            r = pl.multiple_of(s * L, L)
            r2 = pl.multiple_of(s * (L // 2), L // 2)
            xb_ = xn[pl.ds(r, L), :]
            kf = _nn(xb_, wk[...])
            pf = _phi(kf)
            zrow = jnp.sum(pf, axis=0, keepdims=True)
            for g in range(NG):
                sl = slice(g * 128, (g + 1) * 128)
                kk[g, pl.ds(r2, L // 2), :] = _p32(kf[:, sl])
                pk[g, pl.ds(r2, L // 2), :] = _p32(pf[:, sl])
                zs[pl.ds(pl.multiple_of(g * 8 * NSEG + s * 8, 8), 8), :] = jnp.broadcast_to(zrow[:, sl], (8, 128))
            qf = _nt(wqT[...], xb_)
            qT[:, pl.ds(r, L)] = _p32(qf * QSCALE)
            pqT[:, pl.ds(r, L)] = _p32(_phi(qf))
            vf = _nt(wvT[...], xb_)
            vT[:, pl.ds(r, L)] = _p32(vf)
            return c
        lax.fori_loop(0, NSEG, proj, 0)

        def attn(g, c):
            _attn_body(R, g, jnp.maximum(g - 1, 0), g >> 10)
            return c
        lax.fori_loop(0, NG, attn, 0)
        _attn_body(R, NG - 1, NG - 1, li >> 10, do_qk=False)

        @pl.when(li == 0)
        def _():
            w_copy(3).wait()

        def oproj(i, c):
            r = pl.multiple_of(i * L, L)
            r2 = pl.multiple_of(i * (L // 2), L // 2)
            lhs = jnp.concatenate([_b16(ob[g, pl.ds(r2, L // 2), :]) for g in range(NG)], axis=1)
            t = _nn(lhs, wo[...])
            x1 = xf[pl.ds(r, L), :] + t
            xl = _ln(x1)
            wr = wr_ref[...].astype(F32)
            rs = jnp.sum(xl * wr, axis=1, keepdims=True)
            rr[pl.ds(r, L), :] = jnp.broadcast_to(rs, (L, 128))
            x2 = x1 + xl
            xf[pl.ds(r, L), :] = x2
            xb[pl.ds(r, L), :] = xl.astype(BF16)
            xn[pl.ds(r, L), :] = jnp.where(last, x2, _ln(x2)).astype(BF16)
            return c
        lax.fori_loop(0, NSEG, oproj, 0)

        def out_copy(i):
            return pltpu.make_async_copy(xn.at[pl.ds(i * L, L), :], out_hbm.at[0, pl.ds(i * L, L), :], sem_o.at[i])

        @pl.when(last)
        def _():
            for i in range(NSEG):
                out_copy(i).start()

        @pl.when(li == 0)
        def _():
            w_copy(4).wait()
            w_copy(5).wait()
            w_copy(6).wait()

        rv = rr[...]
        idx = lax.broadcasted_iota(jnp.int32, (S, 128), 0)
        m1 = jnp.max(rv)
        i1 = jnp.clip(jnp.min(jnp.where(rv == m1, idx, S)), 0, S - 1)
        rv2 = jnp.where(idx == i1, -jnp.inf, rv)
        m2 = jnp.max(rv2)
        i2 = jnp.clip(jnp.min(jnp.where(rv2 == m2, idx, S)), 0, S - 1)
        sel = ((i1, m1), (i2, m2))
        g1 = pl.multiple_of((i1 // 16) * 16, 16)
        g2 = pl.multiple_of((i2 // 16) * 16, 16)
        xs = jnp.concatenate([xb[pl.ds(g1, 16), :], xb[pl.ds(g2, 16), :]], axis=0)
        gg = _nn(xs, wg[...])
        uu = _nn(xs, wu[...])
        hh = (gg * (1.0 / (1.0 + jnp.exp(-gg))) * uu).astype(BF16)
        yy = _nn(hh, wd[...])
        riota = lax.broadcasted_iota(jnp.int32, (16, D), 0)
        for j, ((ii, mm), gr) in enumerate(zip(sel, (g1, g2))):
            sig = 1.0 / (1.0 + jnp.exp(-jnp.full((16, D), mm, F32)))
            x2 = xf[pl.ds(gr, 16), :]
            x2 = jnp.where(riota == ii - gr, x2 + yy[16 * j:16 * (j + 1)] * sig, x2)
            xf[pl.ds(gr, 16), :] = x2
            xn[pl.ds(gr, 16), :] = jnp.where(last, x2, _ln(x2)).astype(BF16)

        @pl.when(last)
        def _():
            for i in range(NSEG):
                out_copy(i).wait()
            for gr in (g1, g2):
                cp = pltpu.make_async_copy(xn.at[pl.ds(gr, 16), :], out_hbm.at[0, pl.ds(gr, 16), :], sem_o.at[0])
                cp.start()
                cp.wait()
        return carry

    lax.fori_loop(0, 2, layer, 0)


@jax.jit
def pallas_interleave_layers__memory_aug_infini_attn__moe_arch_mod__prompt_kernel(
    A_x: jax.Array,
    A_wq: jax.Array,
    A_wk: jax.Array,
    A_wv: jax.Array,
    A_wo: jax.Array,
    A_beta: jax.Array,
    B_x: jax.Array,
    B_w_r: jax.Array,
    B_w_gate: jax.Array,
    B_w_up: jax.Array,
    B_w_down: jax.Array,
):
    del B_x
    any_spec = pl.BlockSpec(memory_space=pl.ANY)
    small = lambda shape: pl.BlockSpec(shape, lambda: (0,) * len(shape))
    vm = pltpu.VMEM
    scratch = [
        vm((S, D), BF16),
        vm((S, D), F32),
        vm((S, D), BF16),
        vm((D, D), BF16), vm((D, D), BF16), vm((D, D), BF16), vm((D, D), BF16),
        vm((D, D), BF16), vm((D, D), BF16),
        vm((D, FF), BF16), vm((D, FF), BF16), vm((FF, D), BF16),
        vm((D // 2, S), U32), vm((D // 2, S), U32), vm((D // 2, S), U32),
        vm((NG, S // 2, 128), U32), vm((NG, S // 2, 128), U32),
        vm((NG, S // 2, 128), U32),
        vm((S, D), BF16),
        vm((NG * NSEG * 8, 128), F32),
        vm((D, 128), F32),
        vm((S, 128), F32),
        vm((L, QB), F32), vm((L, QB), F32),
    ] + [vm((4 * QB + 8, QB), F32) for _ in range(NSB)] + [
        pltpu.SemaphoreType.DMA((NSEG,)),
        pltpu.SemaphoreType.DMA((7,)),
        pltpu.SemaphoreType.DMA((NSEG,)),
    ]
    return pl.pallas_call(
        _kernel,
        out_shape=jax.ShapeDtypeStruct((1, S, D), BF16),
        in_specs=[any_spec, any_spec, any_spec, any_spec, any_spec,
                  small((1, H)), small((1, D)), any_spec, any_spec, any_spec],
        out_specs=any_spec,
        scratch_shapes=scratch,
        compiler_params=pltpu.CompilerParams(vmem_limit_bytes=110 * 1024 * 1024),
        name="infini_mod",
    )(A_x, A_wq, A_wk, A_wv, A_wo, A_beta.reshape(1, H), B_w_r.reshape(1, D), B_w_gate, B_w_up, B_w_down)
```

```python
import numpy as np
import jax
import jax.numpy as jnp
from jax import lax
import jax.experimental.pallas as pl
import jax.experimental.pallas.tpu as pltpu

F32 = jnp.float32
BF16 = jnp.bfloat16
U32 = jnp.uint32

S, D, H, NSEG, FF = 2048, 1024, 32, 4, 3584
DH = D // H
L = S // NSEG
NG = D // 128
HPG = 128 // DH
QB = 128
NSB = 16
LOG2E = float(np.log2(np.e))
SCALE = float(np.asarray(DH ** -0.5, dtype=np.float32).astype(jnp.bfloat16).astype(np.float32))
QSCALE = SCALE * LOG2E
MASKV = -1e9 * LOG2E


def _phi(t):
    return jnp.where(t > 0, t + 1.0, jnp.exp(t))


def _ln(x):
    m = jnp.sum(x, axis=-1, keepdims=True) * (1.0 / D)
    xc = x - m
    v = jnp.sum(xc * xc, axis=-1, keepdims=True) * (1.0 / D)
    return xc * lax.rsqrt(v + 1e-5)


def _nt(a, b):
    return lax.dot_general(a, b, (((1,), (1,)), ((), ())), preferred_element_type=F32)


def _nn(a, b):
    return jnp.dot(a, b, preferred_element_type=F32)


def _b16(x):
    return pltpu.bitcast(x, BF16)


def _p32(x):
    return pltpu.bitcast(x.astype(BF16), U32)


def _tree(op, xs):
    xs = list(xs)
    while len(xs) > 1:
        nx = [op(xs[i], xs[i + 1]) for i in range(0, len(xs) - 1, 2)]
        if len(xs) % 2:
            nx.append(xs[-1])
        xs = nx
    return xs[0]


def _vsplit(x):
    return [x[i * 8:(i + 1) * 8] for i in range(x.shape[0] // 8)]


class _Sub:
    def __init__(self, idx, s, qb, h):
        self.idx, self.s, self.qb, self.h = idx, s, qb, h
        self.n = qb + 1


def _attn_plan(order=(3, 2, 1, 0), off=10):
    subs = []
    for s in range(NSEG):
        for qb in order:
            for h in range(HPG):
                subs.append(_Sub(len(subs), s, qb, h))
    tiles = [(u, kt) for u in subs for kt in range(u.n)]
    n = len(tiles)
    first = {}
    for i, (u, kt) in enumerate(tiles):
        if kt == 0:
            first[u.idx] = i
    pos = [first[u.idx] + u.n - 1 + off for (u, kt) in tiles]
    deferred = set((u.s, u.qb) for i, (u, kt) in enumerate(tiles) if pos[i] >= n)
    now, prev = {}, {}
    for i, (u, kt) in enumerate(tiles):
        if (u.s, u.qb) in deferred:
            prev.setdefault(max(pos[i] - n, 0), []).append(i)
        else:
            now.setdefault(pos[i], []).append(i)
    return tiles, now, prev


_PLAN = _attn_plan()


class _Refs:
    pass


def _attn_body(R, g, gp, zero, do_qk=True):
    tiles, now, prev = _PLAN
    krow = lax.broadcasted_iota(jnp.int32, (QB, QB), 0)
    qcol = lax.broadcasted_iota(jnp.int32, (QB, QB), 1)
    maskT = jnp.where(krow > qcol, MASKV, 0.0).astype(F32)
    bd = (krow // DH) == (qcol // DH)
    laneh = lax.broadcasted_iota(jnp.int32, (8, QB), 1) // DH
    st, outs, mem = {}, {}, {}

    def qk(i):
        u, kt = tiles[i]
        t0 = u.s * L
        q0 = t0 + u.qb * QB
        qt = _b16(R.qT[pl.ds(pl.multiple_of(g * 64 + u.h * 16, 16), 16), pl.ds(q0, QB)])
        parts = []
        if u.h > 0:
            parts.append(jnp.zeros((u.h * DH, QB), BF16))
        parts.append(qt)
        if u.h < HPG - 1:
            parts.append(jnp.zeros(((HPG - 1 - u.h) * DH, QB), BF16))
        w = jnp.concatenate(parts, axis=0)
        x = _nn(_b16(R.kk[g, pl.ds((t0 + kt * QB) // 2, QB // 2), :]), w)
        if kt == u.qb:
            x = x + maskT
        buf = R.sb[u.idx % NSB]
        buf[pl.ds(kt * QB, QB), :] = x
        mx = _tree(jnp.maximum, _vsplit(x))
        key = ("m", u.idx)
        st[key] = mx if kt == 0 else jnp.maximum(st[key], mx)
        if kt == u.qb:
            buf[pl.ds(4 * QB, 8), :] = jnp.broadcast_to(jnp.max(st[key], axis=0, keepdims=True), (8, QB))

    def pv(i, gg, tag):
        u, kt = tiles[i]
        t0 = u.s * L
        q0 = t0 + u.qb * QB
        buf = R.sb[u.idx % NSB]
        km, kl, ko = ("mf", u.idx, tag), ("l", u.idx, tag), ("o", u.idx, tag)
        if kt == 0:
            st[km] = buf[pl.ds(pl.multiple_of(4 * QB + zero, 8), 8), :]
        m = st[km]
        x = buf[pl.ds(pl.multiple_of(kt * QB + zero, 8), QB), :]
        p = jnp.concatenate([jnp.exp2(v - m) for v in _vsplit(x)], axis=0)
        ls = _tree(jnp.add, _vsplit(p))
        st[kl] = ls if kt == 0 else st[kl] + ls
        vt = _b16(R.vT[pl.ds(pl.multiple_of(gg * 64 + u.h * 16, 16), 16), pl.ds(t0 + kt * QB, QB)])
        ot = _nn(vt, p.astype(BF16))
        st[ko] = ot if kt == 0 else st[ko] + ot
        if kt == u.qb:
            l = jnp.sum(st[kl], axis=0, keepdims=True)
            adot = st[ko] * (1.0 / l)
            gt = R.gs[pl.ds(pl.multiple_of(gg * 128 + u.h * DH, 8), 8), :]
            gt = jnp.concatenate([1.0 - gt] * 4, axis=0)
            o = gt * adot
            if u.s > 0:
                o = R.am[u.s % 2][pl.ds(pl.multiple_of(u.qb * QB + u.h * DH + zero, 8), DH), :] + o
            lst = outs.setdefault((u.s, u.qb, tag), [])
            lst.append(o)
            if len(lst) == HPG:
                oT = jnp.concatenate(lst, axis=0)
                R.ob[gg, pl.ds(q0 // 2, QB // 2), :] = _p32(oT.T)

    def upd(s):
        t0 = s * L
        lhs = _b16(R.vT[pl.ds(pl.multiple_of(g * 64, 64), 64), pl.ds(t0, L)])
        rhs = _b16(R.pk[g, pl.ds(t0 // 2, L // 2), :])
        u_ = jnp.where(bd, _nn(lhs, rhs), 0.0)
        zr = R.zs[pl.ds(pl.multiple_of(g * 8 * NSEG + s * 8, 8), 8), :]
        if s == 0:
            mem["M"], mem["z"] = u_, zr
        else:
            mem["M"], mem["z"] = mem["M"] + u_, mem["z"] + zr

    def nd(s):
        t0 = s * L
        zl = [jnp.where(laneh == h, mem["z"], 0.0) for h in range(HPG)]
        lhs = jnp.concatenate([mem["M"]] + zl, axis=0).astype(BF16)
        for qb in range(L // QB):
            r = _nn(lhs, _b16(R.pqT[pl.ds(pl.multiple_of(g * 64, 64), 64), pl.ds(t0 + qb * QB, QB)]))
            for h in range(HPG):
                den = r[128 + 8 * h:128 + 8 * h + 8] + 1e-6
                gt = R.gs[pl.ds(pl.multiple_of(g * 128 + h * DH, 8), 8), :] * (1.0 / den)
                R.am[s % 2][pl.ds(qb * QB + h * DH, DH), :] = (
                    r[h * DH:(h + 1) * DH] * jnp.concatenate([gt] * 4, axis=0))

    extra = {}
    if do_qk:
        for s in range(NSEG - 1):
            extra.setdefault(40 * s + 2, []).append(("upd", s))
            extra.setdefault(40 * s + 20, []).append(("nd", s + 1))
    for i in range(len(tiles)):
        if do_qk:
            qk(i)
        for kind, s in extra.get(i, []):
            (upd if kind == "upd" else nd)(s)
        for j in prev.get(i, []):
            pv(j, gp, 0)
        if do_qk:
            for j in now.get(i, []):
                pv(j, g, 1)


def _kernel(x_hbm, wq_hbm, wk_hbm, wv_hbm, wo_hbm, beta_ref, wr_ref, wg_hbm, wu_hbm, wd_hbm,
            out_hbm,
            xin, xr, xw, xn, wall, wo, wT, wg, wu, wd,
            qT, pqT, vT, kk, pk, ob, xb, zs, gs, rr, am0, am1, *rest):
    sb = rest[:NSB]
    sem_x, sem_w, sem_d, sem_o, sem_c = rest[NSB:]
    R = _Refs()
    R.qT, R.pqT, R.vT, R.kk, R.pk, R.ob, R.zs, R.gs = qT, pqT, vT, kk, pk, ob, zs, gs
    R.am, R.sb = (am0, am1), sb

    def x_copy(i):
        return pltpu.make_async_copy(x_hbm.at[0, pl.ds(i * L, L), :], xin.at[pl.ds(i * L, L), :], sem_x.at[i])

    def w_copy(j):
        src = (wk_hbm, wq_hbm, wv_hbm, wo_hbm, wg_hbm, wu_hbm)[j]
        dst = (wall.at[pl.ds(0, D), :], wall.at[pl.ds(D, D), :], wall.at[pl.ds(2 * D, D), :], wo, wg, wu)[j]
        return pltpu.make_async_copy(src, dst, sem_w.at[j])

    def wd_copy(j):
        return pltpu.make_async_copy(wd_hbm.at[:, pl.ds(j * 128, 128)], wd.at[j], sem_d.at[j])

    for i in range(NSEG):
        x_copy(i).start()

    b = beta_ref[...].astype(F32)
    sg = 1.0 / (1.0 + jnp.exp(-b))
    lane = lax.broadcasted_iota(jnp.int32, (1, H), 1)
    for h in range(H):
        gh = jnp.sum(jnp.where(lane == h, sg, 0.0), axis=1, keepdims=True)
        gs[pl.ds(h * DH, DH), :] = jnp.broadcast_to(gh, (DH, 128))
    for buf in sb:
        buf[...] = jnp.zeros(buf.shape, F32)
    am0[...] = jnp.zeros(am0.shape, F32)
    am1[...] = jnp.zeros(am1.shape, F32)

    def ln0(i, c):
        x_copy(i).wait()

        @pl.when(i == 0)
        def _():
            w_copy(0).start()

        @pl.when(i == 1)
        def _():
            w_copy(1).start()
            w_copy(2).start()

        @pl.when(i == 2)
        def _():
            for j in range(3, 6):
                w_copy(j).start()
            for j in range(NG):
                wd_copy(j).start()

        r = pl.multiple_of(i * L, L)
        for k in range(L // 64):
            rows = pl.ds(r + k * 64, 64)
            xv = xin[rows, :].astype(F32)
            xr[rows, :] = xv
            xn[rows, :] = _ln(xv).astype(BF16)
        return c
    lax.fori_loop(0, NSEG, ln0, 0)

    def out_copy(i):
        return pltpu.make_async_copy(xn.at[pl.ds(i * L, L), :], out_hbm.at[0, pl.ds(i * L, L), :], sem_o.at[i])

    x_carry = pltpu.make_async_copy(xw, xr, sem_c.at[0])

    def layer(li, carry):
        first = li == 0
        last = li == 1

        def kproj(s, c):
            for j in range(3):
                @pl.when(jnp.logical_and(first, s == j))
                def _():
                    w_copy(j).wait()
            r = pl.multiple_of(s * L, L)
            r2 = pl.multiple_of(s * (L // 2), L // 2)
            kf = _nn(xn[pl.ds(r, L), :], wall[pl.ds(0, D), :])
            pf = _phi(kf)
            zrow = jnp.sum(pf, axis=0, keepdims=True)
            for g in range(NG):
                sl = slice(g * 128, (g + 1) * 128)
                kk[g, pl.ds(r2, L // 2), :] = _p32(kf[:, sl])
                pk[g, pl.ds(r2, L // 2), :] = _p32(pf[:, sl])
                zs[pl.ds(pl.multiple_of(g * 8 * NSEG + s * 8, 8), 8), :] = jnp.broadcast_to(zrow[:, sl], (8, 128))
            for j in range(6):
                rw = pl.multiple_of((s * 6 + j) * 128, 128)
                wT[:, pl.ds(rw, 128)] = wall[pl.ds(rw, 128), :].T
            return c
        lax.fori_loop(0, NSEG, kproj, 0)

        def qvproj(s, c):
            r = pl.multiple_of(s * L, L)
            xb_ = xn[pl.ds(r, L), :]
            qf = _nt(wT[:, pl.ds(D, D)], xb_)
            qT[:, pl.ds(r, L)] = _p32(qf * QSCALE)
            pqT[:, pl.ds(r, L)] = _p32(_phi(qf))
            vf = _nt(wT[:, pl.ds(2 * D, D)], xb_)
            vT[:, pl.ds(r, L)] = _p32(vf)
            return c
        lax.fori_loop(0, NSEG, qvproj, 0)

        def attn(g, c):
            _attn_body(R, g, jnp.maximum(g - 1, 0), g >> 10)
            return c
        lax.fori_loop(0, NG, attn, 0)
        _attn_body(R, NG - 1, NG - 1, li >> 10, do_qk=False)

        @pl.when(first)
        def _():
            w_copy(3).wait()

        @pl.when(last)
        def _():
            x_carry.wait()

        SUB = 128

        def oproj(i, c):
            r = pl.multiple_of(i * L, L)
            r2 = pl.multiple_of(i * (L // 2), L // 2)
            wr = wr_ref[...].astype(F32)
            lane_i = lax.broadcasted_iota(jnp.int32, (8, 128), 1)
            ts = {}
            racc = jnp.full((8, 128), -jnp.inf, F32)

            def dot(j):
                lhs = jnp.concatenate(
                    [_b16(ob[g, pl.ds(r2 + j * SUB // 2, SUB // 2), :]) for g in range(NG)], axis=1)
                ts[j] = _nn(lhs, wo[...])

            def epi(j, racc):
                rows = pl.ds(r + j * SUB, SUB)
                x1 = xr[rows, :] + ts[j]
                m = jnp.sum(x1, axis=-1, keepdims=True) * (1.0 / D)
                xc = x1 - m
                v = jnp.sum(xc * xc, axis=-1, keepdims=True) * (1.0 / D)
                rstd = lax.rsqrt(v + 1e-5)
                xl = xc * rstd
                rs = jnp.sum(xl * wr, axis=1, keepdims=True)
                for q in range(SUB // 8):
                    racc = jnp.where(lane_i == j * (SUB // 8) + q,
                                     jnp.broadcast_to(rs[q * 8:(q + 1) * 8], (8, 128)), racc)
                x2 = x1 + xl
                xw[rows, :] = x2
                xb[rows, :] = xl.astype(BF16)
                c2 = 1.0 + rstd
                s2 = c2 * lax.rsqrt(v * c2 * c2 + 1e-5)
                xn[rows, :] = jnp.where(last, x2, xc * s2).astype(BF16)
                return racc

            nsub = L // SUB
            for j in range(nsub + 1):
                if j < nsub:
                    dot(j)
                if j >= 1:
                    racc = epi(j - 1, racc)
            rr[pl.ds(pl.multiple_of(i * 8, 8), 8), :] = racc

            @pl.when(last)
            def _():
                out_copy(i).start()
            return c
        lax.fori_loop(0, NSEG, oproj, 0)

        @pl.when(first)
        def _():
            w_copy(4).wait()
            w_copy(5).wait()
            for j in range(NG):
                wd_copy(j).wait()

        rv = rr[...]
        prow = lax.broadcasted_iota(jnp.int32, (NSEG * 8, 128), 0)
        plane = lax.broadcasted_iota(jnp.int32, (NSEG * 8, 128), 1)
        idx = (prow // 8) * L + plane * 8 + prow % 8

        def top1(vals):
            mx = jnp.max(jnp.max(vals, axis=0, keepdims=True), axis=1, keepdims=True)
            cand = jnp.where(vals == mx, idx, S - 1)
            ix = jnp.min(jnp.min(cand, axis=0, keepdims=True), axis=1, keepdims=True)
            return mx, ix

        m1, i1v = top1(rv)
        m2, i2v = top1(jnp.where(idx == i1v, -jnp.inf, rv))
        i1 = jnp.clip(i1v[0, 0], 0, S - 1)
        i2 = jnp.clip(i2v[0, 0], 0, S - 1)
        g1 = pl.multiple_of((i1 // 16) * 16, 16)
        g2 = pl.multiple_of((i2 // 16) * 16, 16)
        xs = jnp.concatenate([xb[pl.ds(g1, 16), :], xb[pl.ds(g2, 16), :]], axis=0)
        gg = _nn(xs, wg[...])
        uu = _nn(xs, wu[...])
        hh = (gg * (1.0 / (1.0 + jnp.exp(-gg))) * uu).astype(BF16)
        yy = jnp.concatenate([_nn(hh, wd[j]) for j in range(NG)], axis=1)
        riota = lax.broadcasted_iota(jnp.int32, (16, D), 0)
        for j, (ii, mm, gr) in enumerate(((i1, m1, g1), (i2, m2, g2))):
            sig = 1.0 / (1.0 + jnp.exp(-mm))
            x2 = xw[pl.ds(gr, 16), :]
            x2 = jnp.where(riota == ii - gr, x2 + yy[16 * j:16 * (j + 1)] * sig, x2)
            xw[pl.ds(gr, 16), :] = x2
            xn[pl.ds(gr, 16), :] = jnp.where(last, x2, _ln(x2)).astype(BF16)

        @pl.when(first)
        def _():
            x_carry.start()

        @pl.when(last)
        def _():
            for i in range(NSEG):
                out_copy(i).wait()
            for gr in (g1, g2):
                cp = pltpu.make_async_copy(xn.at[pl.ds(gr, 16), :], out_hbm.at[0, pl.ds(gr, 16), :], sem_o.at[0])
                cp.start()
                cp.wait()
        return carry

    lax.fori_loop(0, 2, layer, 0)


@jax.jit
def pallas_interleave_layers__memory_aug_infini_attn__moe_arch_mod__prompt_kernel(
    A_x: jax.Array,
    A_wq: jax.Array,
    A_wk: jax.Array,
    A_wv: jax.Array,
    A_wo: jax.Array,
    A_beta: jax.Array,
    B_x: jax.Array,
    B_w_r: jax.Array,
    B_w_gate: jax.Array,
    B_w_up: jax.Array,
    B_w_down: jax.Array,
):
    del B_x
    any_spec = pl.BlockSpec(memory_space=pl.ANY)
    small = lambda shape: pl.BlockSpec(shape, lambda: (0,) * len(shape))
    vm = pltpu.VMEM
    scratch = [
        vm((S, D), BF16),
        vm((S, D), F32),
        vm((S, D), F32),
        vm((S, D), BF16),
        vm((3 * D, D), BF16),
        vm((D, D), BF16),
        vm((D, 3 * D), BF16),
        vm((D, FF), BF16), vm((D, FF), BF16), vm((NG, FF, 128), BF16),
        vm((D // 2, S), U32), vm((D // 2, S), U32), vm((D // 2, S), U32),
        vm((NG, S // 2, 128), U32), vm((NG, S // 2, 128), U32),
        vm((NG, S // 2, 128), U32),
        vm((S, D), BF16),
        vm((NG * NSEG * 8, 128), F32),
        vm((D, 128), F32),
        vm((NSEG * 8, 128), F32),
        vm((L, QB), F32), vm((L, QB), F32),
    ] + [vm((4 * QB + 8, QB), F32) for _ in range(NSB)] + [
        pltpu.SemaphoreType.DMA((NSEG,)),
        pltpu.SemaphoreType.DMA((6,)),
        pltpu.SemaphoreType.DMA((NG,)),
        pltpu.SemaphoreType.DMA((NSEG,)),
        pltpu.SemaphoreType.DMA((1,)),
    ]
    return pl.pallas_call(
        _kernel,
        out_shape=jax.ShapeDtypeStruct((1, S, D), BF16),
        in_specs=[any_spec, any_spec, any_spec, any_spec, any_spec,
                  small((1, H)), small((1, D)), any_spec, any_spec, any_spec],
        out_specs=any_spec,
        scratch_shapes=scratch,
        compiler_params=pltpu.CompilerParams(vmem_limit_bytes=110 * 1024 * 1024),
        name="infini_mod",
    )(A_x, A_wq, A_wk, A_wv, A_wo, A_beta.reshape(1, H), B_w_r.reshape(1, D), B_w_gate, B_w_up, B_w_down)
```

```python
import numpy as np
import jax
import jax.numpy as jnp
from jax import lax
import jax.experimental.pallas as pl
import jax.experimental.pallas.tpu as pltpu

F32 = jnp.float32
BF16 = jnp.bfloat16
U32 = jnp.uint32

S, D, H, NSEG, FF = 2048, 1024, 32, 4, 3584
DH = D // H
L = S // NSEG
NG = D // 128
HPG = 128 // DH
QB = 128
SUB, STRIP, NCHAIN = 64, 16, 1
NSB = 16
LOG2E = float(np.log2(np.e))
SCALE = float(np.asarray(DH ** -0.5, dtype=np.float32).astype(jnp.bfloat16).astype(np.float32))
QSCALE = SCALE * LOG2E
MASKV = -1e9 * LOG2E


def _phi(t):
    return jnp.where(t > 0, t + 1.0, jnp.exp(t))


def _ln(x):
    m = jnp.sum(x, axis=-1, keepdims=True) * (1.0 / D)
    xc = x - m
    v = jnp.sum(xc * xc, axis=-1, keepdims=True) * (1.0 / D)
    return xc * lax.rsqrt(v + 1e-5)


def _nt(a, b):
    return lax.dot_general(a, b, (((1,), (1,)), ((), ())), preferred_element_type=F32)


def _nn(a, b):
    return jnp.dot(a, b, preferred_element_type=F32)


def _b16(x):
    return pltpu.bitcast(x, BF16)


def _p32(x):
    return pltpu.bitcast(x.astype(BF16), U32)


def _tree(op, xs):
    xs = list(xs)
    while len(xs) > 1:
        nx = [op(xs[i], xs[i + 1]) for i in range(0, len(xs) - 1, 2)]
        if len(xs) % 2:
            nx.append(xs[-1])
        xs = nx
    return xs[0]


def _vsplit(x):
    return [x[i * 8:(i + 1) * 8] for i in range(x.shape[0] // 8)]


class _Sub:
    def __init__(self, idx, s, qb, h):
        self.idx, self.s, self.qb, self.h = idx, s, qb, h
        self.n = qb + 1


ORDER, OFF, SLOPE, UPD_AT, ND_AT = (0, 1, 2, 3), 14, 0, 2, 20


def _attn_plan(order=ORDER, off=OFF):
    subs = []
    for s in range(NSEG):
        for qb in order:
            for h in range(HPG):
                subs.append(_Sub(len(subs), s, qb, h))
    tiles = [(u, kt) for u in subs for kt in range(u.n)]
    n = len(tiles)
    first = {}
    for i, (u, kt) in enumerate(tiles):
        if kt == 0:
            first[u.idx] = i
    pos = [first[u.idx] + u.n - 1 + off + int(SLOPE * kt) for (u, kt) in tiles]
    deferred = set((u.s, u.qb) for i, (u, kt) in enumerate(tiles) if pos[i] >= n)
    now, prev = {}, {}
    for i, (u, kt) in enumerate(tiles):
        if (u.s, u.qb) in deferred:
            prev.setdefault(max(pos[i] - n, 0), []).append(i)
        else:
            now.setdefault(pos[i], []).append(i)
    return tiles, now, prev


_PLAN = _attn_plan()


class _Refs:
    pass


def _attn_body(R, g, gp, zero, do_qk=True):
    tiles, now, prev = _PLAN
    krow = lax.broadcasted_iota(jnp.int32, (QB, QB), 0)
    qcol = lax.broadcasted_iota(jnp.int32, (QB, QB), 1)
    maskT = jnp.where(krow > qcol, MASKV, 0.0).astype(F32)
    bd = (krow // DH) == (qcol // DH)
    laneh = lax.broadcasted_iota(jnp.int32, (8, QB), 1) // DH
    st, outs, mem = {}, {}, {}

    def qk(i):
        u, kt = tiles[i]
        t0 = u.s * L
        q0 = t0 + u.qb * QB
        qt = _b16(R.qT[pl.ds(pl.multiple_of(g * 64 + u.h * 16, 16), 16), pl.ds(q0, QB)])
        parts = []
        if u.h > 0:
            parts.append(jnp.zeros((u.h * DH, QB), BF16))
        parts.append(qt)
        if u.h < HPG - 1:
            parts.append(jnp.zeros(((HPG - 1 - u.h) * DH, QB), BF16))
        w = jnp.concatenate(parts, axis=0)
        x = _nn(_b16(R.kk[g, pl.ds((t0 + kt * QB) // 2, QB // 2), :]), w)
        if kt == u.qb:
            x = x + maskT
        buf = R.sb[u.idx % NSB]
        buf[pl.ds(kt * QB, QB), :] = x
        mx = _tree(jnp.maximum, _vsplit(x))
        key = ("m", u.idx)
        st[key] = mx if kt == 0 else jnp.maximum(st[key], mx)
        if kt == u.qb:
            buf[pl.ds(4 * QB, 8), :] = jnp.broadcast_to(jnp.max(st[key], axis=0, keepdims=True), (8, QB))

    def pv(i, gg, tag):
        u, kt = tiles[i]
        t0 = u.s * L
        q0 = t0 + u.qb * QB
        buf = R.sb[u.idx % NSB]
        km, kl, ko = ("mf", u.idx, tag), ("l", u.idx, tag), ("o", u.idx, tag)
        if kt == 0:
            st[km] = buf[pl.ds(pl.multiple_of(4 * QB + zero, 8), 8), :]
        m = st[km]
        x = buf[pl.ds(pl.multiple_of(kt * QB + zero, 8), QB), :]
        p = jnp.concatenate([jnp.exp2(v - m) for v in _vsplit(x)], axis=0)
        ls = _tree(jnp.add, _vsplit(p))
        st[kl] = ls if kt == 0 else st[kl] + ls
        vt = _b16(R.vT[pl.ds(pl.multiple_of(gg * 64 + u.h * 16, 16), 16), pl.ds(t0 + kt * QB, QB)])
        ot = _nn(vt, p.astype(BF16))
        st[ko] = ot if kt == 0 else st[ko] + ot
        if kt == u.qb:
            l = jnp.sum(st[kl], axis=0, keepdims=True)
            adot = st[ko] * (1.0 / l)
            gt = R.gs[pl.ds(pl.multiple_of(gg * 128 + u.h * DH, 8), 8), :]
            gt = jnp.concatenate([1.0 - gt] * 4, axis=0)
            o = gt * adot
            if u.s > 0:
                o = R.am[u.s % 2][pl.ds(pl.multiple_of(u.qb * QB + u.h * DH + zero, 8), DH), :] + o
            lst = outs.setdefault((u.s, u.qb, tag), [])
            lst.append(o)
            if len(lst) == HPG:
                oT = jnp.concatenate(lst, axis=0)
                R.ob[gg, pl.ds(q0 // 2, QB // 2), :] = _p32(oT.T)

    def upd(s):
        t0 = s * L
        lhs = _b16(R.vT[pl.ds(pl.multiple_of(g * 64, 64), 64), pl.ds(t0, L)])
        rhs = _b16(R.pk[g, pl.ds(t0 // 2, L // 2), :])
        u_ = jnp.where(bd, _nn(lhs, rhs), 0.0)
        zr = R.zs[pl.ds(pl.multiple_of(g * 8 * NSEG + s * 8, 8), 8), :]
        if s == 0:
            mem["M"], mem["z"] = u_, zr
        else:
            mem["M"], mem["z"] = mem["M"] + u_, mem["z"] + zr

    def nd(s):
        t0 = s * L
        zl = [jnp.where(laneh == h, mem["z"], 0.0) for h in range(HPG)]
        lhs = jnp.concatenate([mem["M"]] + zl, axis=0).astype(BF16)
        for qb in range(L // QB):
            r = _nn(lhs, _b16(R.pqT[pl.ds(pl.multiple_of(g * 64, 64), 64), pl.ds(t0 + qb * QB, QB)]))
            for h in range(HPG):
                den = r[128 + 8 * h:128 + 8 * h + 8] + 1e-6
                gt = R.gs[pl.ds(pl.multiple_of(g * 128 + h * DH, 8), 8), :] * (1.0 / den)
                R.am[s % 2][pl.ds(qb * QB + h * DH, DH), :] = (
                    r[h * DH:(h + 1) * DH] * jnp.concatenate([gt] * 4, axis=0))

    extra = {}
    if do_qk:
        for s in range(NSEG - 1):
            extra.setdefault(40 * s + UPD_AT, []).append(("upd", s))
            extra.setdefault(40 * s + ND_AT, []).append(("nd", s + 1))
    for i in range(len(tiles)):
        if do_qk:
            qk(i)
        for kind, s in extra.get(i, []):
            (upd if kind == "upd" else nd)(s)
        for j in prev.get(i, []):
            pv(j, gp, 0)
        if do_qk:
            for j in now.get(i, []):
                pv(j, g, 1)


def _kernel(x_hbm, wq_hbm, wk_hbm, wv_hbm, wo_hbm, beta_ref, wr_ref, wg_hbm, wu_hbm, wd_hbm,
            out_hbm,
            xin, xr, xw, xn, wall, wo, wo32, wT, wg, wu, wd,
            qT, pqT, vT, kk, pk, ob, xb, zs, gs, rr, tst, am0, am1, *rest):
    sb = rest[:NSB]
    sem_x, sem_w, sem_d, sem_o, sem_c = rest[NSB:]
    R = _Refs()
    R.qT, R.pqT, R.vT, R.kk, R.pk, R.ob, R.zs, R.gs = qT, pqT, vT, kk, pk, ob, zs, gs
    R.am, R.sb = (am0, am1), sb

    def x_copy(i):
        return pltpu.make_async_copy(x_hbm.at[0, pl.ds(i * L, L), :], xin.at[pl.ds(i * L, L), :], sem_x.at[i])

    def w_copy(j):
        src = (wk_hbm, wq_hbm, wv_hbm, wo_hbm, wg_hbm, wu_hbm)[j]
        dst = (wall.at[pl.ds(0, D), :], wall.at[pl.ds(D, D), :], wall.at[pl.ds(2 * D, D), :], wo, wg, wu)[j]
        return pltpu.make_async_copy(src, dst, sem_w.at[j])

    def wd_copy(j):
        return pltpu.make_async_copy(wd_hbm.at[:, pl.ds(j * 128, 128)], wd.at[j], sem_d.at[j])

    for i in range(NSEG):
        x_copy(i).start()

    b = beta_ref[...].astype(F32)
    sg = 1.0 / (1.0 + jnp.exp(-b))
    lane = lax.broadcasted_iota(jnp.int32, (1, H), 1)
    for h in range(H):
        gh = jnp.sum(jnp.where(lane == h, sg, 0.0), axis=1, keepdims=True)
        gs[pl.ds(h * DH, DH), :] = jnp.broadcast_to(gh, (DH, 128))
    for buf in sb:
        buf[...] = jnp.zeros(buf.shape, F32)
    am0[...] = jnp.zeros(am0.shape, F32)
    am1[...] = jnp.zeros(am1.shape, F32)
    tst[...] = jnp.zeros(tst.shape, F32)
    rr[...] = jnp.zeros(rr.shape, F32)

    def ln0(i, c):
        x_copy(i).wait()

        @pl.when(i == 0)
        def _():
            w_copy(0).start()

        @pl.when(i == 1)
        def _():
            w_copy(1).start()
            w_copy(2).start()

        @pl.when(i == 2)
        def _():
            for j in range(3, 6):
                w_copy(j).start()
            for j in range(NG):
                wd_copy(j).start()

        r = pl.multiple_of(i * L, L)
        for k in range(L // 64):
            rows = pl.ds(r + k * 64, 64)
            xv = xin[rows, :].astype(F32)
            xr[rows, :] = xv
            xn[rows, :] = _ln(xv).astype(BF16)
        return c
    lax.fori_loop(0, NSEG, ln0, 0)

    def out_copy(i):
        return pltpu.make_async_copy(xn.at[pl.ds(i * L, L), :], out_hbm.at[0, pl.ds(i * L, L), :], sem_o.at[i])

    x_carry = pltpu.make_async_copy(xw, xr, sem_c.at[0])

    def layer(li, carry):
        first = li == 0
        last = li == 1

        def kproj(s, c):
            for j in range(3):
                @pl.when(jnp.logical_and(first, s == j))
                def _():
                    w_copy(j).wait()
            r = pl.multiple_of(s * L, L)
            r2 = pl.multiple_of(s * (L // 2), L // 2)
            kf = _nn(xn[pl.ds(r, L), :], wall[pl.ds(0, D), :])
            pf = _phi(kf)
            zrow = jnp.sum(pf, axis=0, keepdims=True)
            for g in range(NG):
                sl = slice(g * 128, (g + 1) * 128)
                kk[g, pl.ds(r2, L // 2), :] = _p32(kf[:, sl])
                pk[g, pl.ds(r2, L // 2), :] = _p32(pf[:, sl])
                zs[pl.ds(pl.multiple_of(g * 8 * NSEG + s * 8, 8), 8), :] = jnp.broadcast_to(zrow[:, sl], (8, 128))
            for j in range(6):
                rw = pl.multiple_of((s * 6 + j) * 128, 128)
                wT[:, pl.ds(rw, 128)] = wall[pl.ds(rw, 128), :].T
            return c
        lax.fori_loop(0, NSEG, kproj, 0)

        @pl.when(first)
        def _():
            w_copy(3).wait()

        def qvproj(s, c):
            r = pl.multiple_of(s * L, L)
            wo32[pl.ds(pl.multiple_of(s * (D // 8), D // 8), D // 8), :] = pltpu.bitcast(
                wo[pl.ds(pl.multiple_of(s * (D // 4), D // 4), D // 4), :], U32)
            xb_ = xn[pl.ds(r, L), :]
            qf = _nt(wT[:, pl.ds(D, D)], xb_)
            qT[:, pl.ds(r, L)] = _p32(qf * QSCALE)
            pqT[:, pl.ds(r, L)] = _p32(_phi(qf))
            vf = _nt(wT[:, pl.ds(2 * D, D)], xb_)
            vT[:, pl.ds(r, L)] = _p32(vf)
            return c
        lax.fori_loop(0, NSEG, qvproj, 0)

        def attn(g, c):
            _attn_body(R, g, jnp.maximum(g - 1, 0), g >> 10)
            return c
        lax.fori_loop(0, NG, attn, 0)
        _attn_body(R, NG - 1, NG - 1, li >> 10, do_qk=False)

        @pl.when(last)
        def _():
            x_carry.wait()

        def o_dot(r2, j):
            lhs = jnp.concatenate(
                [_b16(ob[g, pl.ds(r2 + j * SUB // 2, SUB // 2), :]) for g in range(NG)], axis=1)
            return _nn(lhs, _b16(wo32[...]))

        def o_epilogue(t, r0, lane0, racc, deps, cid0, nchain=NCHAIN):
            wr = wr_ref[...].astype(F32)
            lane_i = lax.broadcasted_iota(jnp.int32, (8, 128), 1)
            for k in range(SUB // STRIP):
                rows = pl.ds(r0 + k * STRIP, STRIP)
                x1 = xr[rows, :] + t[k * STRIP:(k + 1) * STRIP]
                m = jnp.sum(x1, axis=-1, keepdims=True) * (1.0 / D)
                cid = (cid0 + k) % nchain
                if deps.get(cid) is not None:
                    m = m + deps[cid]
                xc = x1 - m
                v = jnp.sum(xc * xc, axis=-1, keepdims=True) * (1.0 / D)
                rstd = lax.rsqrt(v + 1e-5)
                xl = xc * rstd
                rs = jnp.sum(xl * wr, axis=1, keepdims=True)
                for q in range(STRIP // 8):
                    racc = jnp.where(lane_i == lane0 + (k * STRIP) // 8 + q,
                                     jnp.broadcast_to(rs[q * 8:(q + 1) * 8], (8, 128)), racc)
                x2 = x1 + xl
                xw[rows, :] = x2
                xb[rows, :] = xl.astype(BF16)
                c2 = 1.0 + rstd
                s2 = c2 * lax.rsqrt(v * c2 * c2 + 1e-5)
                xn[rows, :] = jnp.where(last, x2, xc * s2).astype(BF16)
                deps[cid] = jnp.minimum(jnp.abs(s2), 0.0)
            return racc

        nsub = L // SUB
        ninf = jnp.full((8, 128), -jnp.inf, F32)

        def oproj(i, c):
            r = pl.multiple_of(i * L, L)
            r2 = pl.multiple_of(i * (L // 2), L // 2)
            ip = jnp.where(i == 0, NSEG - 1, i - 1)
            rp = pl.multiple_of(ip * L + (nsub - 1) * SUB, SUB)
            rr_prev = pl.ds(pl.multiple_of(jnp.where(i == 0, NSEG, i - 1) * 8, 8), 8)
            deps = {}
            t_prev = o_dot(r2, 0)
            rr[rr_prev, :] = o_epilogue(tst[pl.ds(pl.multiple_of(i >> 10, 8), SUB), :], rp,
                                        ((nsub - 1) * SUB) // 8, rr[rr_prev, :], deps, 0)
            racc = ninf
            for j in range(1, nsub):
                t_cur = o_dot(r2, j)
                racc = o_epilogue(t_prev, r + (j - 1) * SUB, ((j - 1) * SUB) // 8, racc, deps,
                                  j * (SUB // STRIP))
                t_prev = t_cur
            tst[...] = t_prev
            rr[pl.ds(pl.multiple_of(i * 8, 8), 8), :] = racc

            @pl.when(jnp.logical_and(last, i > 0))
            def _():
                out_copy(i - 1).start()
            return c
        lax.fori_loop(0, NSEG, oproj, 0)
        rr_last = pl.ds((NSEG - 1) * 8, 8)
        rr[rr_last, :] = o_epilogue(tst[pl.ds(pl.multiple_of(li >> 10, 8), SUB), :], (NSEG - 1) * L + (nsub - 1) * SUB,
                                    ((nsub - 1) * SUB) // 8, rr[rr_last, :], {}, 0, nchain=4)

        @pl.when(last)
        def _():
            out_copy(NSEG - 1).start()

        @pl.when(first)
        def _():
            w_copy(4).wait()
            w_copy(5).wait()
            for j in range(NG):
                wd_copy(j).wait()

        rv = rr[pl.ds(0, NSEG * 8), :]
        prow = lax.broadcasted_iota(jnp.int32, (NSEG * 8, 128), 0)
        plane = lax.broadcasted_iota(jnp.int32, (NSEG * 8, 128), 1)
        idx = (prow // 8) * L + plane * 8 + prow % 8

        def top1(vals):
            mx = jnp.max(jnp.max(vals, axis=0, keepdims=True), axis=1, keepdims=True)
            cand = jnp.where(vals == mx, idx, S - 1)
            ix = jnp.min(jnp.min(cand, axis=0, keepdims=True), axis=1, keepdims=True)
            return mx, ix

        m1, i1v = top1(rv)
        m2, i2v = top1(jnp.where(idx == i1v, -jnp.inf, rv))
        i1 = jnp.clip(i1v[0, 0], 0, S - 1)
        i2 = jnp.clip(i2v[0, 0], 0, S - 1)
        g1 = pl.multiple_of((i1 // 16) * 16, 16)
        g2 = pl.multiple_of((i2 // 16) * 16, 16)
        xs = jnp.concatenate([xb[pl.ds(g1, 16), :], xb[pl.ds(g2, 16), :]], axis=0)
        gg = _nn(xs, wg[...])
        uu = _nn(xs, wu[...])
        hh = (gg * (1.0 / (1.0 + jnp.exp(-gg))) * uu).astype(BF16)
        yy = jnp.concatenate([_nn(hh, wd[j]) for j in range(NG)], axis=1)
        riota = lax.broadcasted_iota(jnp.int32, (16, D), 0)
        for j, (ii, mm, gr) in enumerate(((i1, m1, g1), (i2, m2, g2))):
            sig = 1.0 / (1.0 + jnp.exp(-mm))
            x2 = xw[pl.ds(gr, 16), :]
            x2 = jnp.where(riota == ii - gr, x2 + yy[16 * j:16 * (j + 1)] * sig, x2)
            xw[pl.ds(gr, 16), :] = x2
            xn[pl.ds(gr, 16), :] = jnp.where(last, x2, _ln(x2)).astype(BF16)

        @pl.when(first)
        def _():
            x_carry.start()

        @pl.when(last)
        def _():
            for i in range(NSEG):
                out_copy(i).wait()
            for gr in (g1, g2):
                cp = pltpu.make_async_copy(xn.at[pl.ds(gr, 16), :], out_hbm.at[0, pl.ds(gr, 16), :], sem_o.at[0])
                cp.start()
                cp.wait()
        return carry

    lax.fori_loop(0, 2, layer, 0)


@jax.jit
def pallas_interleave_layers__memory_aug_infini_attn__moe_arch_mod__prompt_kernel(
    A_x: jax.Array,
    A_wq: jax.Array,
    A_wk: jax.Array,
    A_wv: jax.Array,
    A_wo: jax.Array,
    A_beta: jax.Array,
    B_x: jax.Array,
    B_w_r: jax.Array,
    B_w_gate: jax.Array,
    B_w_up: jax.Array,
    B_w_down: jax.Array,
):
    del B_x
    any_spec = pl.BlockSpec(memory_space=pl.ANY)
    small = lambda shape: pl.BlockSpec(shape, lambda: (0,) * len(shape))
    vm = pltpu.VMEM
    scratch = [
        vm((S, D), BF16),
        vm((S, D), F32),
        vm((S, D), F32),
        vm((S, D), BF16),
        vm((3 * D, D), BF16),
        vm((D, D), BF16),
        vm((D // 2, D), U32),
        vm((D, 3 * D), BF16),
        vm((D, FF), BF16), vm((D, FF), BF16), vm((NG, FF, 128), BF16),
        vm((D // 2, S), U32), vm((D // 2, S), U32), vm((D // 2, S), U32),
        vm((NG, S // 2, 128), U32), vm((NG, S // 2, 128), U32),
        vm((NG, S // 2, 128), U32),
        vm((S, D), BF16),
        vm((NG * NSEG * 8, 128), F32),
        vm((D, 128), F32),
        vm(((NSEG + 1) * 8, 128), F32),
        vm((SUB, D), F32),
        vm((L, QB), F32), vm((L, QB), F32),
    ] + [vm((4 * QB + 8, QB), F32) for _ in range(NSB)] + [
        pltpu.SemaphoreType.DMA((NSEG,)),
        pltpu.SemaphoreType.DMA((6,)),
        pltpu.SemaphoreType.DMA((NG,)),
        pltpu.SemaphoreType.DMA((NSEG,)),
        pltpu.SemaphoreType.DMA((1,)),
    ]
    return pl.pallas_call(
        _kernel,
        out_shape=jax.ShapeDtypeStruct((1, S, D), BF16),
        in_specs=[any_spec, any_spec, any_spec, any_spec, any_spec,
                  small((1, H)), small((1, D)), any_spec, any_spec, any_spec],
        out_specs=any_spec,
        scratch_shapes=scratch,
        compiler_params=pltpu.CompilerParams(vmem_limit_bytes=110 * 1024 * 1024),
        name="infini_mod",
    )(A_x, A_wq, A_wk, A_wv, A_wo, A_beta.reshape(1, H), B_w_r.reshape(1, D), B_w_gate, B_w_up, B_w_down)
```

```python
import numpy as np
import jax
import jax.numpy as jnp
from jax import lax
import jax.experimental.pallas as pl
import jax.experimental.pallas.tpu as pltpu

F32 = jnp.float32
BF16 = jnp.bfloat16
U32 = jnp.uint32

S, D, H, NSEG, FF = 2048, 1024, 32, 4, 3584
DH = D // H
L = S // NSEG
NG = D // 128
HPG = 128 // DH
QB = 128
SUB, STRIP, NCHAIN = 64, 16, 1
NSB = 16
LOG2E = float(np.log2(np.e))
SCALE = float(np.asarray(DH ** -0.5, dtype=np.float32).astype(jnp.bfloat16).astype(np.float32))
QSCALE = SCALE * LOG2E
MASKV = -1e9 * LOG2E


def _phi(t):
    return jnp.where(t > 0, t + 1.0, jnp.exp(t))


def _ln(x):
    m = jnp.sum(x, axis=-1, keepdims=True) * (1.0 / D)
    xc = x - m
    v = jnp.sum(xc * xc, axis=-1, keepdims=True) * (1.0 / D)
    return xc * lax.rsqrt(v + 1e-5)


def _nt(a, b):
    return lax.dot_general(a, b, (((1,), (1,)), ((), ())), preferred_element_type=F32)


def _nn(a, b):
    return jnp.dot(a, b, preferred_element_type=F32)


def _b16(x):
    return pltpu.bitcast(x, BF16)


def _p32(x):
    return pltpu.bitcast(x.astype(BF16), U32)


def _mul(i, n):
    return i if isinstance(i, int) else pl.multiple_of(i, n)


def _tree(op, xs):
    xs = list(xs)
    while len(xs) > 1:
        nx = [op(xs[i], xs[i + 1]) for i in range(0, len(xs) - 1, 2)]
        if len(xs) % 2:
            nx.append(xs[-1])
        xs = nx
    return xs[0]


def _vsplit(x):
    return [x[i * 8:(i + 1) * 8] for i in range(x.shape[0] // 8)]


class _Sub:
    def __init__(self, idx, s, qb, h):
        self.idx, self.s, self.qb, self.h = idx, s, qb, h
        self.n = qb + 1


ORDER, OFF, SLOPE, UPD_AT, ND_AT = (0, 1, 2, 3), 14, 0, 2, 20


def _attn_plan(order=ORDER, off=OFF):
    subs = []
    for s in range(NSEG):
        for qb in order:
            for h in range(HPG):
                subs.append(_Sub(len(subs), s, qb, h))
    tiles = [(u, kt) for u in subs for kt in range(u.n)]
    n = len(tiles)
    first = {}
    for i, (u, kt) in enumerate(tiles):
        if kt == 0:
            first[u.idx] = i
    pos = [first[u.idx] + u.n - 1 + off + int(SLOPE * kt) for (u, kt) in tiles]
    deferred = set((u.s, u.qb) for i, (u, kt) in enumerate(tiles) if pos[i] >= n)
    now, prev = {}, {}
    for i, (u, kt) in enumerate(tiles):
        if (u.s, u.qb) in deferred:
            prev.setdefault(max(pos[i] - n, 0), []).append(i)
        else:
            now.setdefault(pos[i], []).append(i)
    return tiles, now, prev


_PLAN = _attn_plan()


class _Refs:
    pass


def _attn_body(R, g, gp, zero, do_qk=True):
    tiles, now, prev = _PLAN
    krow = lax.broadcasted_iota(jnp.int32, (QB, QB), 0)
    qcol = lax.broadcasted_iota(jnp.int32, (QB, QB), 1)
    maskT = jnp.where(krow > qcol, MASKV, 0.0).astype(F32)
    bd = (krow // DH) == (qcol // DH)
    laneh = lax.broadcasted_iota(jnp.int32, (8, QB), 1) // DH
    st, outs, mem = {}, {}, {}

    def qk(i):
        u, kt = tiles[i]
        t0 = u.s * L
        q0 = t0 + u.qb * QB
        qt = _b16(R.qT[pl.ds(pl.multiple_of(g * 64 + u.h * 16, 16), 16), pl.ds(q0, QB)])
        parts = []
        if u.h > 0:
            parts.append(jnp.zeros((u.h * DH, QB), BF16))
        parts.append(qt)
        if u.h < HPG - 1:
            parts.append(jnp.zeros(((HPG - 1 - u.h) * DH, QB), BF16))
        w = jnp.concatenate(parts, axis=0)
        x = _nn(_b16(R.kk[g, pl.ds((t0 + kt * QB) // 2, QB // 2), :]), w)
        if kt == u.qb:
            x = x + maskT
        buf = R.sb[u.idx % NSB]
        buf[pl.ds(kt * QB, QB), :] = x
        mx = _tree(jnp.maximum, _vsplit(x))
        key = ("m", u.idx)
        st[key] = mx if kt == 0 else jnp.maximum(st[key], mx)
        if kt == u.qb:
            buf[pl.ds(4 * QB, 8), :] = jnp.broadcast_to(jnp.max(st[key], axis=0, keepdims=True), (8, QB))

    def pv(i, gg, tag):
        u, kt = tiles[i]
        t0 = u.s * L
        q0 = t0 + u.qb * QB
        buf = R.sb[u.idx % NSB]
        km, kl, ko = ("mf", u.idx, tag), ("l", u.idx, tag), ("o", u.idx, tag)
        if kt == 0:
            st[km] = buf[pl.ds(pl.multiple_of(4 * QB + zero, 8), 8), :]
        m = st[km]
        x = buf[pl.ds(pl.multiple_of(kt * QB + zero, 8), QB), :]
        p = jnp.concatenate([jnp.exp2(v - m) for v in _vsplit(x)], axis=0)
        ls = _tree(jnp.add, _vsplit(p))
        st[kl] = ls if kt == 0 else st[kl] + ls
        vt = _b16(R.vT[pl.ds(pl.multiple_of(gg * 64 + u.h * 16, 16), 16), pl.ds(t0 + kt * QB, QB)])
        ot = _nn(vt, p.astype(BF16))
        st[ko] = ot if kt == 0 else st[ko] + ot
        if kt == u.qb:
            l = jnp.sum(st[kl], axis=0, keepdims=True)
            adot = st[ko] * (1.0 / l)
            gt = R.gs[pl.ds(pl.multiple_of(gg * 128 + u.h * DH, 8), 8), :]
            gt = jnp.concatenate([1.0 - gt] * 4, axis=0)
            o = gt * adot
            if u.s > 0:
                o = R.am[u.s % 2][pl.ds(pl.multiple_of(u.qb * QB + u.h * DH + zero, 8), DH), :] + o
            lst = outs.setdefault((u.s, u.qb, tag), [])
            lst.append(o)
            if len(lst) == HPG:
                oT = jnp.concatenate(lst, axis=0)
                R.ob[gg, pl.ds(q0 // 2, QB // 2), :] = _p32(oT.T)

    def upd(s):
        t0 = s * L
        lhs = _b16(R.vT[pl.ds(pl.multiple_of(g * 64, 64), 64), pl.ds(t0, L)])
        rhs = _b16(R.pk[g, pl.ds(t0 // 2, L // 2), :])
        u_ = jnp.where(bd, _nn(lhs, rhs), 0.0)
        zr = R.zs[pl.ds(pl.multiple_of(g * 8 * NSEG + s * 8, 8), 8), :]
        if s == 0:
            mem["M"], mem["z"] = u_, zr
        else:
            mem["M"], mem["z"] = mem["M"] + u_, mem["z"] + zr

    def nd(s):
        t0 = s * L
        zl = [jnp.where(laneh == h, mem["z"], 0.0) for h in range(HPG)]
        lhs = jnp.concatenate([mem["M"]] + zl, axis=0).astype(BF16)
        for qb in range(L // QB):
            r = _nn(lhs, _b16(R.pqT[pl.ds(pl.multiple_of(g * 64, 64), 64), pl.ds(t0 + qb * QB, QB)]))
            for h in range(HPG):
                den = r[128 + 8 * h:128 + 8 * h + 8] + 1e-6
                gt = R.gs[pl.ds(pl.multiple_of(g * 128 + h * DH, 8), 8), :] * (1.0 / den)
                R.am[s % 2][pl.ds(qb * QB + h * DH, DH), :] = (
                    r[h * DH:(h + 1) * DH] * jnp.concatenate([gt] * 4, axis=0))

    extra = {}
    if do_qk:
        for s in range(NSEG - 1):
            extra.setdefault(40 * s + UPD_AT, []).append(("upd", s))
            extra.setdefault(40 * s + ND_AT, []).append(("nd", s + 1))
    for i in range(len(tiles)):
        if do_qk:
            qk(i)
        for kind, s in extra.get(i, []):
            (upd if kind == "upd" else nd)(s)
        for j in prev.get(i, []):
            pv(j, gp, 0)
        if do_qk:
            for j in now.get(i, []):
                pv(j, g, 1)


def _kernel(x_hbm, wq_hbm, wk_hbm, wv_hbm, wo_hbm, beta_ref, wr_ref, wg_hbm, wu_hbm, wd_hbm,
            out_hbm,
            xin, xw, xn, wall, wo, wo32, wT, wg, wu, wd,
            qT, pqT, vT, kk, pk, ob, xb, zs, gs, rr, tst, wrf, am0, am1, *rest):
    sb = rest[:NSB]
    sem_x, sem_w, sem_d, sem_o = rest[NSB:]
    R = _Refs()
    R.qT, R.pqT, R.vT, R.kk, R.pk, R.ob, R.zs, R.gs = qT, pqT, vT, kk, pk, ob, zs, gs
    R.am, R.sb = (am0, am1), sb
    xo = xin

    def x_copy(i):
        return pltpu.make_async_copy(x_hbm.at[0, pl.ds(i * L, L), :], xin.at[pl.ds(i * L, L), :], sem_x.at[i])

    def w_copy(j):
        src = (wk_hbm, wq_hbm, wv_hbm, wo_hbm, wg_hbm, wu_hbm)[j]
        dst = (wall.at[pl.ds(0, D), :], wall.at[pl.ds(D, D), :], wall.at[pl.ds(2 * D, D), :], wo, wg, wu)[j]
        return pltpu.make_async_copy(src, dst, sem_w.at[j])

    def wd_copy(j):
        return pltpu.make_async_copy(wd_hbm.at[:, pl.ds(j * 128, 128)], wd.at[j], sem_d.at[j])

    def out_copy(i):
        return pltpu.make_async_copy(xo.at[pl.ds(i * L, L), :], out_hbm.at[0, pl.ds(i * L, L), :], sem_o.at[i])

    def issue(i, c):
        for j, (kind, n) in enumerate((("x", 0), ("w", 0), ("x", 1), ("x", 2), ("x", 3))):
            @pl.when(i == j)
            def _():
                (x_copy if kind == "x" else w_copy)(n).start()
        return c
    lax.fori_loop(0, 5, issue, 0)

    b = beta_ref[...].astype(F32).reshape(1, H)
    wrf[...] = jnp.broadcast_to(wr_ref[...].astype(F32).reshape(1, D), (8, D))
    sg = 1.0 / (1.0 + jnp.exp(-b))
    lane = lax.broadcasted_iota(jnp.int32, (1, H), 1)
    for h in range(H):
        gh = jnp.sum(jnp.where(lane == h, sg, 0.0), axis=1, keepdims=True)
        gs[pl.ds(h * DH, DH), :] = jnp.broadcast_to(gh, (DH, 128))
    for buf in sb:
        buf[...] = jnp.zeros(buf.shape, F32)
    am0[...] = jnp.zeros(am0.shape, F32)
    am1[...] = jnp.zeros(am1.shape, F32)
    tst[...] = jnp.zeros(tst.shape, F32)
    rr[...] = jnp.zeros(rr.shape, F32)

    def ln_first(i):
        x_copy(i).wait()
        r = pl.multiple_of(i * L, L)
        r2 = pl.multiple_of(i * (L // 2), L // 2)
        for k in range(L // 16):
            xn[pl.ds(r2 + k * 8, 8), :] = _p32(_ln(xin[pl.ds(r + k * 16, 16), :].astype(F32)))

    ln_first(0)
    for j in range(1, 6):
        w_copy(j).start()
    for j in range(NG):
        wd_copy(j).start()

    def layer(first):

        def kproj(s, c):
            if first:
                @pl.when(s == 0)
                def _():
                    w_copy(0).wait()

                @pl.when(s > 0)
                def _():
                    ln_first(s)

                for j in (1, 2):
                    @pl.when(s == j + 1)
                    def _():
                        w_copy(j).wait()
            r2 = pl.multiple_of(s * (L // 2), L // 2)
            kf = _nn(_b16(xn[pl.ds(r2, L // 2), :]), wall[pl.ds(0, D), :])
            pf = _phi(kf)
            zrow = jnp.sum(pf, axis=0, keepdims=True)
            for g in range(NG):
                sl = slice(g * 128, (g + 1) * 128)
                kk[g, pl.ds(r2, L // 2), :] = _p32(kf[:, sl])
                pk[g, pl.ds(r2, L // 2), :] = _p32(pf[:, sl])
                zs[pl.ds(pl.multiple_of(g * 8 * NSEG + s * 8, 8), 8), :] = jnp.broadcast_to(zrow[:, sl], (8, 128))
            if first:
                for j in range(D // 128):
                    rw = pl.multiple_of(jnp.maximum(s - 1, 0) * D + j * 128, 128)
                    wT[:, pl.ds(rw, 128)] = wall[pl.ds(rw, 128), :].T
            return c
        lax.fori_loop(0, NSEG, kproj, 0)

        if first:
            w_copy(3).wait()

        def qvproj(s, c):
            r = pl.multiple_of(s * L, L)
            r2 = pl.multiple_of(s * (L // 2), L // 2)
            if first:
                wo32[pl.ds(pl.multiple_of(s * (D // 8), D // 8), D // 8), :] = pltpu.bitcast(
                    wo[pl.ds(pl.multiple_of(s * (D // 4), D // 4), D // 4), :], U32)
            xb_ = _b16(xn[pl.ds(r2, L // 2), :])
            qf = _nt(wT[:, pl.ds(D, D)], xb_)
            qT[:, pl.ds(r, L)] = _p32(qf * QSCALE)
            pqT[:, pl.ds(r, L)] = _p32(_phi(qf))
            vf = _nt(wT[:, pl.ds(2 * D, D)], xb_)
            vT[:, pl.ds(r, L)] = _p32(vf)
            return c
        lax.fori_loop(0, NSEG, qvproj, 0)

        def attn(g, c):
            _attn_body(R, g, jnp.maximum(g - 1, 0), g >> 10)
            return c
        lax.fori_loop(0, NG, attn, 0)
        _attn_body(R, NG - 1, NG - 1, 0, do_qk=False)

        def o_dot(r2, j):
            lhs = jnp.concatenate(
                [_b16(ob[g, pl.ds(r2 + j * SUB // 2, SUB // 2), :]) for g in range(NG)], axis=1)
            return _nn(lhs, _b16(wo32[...]))

        def o_epilogue(t, r0, lane0, racc, deps, cid0, nchain=NCHAIN):
            wr = wrf[pl.ds(0, 1), :]
            lane_i = lax.broadcasted_iota(jnp.int32, (8, 128), 1)
            for k in range(SUB // STRIP):
                rows = pl.ds(r0 + k * STRIP, STRIP)
                rows2 = pl.ds(_mul(r0 // 2 + k * (STRIP // 2), STRIP // 2), STRIP // 2)
                xres = xin[rows, :].astype(F32) if first else xw[rows, :]
                x1 = xres + t[k * STRIP:(k + 1) * STRIP]
                m = jnp.sum(x1, axis=-1, keepdims=True) * (1.0 / D)
                cid = (cid0 + k) % nchain
                if deps.get(cid) is not None:
                    m = m + deps[cid]
                xc = x1 - m
                v = jnp.sum(xc * xc, axis=-1, keepdims=True) * (1.0 / D)
                rstd = lax.rsqrt(v + 1e-5)
                xl = xc * rstd
                rs = jnp.sum(xl * wr, axis=1, keepdims=True)
                for q in range(STRIP // 8):
                    racc = jnp.where(lane_i == lane0 + (k * STRIP) // 8 + q,
                                     jnp.broadcast_to(rs[q * 8:(q + 1) * 8], (8, 128)), racc)
                xb[rows2, :] = _p32(xl)
                if first:
                    xw[rows, :] = x1 + xl
                    c2 = 1.0 + rstd
                    s2 = c2 * lax.rsqrt(v * c2 * c2 + 1e-5)
                    xn[rows2, :] = _p32(xc * s2)
                    deps[cid] = jnp.minimum(jnp.abs(s2), 0.0)
                else:
                    xo[rows, :] = (x1 + xl).astype(BF16)
                    deps[cid] = jnp.minimum(jnp.abs(rstd), 0.0)
            return racc

        nsub = L // SUB
        ninf = jnp.full((8, 128), -jnp.inf, F32)

        def oproj(i, c):
            r = pl.multiple_of(i * L, L)
            r2 = pl.multiple_of(i * (L // 2), L // 2)
            ip = jnp.where(i == 0, NSEG - 1, i - 1)
            rp = pl.multiple_of(ip * L + (nsub - 1) * SUB, SUB)
            rr_prev = pl.ds(pl.multiple_of(jnp.where(i == 0, NSEG, i - 1) * 8, 8), 8)
            deps = {}
            t_prev = o_dot(r2, 0)
            rr[rr_prev, :] = o_epilogue(tst[pl.ds(pl.multiple_of(i >> 10, 8), SUB), :], rp,
                                        ((nsub - 1) * SUB) // 8, rr[rr_prev, :], deps, 0)
            racc = ninf
            for j in range(1, nsub):
                t_cur = o_dot(r2, j)
                racc = o_epilogue(t_prev, r + (j - 1) * SUB, ((j - 1) * SUB) // 8, racc, deps,
                                  j * (SUB // STRIP))
                t_prev = t_cur
            tst[...] = t_prev
            rr[pl.ds(pl.multiple_of(i * 8, 8), 8), :] = racc

            if not first:
                @pl.when(i > 0)
                def _():
                    out_copy(i - 1).start()
            return c
        lax.fori_loop(0, NSEG, oproj, 0)
        rr_last = pl.ds((NSEG - 1) * 8, 8)
        rr[rr_last, :] = o_epilogue(tst[...], (NSEG - 1) * L + (nsub - 1) * SUB,
                                    ((nsub - 1) * SUB) // 8, rr[rr_last, :], {}, 0, nchain=4)
        if not first:
            out_copy(NSEG - 1).start()

        if first:
            w_copy(4).wait()
            w_copy(5).wait()
            for j in range(NG):
                wd_copy(j).wait()

        rv = rr[pl.ds(0, NSEG * 8), :]
        prow = lax.broadcasted_iota(jnp.int32, (NSEG * 8, 128), 0)
        plane = lax.broadcasted_iota(jnp.int32, (NSEG * 8, 128), 1)
        idx = (prow // 8) * L + plane * 8 + prow % 8

        def top1(vals):
            mx = jnp.max(jnp.max(vals, axis=0, keepdims=True), axis=1, keepdims=True)
            cand = jnp.where(vals == mx, idx, S - 1)
            ix = jnp.min(jnp.min(cand, axis=0, keepdims=True), axis=1, keepdims=True)
            return mx, ix

        m1, i1v = top1(rv)
        m2, i2v = top1(jnp.where(idx == i1v, -jnp.inf, rv))
        i1 = jnp.clip(i1v[0, 0], 0, S - 1)
        i2 = jnp.clip(i2v[0, 0], 0, S - 1)
        g1 = pl.multiple_of((i1 // 16) * 16, 16)
        g2 = pl.multiple_of((i2 // 16) * 16, 16)
        xs = jnp.concatenate([_b16(xb[pl.ds(pl.multiple_of(g1 // 2, 8), 8), :]),
                              _b16(xb[pl.ds(pl.multiple_of(g2 // 2, 8), 8), :])], axis=0)
        gg = _nn(xs, wg[...])
        uu = _nn(xs, wu[...])
        hh = (gg * (1.0 / (1.0 + jnp.exp(-gg))) * uu).astype(BF16)
        yy = jnp.concatenate([_nn(hh, wd[j]) for j in range(NG)], axis=1)
        riota = lax.broadcasted_iota(jnp.int32, (16, D), 0)
        if not first:
            for i in range(NSEG):
                out_copy(i).wait()
        for j, (ii, mm, gr) in enumerate(((i1, m1, g1), (i2, m2, g2))):
            sig = 1.0 / (1.0 + jnp.exp(-mm))
            upd_ = yy[16 * j:16 * (j + 1)] * sig
            if first:
                x2 = xw[pl.ds(gr, 16), :]
                x2 = jnp.where(riota == ii - gr, x2 + upd_, x2)
                xw[pl.ds(gr, 16), :] = x2
                xn[pl.ds(pl.multiple_of(gr // 2, 8), 8), :] = _p32(_ln(x2))
            else:
                x2 = xo[pl.ds(gr, 16), :].astype(F32)
                xo[pl.ds(gr, 16), :] = jnp.where(riota == ii - gr, x2 + upd_, x2).astype(BF16)
                cp = pltpu.make_async_copy(xo.at[pl.ds(gr, 16), :], out_hbm.at[0, pl.ds(gr, 16), :], sem_o.at[0])
                cp.start()
                cp.wait()

    layer(True)
    layer(False)


@jax.jit
def pallas_interleave_layers__memory_aug_infini_attn__moe_arch_mod__prompt_kernel(
    A_x: jax.Array,
    A_wq: jax.Array,
    A_wk: jax.Array,
    A_wv: jax.Array,
    A_wo: jax.Array,
    A_beta: jax.Array,
    B_x: jax.Array,
    B_w_r: jax.Array,
    B_w_gate: jax.Array,
    B_w_up: jax.Array,
    B_w_down: jax.Array,
):
    del B_x
    any_spec = pl.BlockSpec(memory_space=pl.ANY)
    small = lambda shape: pl.BlockSpec(shape, lambda: (0,) * len(shape))
    vm = pltpu.VMEM
    scratch = [
        vm((S, D), BF16),
        vm((S, D), F32),
        vm((S // 2, D), U32),
        vm((3 * D, D), BF16),
        vm((D, D), BF16),
        vm((D // 2, D), U32),
        vm((D, 3 * D), BF16),
        vm((D, FF), BF16), vm((D, FF), BF16), vm((NG, FF, 128), BF16),
        vm((D // 2, S), U32), vm((D // 2, S), U32), vm((D // 2, S), U32),
        vm((NG, S // 2, 128), U32), vm((NG, S // 2, 128), U32),
        vm((NG, S // 2, 128), U32),
        vm((S // 2, D), U32),
        vm((NG * NSEG * 8, 128), F32),
        vm((D, 128), F32),
        vm(((NSEG + 1) * 8, 128), F32),
        vm((SUB, D), F32),
        vm((8, D), F32),
        vm((L, QB), F32), vm((L, QB), F32),
    ] + [vm((4 * QB + 8, QB), F32) for _ in range(NSB)] + [
        pltpu.SemaphoreType.DMA((NSEG,)),
        pltpu.SemaphoreType.DMA((6,)),
        pltpu.SemaphoreType.DMA((NG,)),
        pltpu.SemaphoreType.DMA((NSEG,)),
    ]
    return pl.pallas_call(
        _kernel,
        out_shape=jax.ShapeDtypeStruct((1, S, D), BF16),
        in_specs=[any_spec, any_spec, any_spec, any_spec, any_spec,
                  small((H,)), small((D,)), any_spec, any_spec, any_spec],
        out_specs=any_spec,
        scratch_shapes=scratch,
        compiler_params=pltpu.CompilerParams(vmem_limit_bytes=110 * 1024 * 1024),
        name="infini_mod",
    )(A_x, A_wq, A_wk, A_wv, A_wo, A_beta, B_w_r, B_w_gate, B_w_up, B_w_down)
```

```python
import numpy as np
import jax
import jax.numpy as jnp
from jax import lax
import jax.experimental.pallas as pl
import jax.experimental.pallas.tpu as pltpu

F32 = jnp.float32
BF16 = jnp.bfloat16
U32 = jnp.uint32

S, D, H, NSEG, FF = 2048, 1024, 32, 4, 3584
DH = D // H
L = S // NSEG
NG = D // 128
HPG = 128 // DH
QB = 128
SUB, STRIP, NCHAIN = 64, 16, 1
LN_CHAIN, LN_FIRST = 4, True


def LNK(a, b):
    if LN_FIRST:
        a(); b()
    else:
        b(); a()


NSB = 16
LOG2E = float(np.log2(np.e))
SCALE = float(np.asarray(DH ** -0.5, dtype=np.float32).astype(jnp.bfloat16).astype(np.float32))
QSCALE = SCALE * LOG2E
MASKV = -1e9 * LOG2E


def _phi(t):
    return jnp.where(t > 0, t + 1.0, jnp.exp(t))


def _ln(x):
    m = jnp.sum(x, axis=-1, keepdims=True) * (1.0 / D)
    xc = x - m
    v = jnp.sum(xc * xc, axis=-1, keepdims=True) * (1.0 / D)
    return xc * lax.rsqrt(v + 1e-5)


def _nt(a, b):
    return lax.dot_general(a, b, (((1,), (1,)), ((), ())), preferred_element_type=F32)


def _nn(a, b):
    return jnp.dot(a, b, preferred_element_type=F32)


def _b16(x):
    return pltpu.bitcast(x, BF16)


def _p32(x):
    return pltpu.bitcast(x.astype(BF16), U32)


def _mul(i, n):
    return i if isinstance(i, int) else pl.multiple_of(i, n)


def _tree(op, xs):
    xs = list(xs)
    while len(xs) > 1:
        nx = [op(xs[i], xs[i + 1]) for i in range(0, len(xs) - 1, 2)]
        if len(xs) % 2:
            nx.append(xs[-1])
        xs = nx
    return xs[0]


def _vsplit(x):
    return [x[i * 8:(i + 1) * 8] for i in range(x.shape[0] // 8)]


class _Sub:
    def __init__(self, idx, s, qb, h):
        self.idx, self.s, self.qb, self.h = idx, s, qb, h
        self.n = qb + 1


ORDER, OFF, SLOPE, UPD_AT, ND_AT = (0, 1, 2, 3), 14, 0, 2, 20


def _attn_plan(order=ORDER, off=OFF):
    subs = []
    for s in range(NSEG):
        for qb in order:
            for h in range(HPG):
                subs.append(_Sub(len(subs), s, qb, h))
    tiles = [(u, kt) for u in subs for kt in range(u.n)]
    n = len(tiles)
    first = {}
    for i, (u, kt) in enumerate(tiles):
        if kt == 0:
            first[u.idx] = i
    pos = [first[u.idx] + u.n - 1 + off + int(SLOPE * kt) for (u, kt) in tiles]
    deferred = set((u.s, u.qb) for i, (u, kt) in enumerate(tiles) if pos[i] >= n)
    now, prev = {}, {}
    for i, (u, kt) in enumerate(tiles):
        if (u.s, u.qb) in deferred:
            prev.setdefault(max(pos[i] - n, 0), []).append(i)
        else:
            now.setdefault(pos[i], []).append(i)
    return tiles, now, prev


_PLAN = _attn_plan()


class _Refs:
    pass


def _attn_body(R, g, gp, zero, do_qk=True):
    tiles, now, prev = _PLAN
    krow = lax.broadcasted_iota(jnp.int32, (QB, QB), 0)
    qcol = lax.broadcasted_iota(jnp.int32, (QB, QB), 1)
    maskT = jnp.where(krow > qcol, MASKV, 0.0).astype(F32)
    bd = (krow // DH) == (qcol // DH)
    laneh = lax.broadcasted_iota(jnp.int32, (8, QB), 1) // DH
    st, outs, mem = {}, {}, {}

    def qk(i):
        u, kt = tiles[i]
        t0 = u.s * L
        q0 = t0 + u.qb * QB
        qt = _b16(R.qT[pl.ds(pl.multiple_of(g * 64 + u.h * 16, 16), 16), pl.ds(q0, QB)])
        parts = []
        if u.h > 0:
            parts.append(jnp.zeros((u.h * DH, QB), BF16))
        parts.append(qt)
        if u.h < HPG - 1:
            parts.append(jnp.zeros(((HPG - 1 - u.h) * DH, QB), BF16))
        w = jnp.concatenate(parts, axis=0)
        x = _nn(_b16(R.kk[g, pl.ds((t0 + kt * QB) // 2, QB // 2), :]), w)
        if kt == u.qb:
            x = x + maskT
        buf = R.sb[u.idx % NSB]
        buf[pl.ds(kt * QB, QB), :] = x
        mx = _tree(jnp.maximum, _vsplit(x))
        key = ("m", u.idx)
        st[key] = mx if kt == 0 else jnp.maximum(st[key], mx)
        if kt == u.qb:
            buf[pl.ds(4 * QB, 8), :] = jnp.broadcast_to(jnp.max(st[key], axis=0, keepdims=True), (8, QB))

    def pv(i, gg, tag):
        u, kt = tiles[i]
        t0 = u.s * L
        q0 = t0 + u.qb * QB
        buf = R.sb[u.idx % NSB]
        km, kl, ko = ("mf", u.idx, tag), ("l", u.idx, tag), ("o", u.idx, tag)
        if kt == 0:
            st[km] = buf[pl.ds(pl.multiple_of(4 * QB + zero, 8), 8), :]
        m = st[km]
        x = buf[pl.ds(pl.multiple_of(kt * QB + zero, 8), QB), :]
        p = jnp.concatenate([jnp.exp2(v - m) for v in _vsplit(x)], axis=0)
        ls = _tree(jnp.add, _vsplit(p))
        st[kl] = ls if kt == 0 else st[kl] + ls
        vt = _b16(R.vT[pl.ds(pl.multiple_of(gg * 64 + u.h * 16, 16), 16), pl.ds(t0 + kt * QB, QB)])
        ot = _nn(vt, p.astype(BF16))
        st[ko] = ot if kt == 0 else st[ko] + ot
        if kt == u.qb:
            l = jnp.sum(st[kl], axis=0, keepdims=True)
            adot = st[ko] * (1.0 / l)
            gt = R.gs[pl.ds(pl.multiple_of(gg * 128 + u.h * DH, 8), 8), :]
            gt = jnp.concatenate([1.0 - gt] * 4, axis=0)
            o = gt * adot
            if u.s > 0:
                o = R.am[u.s % 2][pl.ds(pl.multiple_of(u.qb * QB + u.h * DH + zero, 8), DH), :] + o
            lst = outs.setdefault((u.s, u.qb, tag), [])
            lst.append(o)
            if len(lst) == HPG:
                oT = jnp.concatenate(lst, axis=0)
                R.ob[gg, pl.ds(q0 // 2, QB // 2), :] = _p32(oT.T)

    def upd(s):
        t0 = s * L
        lhs = _b16(R.vT[pl.ds(pl.multiple_of(g * 64, 64), 64), pl.ds(t0, L)])
        rhs = _b16(R.pk[g, pl.ds(t0 // 2, L // 2), :])
        u_ = jnp.where(bd, _nn(lhs, rhs), 0.0)
        zr = R.zs[pl.ds(pl.multiple_of(g * 8 * NSEG + s * 8, 8), 8), :]
        if s == 0:
            mem["M"], mem["z"] = u_, zr
        else:
            mem["M"], mem["z"] = mem["M"] + u_, mem["z"] + zr

    def nd(s):
        t0 = s * L
        zl = [jnp.where(laneh == h, mem["z"], 0.0) for h in range(HPG)]
        lhs = jnp.concatenate([mem["M"]] + zl, axis=0).astype(BF16)
        for qb in range(L // QB):
            r = _nn(lhs, _b16(R.pqT[pl.ds(pl.multiple_of(g * 64, 64), 64), pl.ds(t0 + qb * QB, QB)]))
            for h in range(HPG):
                den = r[128 + 8 * h:128 + 8 * h + 8] + 1e-6
                gt = R.gs[pl.ds(pl.multiple_of(g * 128 + h * DH, 8), 8), :] * (1.0 / den)
                R.am[s % 2][pl.ds(qb * QB + h * DH, DH), :] = (
                    r[h * DH:(h + 1) * DH] * jnp.concatenate([gt] * 4, axis=0))

    extra = {}
    if do_qk:
        for s in range(NSEG - 1):
            extra.setdefault(40 * s + UPD_AT, []).append(("upd", s))
            extra.setdefault(40 * s + ND_AT, []).append(("nd", s + 1))
    for i in range(len(tiles)):
        if do_qk:
            qk(i)
        for kind, s in extra.get(i, []):
            (upd if kind == "upd" else nd)(s)
        for j in prev.get(i, []):
            pv(j, gp, 0)
        if do_qk:
            for j in now.get(i, []):
                pv(j, g, 1)


def _kernel(x_hbm, wq_hbm, wk_hbm, wv_hbm, wo_hbm, beta_ref, wr_ref, wg_hbm, wu_hbm, wd_hbm,
            out_hbm,
            xin, xw, xn, xne, xno, wall, wo, wo32, wT, wg, wu, wd,
            qT, pqT, vT, kk, pk, ob, xb, zs, gs, rr, tst, wrf, am0, am1, *rest):
    sb = rest[:NSB]
    sem_x, sem_w, sem_d, sem_o = rest[NSB:]
    R = _Refs()
    R.qT, R.pqT, R.vT, R.kk, R.pk, R.ob, R.zs, R.gs = qT, pqT, vT, kk, pk, ob, zs, gs
    R.am, R.sb = (am0, am1), sb
    xo = xin

    def x_copy(i):
        return pltpu.make_async_copy(x_hbm.at[0, pl.ds(i * L, L), :], xin.at[pl.ds(i * L, L), :], sem_x.at[i])

    def w_copy(j):
        src = (wk_hbm, wq_hbm, wv_hbm, wo_hbm, wg_hbm, wu_hbm)[j]
        dst = (wall.at[pl.ds(0, D), :], wall.at[pl.ds(D, D), :], wall.at[pl.ds(2 * D, D), :], wo, wg, wu)[j]
        return pltpu.make_async_copy(src, dst, sem_w.at[j])

    def wd_copy(j):
        return pltpu.make_async_copy(wd_hbm.at[:, pl.ds(j * 128, 128)], wd.at[j], sem_d.at[j])

    def out_copy(i):
        return pltpu.make_async_copy(xo.at[pl.ds(i * L, L), :], out_hbm.at[0, pl.ds(i * L, L), :], sem_o.at[i])

    x_copy(0).start()
    w_copy(0).start()

    b = beta_ref[...].astype(F32).reshape(1, H)
    wrf[...] = jnp.broadcast_to(wr_ref[...].astype(F32).reshape(1, D), (8, D))
    sg = 1.0 / (1.0 + jnp.exp(-b))
    lane = lax.broadcasted_iota(jnp.int32, (1, H), 1)
    for h in range(H):
        gh = jnp.sum(jnp.where(lane == h, sg, 0.0), axis=1, keepdims=True)
        gs[pl.ds(h * DH, DH), :] = jnp.broadcast_to(gh, (DH, 128))
    for buf in sb:
        buf[...] = jnp.zeros(buf.shape, F32)
    am0[...] = jnp.zeros(am0.shape, F32)
    am1[...] = jnp.zeros(am1.shape, F32)
    tst[...] = jnp.zeros(tst.shape, F32)
    rr[...] = jnp.zeros(rr.shape, F32)

    def ln_first(blk, dst, dblk, nchain=0):
        r = _mul(blk * L, L)
        r2 = _mul(blk * (L // 2), L // 2)
        d2 = _mul(dblk * (L // 2), L // 2)
        deps = {}
        for k in range(L // 16):
            xv = xin[pl.ds(r + k * 16, 16), :].astype(F32)
            m = jnp.sum(xv, axis=-1, keepdims=True) * (1.0 / D)
            if nchain and k >= nchain:
                m = m + deps[k % nchain]
            xc = xv - m
            rstd = lax.rsqrt(jnp.sum(xc * xc, axis=-1, keepdims=True) * (1.0 / D) + 1e-5)
            v = _p32(xc * rstd)
            xn[pl.ds(r2 + k * 8, 8), :] = v
            dst[pl.ds(d2 + k * 8, 8), :] = v
            if nchain:
                deps[k % nchain] = jnp.minimum(jnp.abs(rstd), 0.0)

    x_copy(0).wait()
    ln_first(0, xne, 0)

    order = [("x", 1), ("x", 2), ("x", 3)] + [("w", j) for j in range(1, 6)] + [("d", j) for j in range(NG)]

    def issue(i, c):
        for j, (kind, n) in enumerate(order):
            @pl.when(i == j)
            def _():
                {"x": x_copy, "w": w_copy, "d": wd_copy}[kind](n).start()
        return c
    lax.fori_loop(0, len(order), issue, 0)

    def layer(first):

        def kproj_main(s, src, sblk):
            r2 = pl.multiple_of(s * (L // 2), L // 2)
            xa = _b16(src[pl.ds(_mul(sblk * (L // 2), L // 2), L // 2), :])
            kf = _nn(xa, wall[pl.ds(0, D), :])
            pf = _phi(kf)
            zrow = jnp.sum(pf, axis=0, keepdims=True)
            for g in range(NG):
                sl = slice(g * 128, (g + 1) * 128)
                kk[g, pl.ds(r2, L // 2), :] = _p32(kf[:, sl])
                pk[g, pl.ds(r2, L // 2), :] = _p32(pf[:, sl])
                zs[pl.ds(pl.multiple_of(g * 8 * NSEG + s * 8, 8), 8), :] = jnp.broadcast_to(zrow[:, sl], (8, 128))
            if first:
                for j in range(D // 128):
                    rw = pl.multiple_of(jnp.maximum(s - 1, 0) * D + j * 128, 128)
                    wT[:, pl.ds(rw, 128)] = wall[pl.ds(rw, 128), :].T

        def kproj(s, c):
            if not first:
                kproj_main(s, xn, s)
                return c

            @pl.when(s == 0)
            def _():
                w_copy(0).wait()

            @pl.when(s < NSEG - 1)
            def _():
                x_copy(s + 1).wait()

            for j in (1, 2):
                @pl.when(s == j + 1)
                def _():
                    w_copy(j).wait()

            nxt = jnp.minimum(s + 1, NSEG - 1)

            @pl.when(s % 2 == 0)
            def _():
                LNK(lambda: ln_first(nxt, xno, s // 2, LN_CHAIN), lambda: kproj_main(s, xne, s // 2))

            @pl.when(s % 2 == 1)
            def _():
                LNK(lambda: ln_first(nxt, xne, s // 2 + 1, LN_CHAIN), lambda: kproj_main(s, xno, s // 2))
            return c
        lax.fori_loop(0, NSEG, kproj, 0)

        if first:
            w_copy(3).wait()

        def qvproj(s, c):
            r = pl.multiple_of(s * L, L)
            r2 = pl.multiple_of(s * (L // 2), L // 2)
            if first:
                wo32[pl.ds(pl.multiple_of(s * (D // 8), D // 8), D // 8), :] = pltpu.bitcast(
                    wo[pl.ds(pl.multiple_of(s * (D // 4), D // 4), D // 4), :], U32)
            xb_ = _b16(xn[pl.ds(r2, L // 2), :])
            qf = _nt(wT[:, pl.ds(D, D)], xb_)
            qT[:, pl.ds(r, L)] = _p32(qf * QSCALE)
            pqT[:, pl.ds(r, L)] = _p32(_phi(qf))
            vf = _nt(wT[:, pl.ds(2 * D, D)], xb_)
            vT[:, pl.ds(r, L)] = _p32(vf)
            return c
        lax.fori_loop(0, NSEG, qvproj, 0)

        def attn(g, c):
            _attn_body(R, g, jnp.maximum(g - 1, 0), g >> 10)
            return c
        lax.fori_loop(0, NG, attn, 0)
        _attn_body(R, NG - 1, NG - 1, 0, do_qk=False)

        def o_dot(r2, j):
            lhs = jnp.concatenate(
                [_b16(ob[g, pl.ds(r2 + j * SUB // 2, SUB // 2), :]) for g in range(NG)], axis=1)
            return _nn(lhs, _b16(wo32[...]))

        def o_epilogue(t, r0, lane0, racc, deps, cid0, nchain=NCHAIN):
            wr = wrf[pl.ds(0, 1), :]
            lane_i = lax.broadcasted_iota(jnp.int32, (8, 128), 1)
            for k in range(SUB // STRIP):
                rows = pl.ds(r0 + k * STRIP, STRIP)
                rows2 = pl.ds(_mul(r0 // 2 + k * (STRIP // 2), STRIP // 2), STRIP // 2)
                xres = xin[rows, :].astype(F32) if first else xw[rows, :]
                x1 = xres + t[k * STRIP:(k + 1) * STRIP]
                m = jnp.sum(x1, axis=-1, keepdims=True) * (1.0 / D)
                cid = (cid0 + k) % nchain
                if deps.get(cid) is not None:
                    m = m + deps[cid]
                xc = x1 - m
                v = jnp.sum(xc * xc, axis=-1, keepdims=True) * (1.0 / D)
                rstd = lax.rsqrt(v + 1e-5)
                xl = xc * rstd
                rs = jnp.sum(xl * wr, axis=1, keepdims=True)
                for q in range(STRIP // 8):
                    racc = jnp.where(lane_i == lane0 + (k * STRIP) // 8 + q,
                                     jnp.broadcast_to(rs[q * 8:(q + 1) * 8], (8, 128)), racc)
                xb[rows2, :] = _p32(xl)
                if first:
                    xw[rows, :] = x1 + xl
                    c2 = 1.0 + rstd
                    s2 = c2 * lax.rsqrt(v * c2 * c2 + 1e-5)
                    xn[rows2, :] = _p32(xc * s2)
                    deps[cid] = jnp.minimum(jnp.abs(s2), 0.0)
                else:
                    xo[rows, :] = (x1 + xl).astype(BF16)
                    deps[cid] = jnp.minimum(jnp.abs(rstd), 0.0)
            return racc

        nsub = L // SUB
        ninf = jnp.full((8, 128), -jnp.inf, F32)

        def oproj(i, c):
            r = pl.multiple_of(i * L, L)
            r2 = pl.multiple_of(i * (L // 2), L // 2)
            ip = jnp.where(i == 0, NSEG - 1, i - 1)
            rp = pl.multiple_of(ip * L + (nsub - 1) * SUB, SUB)
            rr_prev = pl.ds(pl.multiple_of(jnp.where(i == 0, NSEG, i - 1) * 8, 8), 8)
            deps = {}
            t_prev = o_dot(r2, 0)
            rr[rr_prev, :] = o_epilogue(tst[pl.ds(pl.multiple_of(i >> 10, 8), SUB), :], rp,
                                        ((nsub - 1) * SUB) // 8, rr[rr_prev, :], deps, 0)
            racc = ninf
            for j in range(1, nsub):
                t_cur = o_dot(r2, j)
                racc = o_epilogue(t_prev, r + (j - 1) * SUB, ((j - 1) * SUB) // 8, racc, deps,
                                  j * (SUB // STRIP))
                t_prev = t_cur
            tst[...] = t_prev
            rr[pl.ds(pl.multiple_of(i * 8, 8), 8), :] = racc

            if not first:
                @pl.when(i > 0)
                def _():
                    out_copy(i - 1).start()
            return c
        lax.fori_loop(0, NSEG, oproj, 0)
        rr_last = pl.ds((NSEG - 1) * 8, 8)
        rr[rr_last, :] = o_epilogue(tst[...], (NSEG - 1) * L + (nsub - 1) * SUB,
                                    ((nsub - 1) * SUB) // 8, rr[rr_last, :], {}, 0, nchain=4)
        if not first:
            out_copy(NSEG - 1).start()

        if first:
            w_copy(4).wait()
            w_copy(5).wait()
            for j in range(NG):
                wd_copy(j).wait()

        rv = rr[pl.ds(0, NSEG * 8), :]
        prow = lax.broadcasted_iota(jnp.int32, (NSEG * 8, 128), 0)
        plane = lax.broadcasted_iota(jnp.int32, (NSEG * 8, 128), 1)
        idx = (prow // 8) * L + plane * 8 + prow % 8

        def top1(vals):
            mx = jnp.max(jnp.max(vals, axis=0, keepdims=True), axis=1, keepdims=True)
            cand = jnp.where(vals == mx, idx, S - 1)
            ix = jnp.min(jnp.min(cand, axis=0, keepdims=True), axis=1, keepdims=True)
            return mx, ix

        m1, i1v = top1(rv)
        m2, i2v = top1(jnp.where(idx == i1v, -jnp.inf, rv))
        i1 = jnp.clip(i1v[0, 0], 0, S - 1)
        i2 = jnp.clip(i2v[0, 0], 0, S - 1)
        g1 = pl.multiple_of((i1 // 16) * 16, 16)
        g2 = pl.multiple_of((i2 // 16) * 16, 16)
        xs = jnp.concatenate([_b16(xb[pl.ds(pl.multiple_of(g1 // 2, 8), 8), :]),
                              _b16(xb[pl.ds(pl.multiple_of(g2 // 2, 8), 8), :])], axis=0)
        gg = _nn(xs, wg[...])
        uu = _nn(xs, wu[...])
        hh = (gg * (1.0 / (1.0 + jnp.exp(-gg))) * uu).astype(BF16)
        yy = jnp.concatenate([_nn(hh, wd[j]) for j in range(NG)], axis=1)
        riota = lax.broadcasted_iota(jnp.int32, (16, D), 0)
        if not first:
            for i in range(NSEG):
                out_copy(i).wait()
        for j, (ii, mm, gr) in enumerate(((i1, m1, g1), (i2, m2, g2))):
            sig = 1.0 / (1.0 + jnp.exp(-mm))
            upd_ = yy[16 * j:16 * (j + 1)] * sig
            if first:
                x2 = xw[pl.ds(gr, 16), :]
                x2 = jnp.where(riota == ii - gr, x2 + upd_, x2)
                xw[pl.ds(gr, 16), :] = x2
                xn[pl.ds(pl.multiple_of(gr // 2, 8), 8), :] = _p32(_ln(x2))
            else:
                x2 = xo[pl.ds(gr, 16), :].astype(F32)
                xo[pl.ds(gr, 16), :] = jnp.where(riota == ii - gr, x2 + upd_, x2).astype(BF16)
                cp = pltpu.make_async_copy(xo.at[pl.ds(gr, 16), :], out_hbm.at[0, pl.ds(gr, 16), :], sem_o.at[0])
                cp.start()
                cp.wait()

    layer(True)
    layer(False)


@jax.jit
def pallas_interleave_layers__memory_aug_infini_attn__moe_arch_mod__prompt_kernel(
    A_x: jax.Array,
    A_wq: jax.Array,
    A_wk: jax.Array,
    A_wv: jax.Array,
    A_wo: jax.Array,
    A_beta: jax.Array,
    B_x: jax.Array,
    B_w_r: jax.Array,
    B_w_gate: jax.Array,
    B_w_up: jax.Array,
    B_w_down: jax.Array,
):
    del B_x
    any_spec = pl.BlockSpec(memory_space=pl.ANY)
    small = lambda shape: pl.BlockSpec(shape, lambda: (0,) * len(shape))
    vm = pltpu.VMEM
    scratch = [
        vm((S, D), BF16),
        vm((S, D), F32),
        vm((S // 2, D), U32),
        vm((3 * L // 2, D), U32), vm((L, D), U32),
        vm((3 * D, D), BF16),
        vm((D, D), BF16),
        vm((D // 2, D), U32),
        vm((D, 3 * D), BF16),
        vm((D, FF), BF16), vm((D, FF), BF16), vm((NG, FF, 128), BF16),
        vm((D // 2, S), U32), vm((D // 2, S), U32), vm((D // 2, S), U32),
        vm((NG, S // 2, 128), U32), vm((NG, S // 2, 128), U32),
        vm((NG, S // 2, 128), U32),
        vm((S // 2, D), U32),
        vm((NG * NSEG * 8, 128), F32),
        vm((D, 128), F32),
        vm(((NSEG + 1) * 8, 128), F32),
        vm((SUB, D), F32),
        vm((8, D), F32),
        vm((L, QB), F32), vm((L, QB), F32),
    ] + [vm((4 * QB + 8, QB), F32) for _ in range(NSB)] + [
        pltpu.SemaphoreType.DMA((NSEG,)),
        pltpu.SemaphoreType.DMA((6,)),
        pltpu.SemaphoreType.DMA((NG,)),
        pltpu.SemaphoreType.DMA((NSEG,)),
    ]
    return pl.pallas_call(
        _kernel,
        out_shape=jax.ShapeDtypeStruct((1, S, D), BF16),
        in_specs=[any_spec, any_spec, any_spec, any_spec, any_spec,
                  small((H,)), small((D,)), any_spec, any_spec, any_spec],
        out_specs=any_spec,
        scratch_shapes=scratch,
        compiler_params=pltpu.CompilerParams(vmem_limit_bytes=110 * 1024 * 1024),
        name="infini_mod",
    )(A_x, A_wq, A_wk, A_wv, A_wo, A_beta, B_w_r, B_w_gate, B_w_up, B_w_down)
```

```python
import numpy as np
import jax
import jax.numpy as jnp
from jax import lax
import jax.experimental.pallas as pl
import jax.experimental.pallas.tpu as pltpu

F32 = jnp.float32
BF16 = jnp.bfloat16
U32 = jnp.uint32

S, D, H, NSEG, FF = 2048, 1024, 32, 4, 3584
DH = D // H
L = S // NSEG
NG = D // 128
HPG = 128 // DH
QB = 128
SUB, STRIP, NCHAIN = 64, 16, 1
LN_CHAIN = 4


NSB = 16
LOG2E = float(np.log2(np.e))
SCALE = float(np.asarray(DH ** -0.5, dtype=np.float32).astype(jnp.bfloat16).astype(np.float32))
QSCALE = SCALE * LOG2E
MASKV = -1e9 * LOG2E


def _phi(t):
    return jnp.where(t > 0, t + 1.0, jnp.exp(t))


def _ln(x):
    m = jnp.sum(x, axis=-1, keepdims=True) * (1.0 / D)
    xc = x - m
    v = jnp.sum(xc * xc, axis=-1, keepdims=True) * (1.0 / D)
    return xc * lax.rsqrt(v + 1e-5)


def _nt(a, b):
    return lax.dot_general(a, b, (((1,), (1,)), ((), ())), preferred_element_type=F32)


def _nn(a, b):
    return jnp.dot(a, b, preferred_element_type=F32)


def _b16(x):
    return pltpu.bitcast(x, BF16)


def _p32(x):
    return pltpu.bitcast(x.astype(BF16), U32)


def _mul(i, n):
    return i if isinstance(i, int) else pl.multiple_of(i, n)


def _tree(op, xs):
    xs = list(xs)
    while len(xs) > 1:
        nx = [op(xs[i], xs[i + 1]) for i in range(0, len(xs) - 1, 2)]
        if len(xs) % 2:
            nx.append(xs[-1])
        xs = nx
    return xs[0]


def _vsplit(x):
    return [x[i * 8:(i + 1) * 8] for i in range(x.shape[0] // 8)]


class _Sub:
    def __init__(self, idx, s, qb, h):
        self.idx, self.s, self.qb, self.h = idx, s, qb, h
        self.n = qb + 1


ORDER, OFF, SLOPE, UPD_AT, ND_AT = (0, 1, 2, 3), 16, 0, 10, 30


def _attn_plan(order=ORDER, off=OFF):
    subs = []
    for s in range(NSEG):
        for qb in order:
            for h in range(HPG):
                subs.append(_Sub(len(subs), s, qb, h))
    tiles = [(u, kt) for u in subs for kt in range(u.n)]
    n = len(tiles)
    first = {}
    for i, (u, kt) in enumerate(tiles):
        if kt == 0:
            first[u.idx] = i
    pos = [first[u.idx] + u.n - 1 + off + int(SLOPE * kt) for (u, kt) in tiles]
    deferred = set((u.s, u.qb) for i, (u, kt) in enumerate(tiles) if pos[i] >= n)
    now, prev = {}, {}
    for i, (u, kt) in enumerate(tiles):
        if (u.s, u.qb) in deferred:
            prev.setdefault(max(pos[i] - n, 0), []).append(i)
        else:
            now.setdefault(pos[i], []).append(i)
    return tiles, now, prev


_PLAN = _attn_plan()


class _Refs:
    pass


def _attn_body(R, g, gp, zero, do_qk=True):
    tiles, now, prev = _PLAN
    krow = lax.broadcasted_iota(jnp.int32, (QB, QB), 0)
    qcol = lax.broadcasted_iota(jnp.int32, (QB, QB), 1)
    bd = (krow // DH) == (qcol // DH)
    laneh = lax.broadcasted_iota(jnp.int32, (8, QB), 1) // DH
    st, outs, mem = {}, {}, {}

    HB = QB // 2
    lo8 = lax.broadcasted_iota(jnp.int32, (8, QB), 1) < HB
    tri = jnp.where(krow[:HB] > qcol[:HB] % HB, MASKV, 0.0).astype(F32)
    swap = lambda v: pltpu.roll(v, HB, 1)

    def put(u, kt, x):
        buf = R.sb[u.idx % NSB]
        buf[pl.ds(kt * QB, QB), :] = x
        mx = _tree(jnp.maximum, _vsplit(x))
        key = ("m", u.idx)
        st[key] = jnp.maximum(st[key], mx) if key in st else mx
        if kt == (u.qb if (u.h % 2 == 0 or u.qb == 0) else u.qb - 1):
            buf[pl.ds(4 * QB, 8), :] = jnp.broadcast_to(jnp.max(st[key], axis=0, keepdims=True), (8, QB))

    def qk(i):
        u, kt = tiles[i]
        t0 = u.s * L
        q0 = t0 + u.qb * QB
        qrow = lambda ref, h: ref[pl.ds(pl.multiple_of(g * 64 + h * 16, 16), 16), pl.ds(q0, QB)]
        k0 = (t0 + kt * QB) // 2
        if kt < u.qb:
            parts = []
            if u.h > 0:
                parts.append(jnp.zeros((u.h * 16, QB), U32))
            parts.append(qrow(R.qT, u.h))
            if u.h < HPG - 1:
                parts.append(jnp.zeros(((HPG - 1 - u.h) * 16, QB), U32))
            put(u, kt, _nn(_b16(R.kk[g, pl.ds(k0, QB // 2), :]), _b16(jnp.concatenate(parts, axis=0))))
            return
        if u.h % 2 == 1:
            return
        lane16 = lax.broadcasted_iota(jnp.int32, (16, QB), 1) < HB
        z = jnp.uint32(0)

        def packed(rows, wa, wb):
            parts = []
            if u.h > 0:
                parts.append(jnp.zeros((u.h * 16, QB), U32))
            parts += [jnp.where(lane16, wa, z), jnp.where(lane16, z, wb)]
            if u.h < HPG - 2:
                parts.append(jnp.zeros(((HPG - 2 - u.h) * 16, QB), U32))
            return _nn(_b16(R.kk[g, pl.ds(k0, rows // 2), :]), _b16(jnp.concatenate(parts, axis=0)))

        X = packed(QB, qrow(R.qS, u.h), qrow(R.qT, u.h + 1))
        Y = packed(HB, qrow(R.qT, u.h), qrow(R.qS, u.h + 1)) + tri
        X0, X1 = _vsplit(X[:HB]), _vsplit(X[HB:] + tri)
        Y = _vsplit(Y)
        put(u, kt, jnp.concatenate([jnp.where(lo8, y, swap(x)) for x, y in zip(X0, Y)]
                                   + [jnp.where(lo8, MASKV, swap(x)) for x in X1], axis=0))
        put(tiles[i + 1 + u.qb][0], kt,
            jnp.concatenate([jnp.where(lo8, swap(y), x) for x, y in zip(X0, Y)]
                            + [jnp.where(lo8, MASKV, x) for x in X1], axis=0))

    def pv(i, gg, tag):
        u, kt = tiles[i]
        t0 = u.s * L
        q0 = t0 + u.qb * QB
        buf = R.sb[u.idx % NSB]
        km, kl, ko = ("mf", u.idx, tag), ("l", u.idx, tag), ("o", u.idx, tag)
        if kt == 0:
            st[km] = buf[pl.ds(pl.multiple_of(4 * QB + zero, 8), 8), :]
        m = st[km]
        x = buf[pl.ds(pl.multiple_of(kt * QB + zero, 8), QB), :]
        p = jnp.concatenate([jnp.exp2(v - m) for v in _vsplit(x)], axis=0)
        ls = _tree(jnp.add, _vsplit(p))
        st[kl] = ls if kt == 0 else st[kl] + ls
        vt = _b16(R.vT[pl.ds(pl.multiple_of(gg * 64 + u.h * 16, 16), 16), pl.ds(t0 + kt * QB, QB)])
        ot = _nn(vt, p.astype(BF16))
        st[ko] = ot if kt == 0 else st[ko] + ot
        if kt == u.qb:
            l = jnp.sum(st[kl], axis=0, keepdims=True)
            adot = st[ko] * (1.0 / l)
            gt = R.gs[pl.ds(pl.multiple_of(gg * 128 + u.h * DH, 8), 8), :]
            gt = jnp.concatenate([1.0 - gt] * 4, axis=0)
            o = gt * adot
            if u.s > 0:
                o = R.am[u.s % 2][pl.ds(pl.multiple_of(u.qb * QB + u.h * DH + zero, 8), DH), :] + o
            lst = outs.setdefault((u.s, u.qb, tag), [])
            lst.append(o)
            if len(lst) == HPG:
                oT = jnp.concatenate(lst, axis=0)
                R.ob[gg, pl.ds(q0 // 2, QB // 2), :] = _p32(oT.T)

    def upd(s):
        t0 = s * L
        lhs = _b16(R.vT[pl.ds(pl.multiple_of(g * 64, 64), 64), pl.ds(t0, L)])
        rhs = _b16(R.pk[g, pl.ds(t0 // 2, L // 2), :])
        u_ = jnp.where(bd, _nn(lhs, rhs), 0.0)
        zr = R.zs[pl.ds(pl.multiple_of(g * 8 * NSEG + s * 8, 8), 8), :]
        if s == 0:
            mem["M"], mem["z"] = u_, zr
        else:
            mem["M"], mem["z"] = mem["M"] + u_, mem["z"] + zr

    def nd(s):
        t0 = s * L
        zl = [jnp.where(laneh == h, mem["z"], 0.0) for h in range(HPG)]
        lhs = jnp.concatenate([mem["M"]] + zl, axis=0).astype(BF16)
        for qb in range(L // QB):
            r = _nn(lhs, _b16(R.pqT[pl.ds(pl.multiple_of(g * 64, 64), 64), pl.ds(t0 + qb * QB, QB)]))
            for h in range(HPG):
                den = r[128 + 8 * h:128 + 8 * h + 8] + 1e-6
                gt = R.gs[pl.ds(pl.multiple_of(g * 128 + h * DH, 8), 8), :] * (1.0 / den)
                R.am[s % 2][pl.ds(qb * QB + h * DH, DH), :] = (
                    r[h * DH:(h + 1) * DH] * jnp.concatenate([gt] * 4, axis=0))

    extra = {}
    if do_qk:
        for s in range(NSEG - 1):
            extra.setdefault(40 * s + UPD_AT, []).append(("upd", s))
            extra.setdefault(40 * s + ND_AT, []).append(("nd", s + 1))
    for i in range(len(tiles)):
        if do_qk:
            qk(i)
        for kind, s in extra.get(i, []):
            (upd if kind == "upd" else nd)(s)
        for j in prev.get(i, []):
            pv(j, gp, 0)
        if do_qk:
            for j in now.get(i, []):
                pv(j, g, 1)


def _kernel(x_hbm, wq_hbm, wk_hbm, wv_hbm, wo_hbm, beta_ref, wr_ref, wg_hbm, wu_hbm, wd_hbm,
            out_hbm,
            xin, xw, xn, wall, wo, wo32, wT, wg, wu, wd,
            qT, qS, pqT, vT, kk, pk, ob, xb, zs, gs, rr, tst, wrf, am0, am1, *rest):
    sb = rest[:NSB]
    sem_x, sem_w, sem_d, sem_o = rest[NSB:]
    R = _Refs()
    R.qS = qS
    R.qT, R.pqT, R.vT, R.kk, R.pk, R.ob, R.zs, R.gs = qT, pqT, vT, kk, pk, ob, zs, gs
    R.am, R.sb = (am0, am1), sb
    xo = xin

    def x_copy(i):
        return pltpu.make_async_copy(x_hbm.at[0, pl.ds(i * L, L), :], xin.at[pl.ds(i * L, L), :], sem_x.at[i])

    def w_copy(j):
        half = lambda ref, c: ref.at[pl.ds(0, D), pl.ds(c * (D // 2), D // 2)]
        src = (half(wk_hbm, 0), wq_hbm, wv_hbm, wo_hbm, wg_hbm, wu_hbm, half(wk_hbm, 1))[j]
        dst = (half(wall, 0), wall.at[pl.ds(D, D), :], wall.at[pl.ds(2 * D, D), :], wo, wg, wu, half(wall, 1))[j]
        return pltpu.make_async_copy(src, dst, sem_w.at[j])

    def wd_copy(j):
        return pltpu.make_async_copy(wd_hbm.at[:, pl.ds(j * 128, 128)], wd.at[j], sem_d.at[j])

    def out_copy(i):
        return pltpu.make_async_copy(xo.at[pl.ds(i * L, L), :], out_hbm.at[0, pl.ds(i * L, L), :], sem_o.at[i])

    x_copy(0).start()
    w_copy(0).start()

    b = beta_ref[...].astype(F32).reshape(1, H)
    wrf[...] = jnp.broadcast_to(wr_ref[...].astype(F32).reshape(1, D), (8, D))
    sg = 1.0 / (1.0 + jnp.exp(-b))
    lane = lax.broadcasted_iota(jnp.int32, (1, H), 1)
    for h in range(H):
        gh = jnp.sum(jnp.where(lane == h, sg, 0.0), axis=1, keepdims=True)
        gs[pl.ds(h * DH, DH), :] = jnp.broadcast_to(gh, (DH, 128))
    for buf in sb:
        buf[...] = jnp.zeros(buf.shape, F32)
    am0[...] = jnp.zeros(am0.shape, F32)
    am1[...] = jnp.zeros(am1.shape, F32)
    tst[...] = jnp.zeros(tst.shape, F32)
    rr[...] = jnp.zeros(rr.shape, F32)

    def ln_first(blk, nchain=0):
        deps = {}
        for k in range(L // 16):
            xv = xin[pl.ds(blk * L + k * 16, 16), :].astype(F32)
            m = jnp.sum(xv, axis=-1, keepdims=True) * (1.0 / D)
            if nchain and k >= nchain:
                m = m + deps[k % nchain]
            xc = xv - m
            rstd = lax.rsqrt(jnp.sum(xc * xc, axis=-1, keepdims=True) * (1.0 / D) + 1e-5)
            xn[pl.ds(blk * (L // 2) + k * 8, 8), :] = _p32(xc * rstd)
            if nchain:
                deps[k % nchain] = jnp.minimum(jnp.abs(rstd), 0.0)

    x_copy(0).wait()
    ln_first(0)

    order = ([("w", 6), ("x", 1), ("x", 2), ("x", 3)] + [("w", j) for j in range(1, 6)]
             + [("d", j) for j in range(NG)])

    def issue(i, c):
        for j, (kind, n) in enumerate(order):
            @pl.when(i == j)
            def _():
                {"x": x_copy, "w": w_copy, "d": wd_copy}[kind](n).start()
        return c
    lax.fori_loop(0, len(order), issue, 0)

    def layer(first):

        def kproj_main(s, g0=0, g1=NG):
            r2 = _mul(s * (L // 2), L // 2)
            kf = _nn(_b16(xn[pl.ds(r2, L // 2), :]), wall[pl.ds(0, D), pl.ds(g0 * 128, (g1 - g0) * 128)])
            pf = _phi(kf)
            zrow = jnp.sum(pf, axis=0, keepdims=True)
            for g in range(g0, g1):
                sl = slice((g - g0) * 128, (g - g0 + 1) * 128)
                kk[g, pl.ds(r2, L // 2), :] = _p32(kf[:, sl])
                pk[g, pl.ds(r2, L // 2), :] = _p32(pf[:, sl])
                zs[pl.ds(_mul(g * 8 * NSEG + s * 8, 8), 8), :] = jnp.broadcast_to(zrow[:, sl], (8, 128))

        def transpose_w(j):
            for c_ in range(D // 128):
                rw = j * D + c_ * 128
                wT[:, pl.ds(rw, 128)] = wall[pl.ds(rw, 128), :].T

        def kproj_first(step, c):
            @pl.when(step == 0)
            def _():
                w_copy(0).wait()
                kproj_main(0, 0, NG // 2)

            @pl.when(step == 1)
            def _():
                w_copy(6).wait()
                kproj_main(0, NG // 2, NG)

            @pl.when(step == 2)
            def _():
                x_copy(1).wait()
                ln_first(1)

            @pl.when(step == 3)
            def _():
                x_copy(2).wait()
                ln_first(2, LN_CHAIN)
                kproj_main(1)

            @pl.when(step == 4)
            def _():
                x_copy(3).wait()
                w_copy(1).wait()
                ln_first(3, LN_CHAIN)
                kproj_main(2)
                transpose_w(1)

            @pl.when(step == 5)
            def _():
                w_copy(2).wait()
                kproj_main(3)
                transpose_w(2)
            return c

        def kproj(s, c):
            kproj_main(s)
            return c

        if first:
            lax.fori_loop(0, 6, kproj_first, 0)
        else:
            lax.fori_loop(0, NSEG, kproj, 0)

        if first:
            w_copy(3).wait()

        def qvproj(s, c):
            r = pl.multiple_of(s * L, L)
            r2 = pl.multiple_of(s * (L // 2), L // 2)
            if first:
                wo32[pl.ds(pl.multiple_of(s * (D // 8), D // 8), D // 8), :] = pltpu.bitcast(
                    wo[pl.ds(pl.multiple_of(s * (D // 4), D // 4), D // 4), :], U32)
            xb_ = _b16(xn[pl.ds(r2, L // 2), :])
            qf = _nt(wT[:, pl.ds(D, D)], xb_)
            q16 = _p32(qf * QSCALE)
            qT[:, pl.ds(r, L)] = q16
            for c_ in range(L // QB):
                qS[:, pl.ds(r + c_ * QB, QB)] = pltpu.roll(q16[:, c_ * QB:(c_ + 1) * QB], QB // 2, 1)
            pqT[:, pl.ds(r, L)] = _p32(_phi(qf))
            vf = _nt(wT[:, pl.ds(2 * D, D)], xb_)
            vT[:, pl.ds(r, L)] = _p32(vf)
            return c
        lax.fori_loop(0, NSEG, qvproj, 0)

        def attn(g, c):
            _attn_body(R, g, jnp.maximum(g - 1, 0), g >> 10)
            return c
        lax.fori_loop(0, NG, attn, 0)
        _attn_body(R, NG - 1, NG - 1, 0, do_qk=False)

        def o_dot(r2, j):
            lhs = jnp.concatenate(
                [_b16(ob[g, pl.ds(r2 + j * SUB // 2, SUB // 2), :]) for g in range(NG)], axis=1)
            return _nn(lhs, _b16(wo32[...]))

        def o_epilogue(t, r0, lane0, racc, deps, cid0, nchain=NCHAIN):
            wr = wrf[pl.ds(0, 1), :]
            lane_i = lax.broadcasted_iota(jnp.int32, (8, 128), 1)
            for k in range(SUB // STRIP):
                rows = pl.ds(r0 + k * STRIP, STRIP)
                rows2 = pl.ds(_mul(r0 // 2 + k * (STRIP // 2), STRIP // 2), STRIP // 2)
                xres = xin[rows, :].astype(F32) if first else xw[rows, :]
                x1 = xres + t[k * STRIP:(k + 1) * STRIP]
                m = jnp.sum(x1, axis=-1, keepdims=True) * (1.0 / D)
                cid = (cid0 + k) % nchain
                if deps.get(cid) is not None:
                    m = m + deps[cid]
                xc = x1 - m
                v = jnp.sum(xc * xc, axis=-1, keepdims=True) * (1.0 / D)
                rstd = lax.rsqrt(v + 1e-5)
                xl = xc * rstd
                rs = jnp.sum(xl * wr, axis=1, keepdims=True)
                for q in range(STRIP // 8):
                    racc = jnp.where(lane_i == lane0 + (k * STRIP) // 8 + q,
                                     jnp.broadcast_to(rs[q * 8:(q + 1) * 8], (8, 128)), racc)
                xb[rows2, :] = _p32(xl)
                if first:
                    xw[rows, :] = x1 + xl
                    c2 = 1.0 + rstd
                    s2 = c2 * lax.rsqrt(v * c2 * c2 + 1e-5)
                    xn[rows2, :] = _p32(xc * s2)
                    deps[cid] = jnp.minimum(jnp.abs(s2), 0.0)
                else:
                    xo[rows, :] = (x1 + xl).astype(BF16)
                    deps[cid] = jnp.minimum(jnp.abs(rstd), 0.0)
            return racc

        nsub = L // SUB
        ninf = jnp.full((8, 128), -jnp.inf, F32)

        def oproj(i, c):
            r = pl.multiple_of(i * L, L)
            r2 = pl.multiple_of(i * (L // 2), L // 2)
            ip = jnp.where(i == 0, NSEG - 1, i - 1)
            rp = pl.multiple_of(ip * L + (nsub - 1) * SUB, SUB)
            rr_prev = pl.ds(pl.multiple_of(jnp.where(i == 0, NSEG, i - 1) * 8, 8), 8)
            deps = {}
            t_prev = o_dot(r2, 0)
            rr[rr_prev, :] = o_epilogue(tst[pl.ds(pl.multiple_of(i >> 10, 8), SUB), :], rp,
                                        ((nsub - 1) * SUB) // 8, rr[rr_prev, :], deps, 0)
            racc = ninf
            for j in range(1, nsub):
                t_cur = o_dot(r2, j)
                racc = o_epilogue(t_prev, r + (j - 1) * SUB, ((j - 1) * SUB) // 8, racc, deps,
                                  j * (SUB // STRIP))
                t_prev = t_cur
            tst[...] = t_prev
            rr[pl.ds(pl.multiple_of(i * 8, 8), 8), :] = racc

            if not first:
                @pl.when(i > 0)
                def _():
                    out_copy(i - 1).start()
            return c
        lax.fori_loop(0, NSEG, oproj, 0)
        rr_last = pl.ds((NSEG - 1) * 8, 8)
        rr[rr_last, :] = o_epilogue(tst[...], (NSEG - 1) * L + (nsub - 1) * SUB,
                                    ((nsub - 1) * SUB) // 8, rr[rr_last, :], {}, 0, nchain=4)
        if not first:
            out_copy(NSEG - 1).start()

        if first:
            w_copy(4).wait()
            w_copy(5).wait()
            for j in range(NG):
                wd_copy(j).wait()

        rv = rr[pl.ds(0, NSEG * 8), :]
        prow = lax.broadcasted_iota(jnp.int32, (NSEG * 8, 128), 0)
        plane = lax.broadcasted_iota(jnp.int32, (NSEG * 8, 128), 1)
        idx = (prow // 8) * L + plane * 8 + prow % 8

        def top1(vals):
            mx = jnp.max(jnp.max(vals, axis=0, keepdims=True), axis=1, keepdims=True)
            cand = jnp.where(vals == mx, idx, S - 1)
            ix = jnp.min(jnp.min(cand, axis=0, keepdims=True), axis=1, keepdims=True)
            return mx, ix

        m1, i1v = top1(rv)
        m2, i2v = top1(jnp.where(idx == i1v, -jnp.inf, rv))
        i1 = jnp.clip(i1v[0, 0], 0, S - 1)
        i2 = jnp.clip(i2v[0, 0], 0, S - 1)
        g1 = pl.multiple_of((i1 // 16) * 16, 16)
        g2 = pl.multiple_of((i2 // 16) * 16, 16)
        xs = jnp.concatenate([_b16(xb[pl.ds(pl.multiple_of(g1 // 2, 8), 8), :]),
                              _b16(xb[pl.ds(pl.multiple_of(g2 // 2, 8), 8), :])], axis=0)
        gg = _nn(xs, wg[...])
        uu = _nn(xs, wu[...])
        hh = (gg * (1.0 / (1.0 + jnp.exp(-gg))) * uu).astype(BF16)
        yy = jnp.concatenate([_nn(hh, wd[j]) for j in range(NG)], axis=1)
        riota = lax.broadcasted_iota(jnp.int32, (16, D), 0)
        if not first:
            for i in range(NSEG):
                out_copy(i).wait()
        for j, (ii, mm, gr) in enumerate(((i1, m1, g1), (i2, m2, g2))):
            sig = 1.0 / (1.0 + jnp.exp(-mm))
            upd_ = yy[16 * j:16 * (j + 1)] * sig
            if first:
                x2 = xw[pl.ds(gr, 16), :]
                x2 = jnp.where(riota == ii - gr, x2 + upd_, x2)
                xw[pl.ds(gr, 16), :] = x2
                xn[pl.ds(pl.multiple_of(gr // 2, 8), 8), :] = _p32(_ln(x2))
            else:
                x2 = xo[pl.ds(gr, 16), :].astype(F32)
                xo[pl.ds(gr, 16), :] = jnp.where(riota == ii - gr, x2 + upd_, x2).astype(BF16)
                cp = pltpu.make_async_copy(xo.at[pl.ds(gr, 16), :], out_hbm.at[0, pl.ds(gr, 16), :], sem_o.at[0])
                cp.start()
                cp.wait()

    layer(True)
    layer(False)


@jax.jit
def pallas_interleave_layers__memory_aug_infini_attn__moe_arch_mod__prompt_kernel(
    A_x: jax.Array,
    A_wq: jax.Array,
    A_wk: jax.Array,
    A_wv: jax.Array,
    A_wo: jax.Array,
    A_beta: jax.Array,
    B_x: jax.Array,
    B_w_r: jax.Array,
    B_w_gate: jax.Array,
    B_w_up: jax.Array,
    B_w_down: jax.Array,
):
    del B_x
    any_spec = pl.BlockSpec(memory_space=pl.ANY)
    small = lambda shape: pl.BlockSpec(shape, lambda: (0,) * len(shape))
    vm = pltpu.VMEM
    scratch = [
        vm((S, D), BF16),
        vm((S, D), F32),
        vm((S // 2, D), U32),
        vm((3 * D, D), BF16),
        vm((D, D), BF16),
        vm((D // 2, D), U32),
        vm((D, 3 * D), BF16),
        vm((D, FF), BF16), vm((D, FF), BF16), vm((NG, FF, 128), BF16),
        vm((D // 2, S), U32), vm((D // 2, S), U32),
        vm((D // 2, S), U32), vm((D // 2, S), U32),
        vm((NG, S // 2, 128), U32), vm((NG, S // 2, 128), U32),
        vm((NG, S // 2, 128), U32),
        vm((S // 2, D), U32),
        vm((NG * NSEG * 8, 128), F32),
        vm((D, 128), F32),
        vm(((NSEG + 1) * 8, 128), F32),
        vm((SUB, D), F32),
        vm((8, D), F32),
        vm((L, QB), F32), vm((L, QB), F32),
    ] + [vm((4 * QB + 8, QB), F32) for _ in range(NSB)] + [
        pltpu.SemaphoreType.DMA((NSEG,)),
        pltpu.SemaphoreType.DMA((7,)),
        pltpu.SemaphoreType.DMA((NG,)),
        pltpu.SemaphoreType.DMA((NSEG,)),
    ]
    return pl.pallas_call(
        _kernel,
        out_shape=jax.ShapeDtypeStruct((1, S, D), BF16),
        in_specs=[any_spec, any_spec, any_spec, any_spec, any_spec,
                  small((H,)), small((D,)), any_spec, any_spec, any_spec],
        out_specs=any_spec,
        scratch_shapes=scratch,
        compiler_params=pltpu.CompilerParams(vmem_limit_bytes=110 * 1024 * 1024),
        name="infini_mod",
    )(A_x, A_wq, A_wk, A_wv, A_wo, A_beta, B_w_r, B_w_gate, B_w_up, B_w_down)
```

```python
import numpy as np
import jax
import jax.numpy as jnp
from jax import lax
import jax.experimental.pallas as pl
import jax.experimental.pallas.tpu as pltpu

F32 = jnp.float32
BF16 = jnp.bfloat16
U32 = jnp.uint32

S, D, H, NSEG, FF = 2048, 1024, 32, 4, 3584
DH = D // H
L = S // NSEG
NG = D // 128
HPG = 128 // DH
QB = 128
SUB = 64
O_PACE = {True: (16, 1), False: (16, 1)}
LN_CHAIN = 4


NSB = 16
LOG2E = float(np.log2(np.e))
SCALE = float(np.asarray(DH ** -0.5, dtype=np.float32).astype(jnp.bfloat16).astype(np.float32))
QSCALE = SCALE * LOG2E
MASKV = -1e9 * LOG2E


def _phi(t):
    return jnp.where(t > 0, t + 1.0, jnp.exp(t))


def _ln(x):
    m = jnp.sum(x, axis=-1, keepdims=True) * (1.0 / D)
    xc = x - m
    v = jnp.sum(xc * xc, axis=-1, keepdims=True) * (1.0 / D)
    return xc * lax.rsqrt(v + 1e-5)


def _nt(a, b):
    return lax.dot_general(a, b, (((1,), (1,)), ((), ())), preferred_element_type=F32)


def _nn(a, b):
    return jnp.dot(a, b, preferred_element_type=F32)


def _b16(x):
    return pltpu.bitcast(x, BF16)


def _p32(x):
    return pltpu.bitcast(x.astype(BF16), U32)


def _mul(i, n):
    return i if isinstance(i, int) else pl.multiple_of(i, n)


def _tree(op, xs):
    xs = list(xs)
    while len(xs) > 1:
        nx = [op(xs[i], xs[i + 1]) for i in range(0, len(xs) - 1, 2)]
        if len(xs) % 2:
            nx.append(xs[-1])
        xs = nx
    return xs[0]


def _vsplit(x):
    return [x[i * 8:(i + 1) * 8] for i in range(x.shape[0] // 8)]


class _Sub:
    def __init__(self, idx, s, qb, h):
        self.idx, self.s, self.qb, self.h = idx, s, qb, h
        self.n = qb + 1


ORDER, OFF, SLOPE, UPD_AT, ND_AT = (0, 1, 2, 3), 16, 0, 10, 30


def _attn_plan(order=ORDER, off=OFF):
    subs = []
    for s in range(NSEG):
        for qb in order:
            for h in range(HPG):
                subs.append(_Sub(len(subs), s, qb, h))
    tiles = [(u, kt) for u in subs for kt in range(u.n)]
    n = len(tiles)
    first = {}
    for i, (u, kt) in enumerate(tiles):
        if kt == 0:
            first[u.idx] = i
    pos = [first[u.idx] + u.n - 1 + off + int(SLOPE * kt) for (u, kt) in tiles]
    deferred = set((u.s, u.qb) for i, (u, kt) in enumerate(tiles) if pos[i] >= n)
    now, prev = {}, {}
    for i, (u, kt) in enumerate(tiles):
        if (u.s, u.qb) in deferred:
            prev.setdefault(max(pos[i] - n, 0), []).append(i)
        else:
            now.setdefault(pos[i], []).append(i)
    return tiles, now, prev


_PLAN = _attn_plan()


class _Refs:
    pass


def _attn_body(R, g, gp, zero, do_qk=True):
    tiles, now, prev = _PLAN
    krow = lax.broadcasted_iota(jnp.int32, (QB, QB), 0)
    qcol = lax.broadcasted_iota(jnp.int32, (QB, QB), 1)
    bd = (krow // DH) == (qcol // DH)
    laneh = lax.broadcasted_iota(jnp.int32, (8, QB), 1) // DH
    st, outs, mem = {}, {}, {}

    HB = QB // 2
    lo8 = lax.broadcasted_iota(jnp.int32, (8, QB), 1) < HB
    tri = jnp.where(krow[:HB] > qcol[:HB] % HB, MASKV, 0.0).astype(F32)
    swap = lambda v: pltpu.roll(v, HB, 1)

    def put(u, kt, x):
        buf = R.sb[u.idx % NSB]
        buf[pl.ds(kt * QB, QB), :] = x
        mx = _tree(jnp.maximum, _vsplit(x))
        key = ("m", u.idx)
        st[key] = jnp.maximum(st[key], mx) if key in st else mx
        if kt == (u.qb if (u.h % 2 == 0 or u.qb == 0) else u.qb - 1):
            buf[pl.ds(4 * QB, 8), :] = jnp.broadcast_to(jnp.max(st[key], axis=0, keepdims=True), (8, QB))

    def qk(i):
        u, kt = tiles[i]
        t0 = u.s * L
        q0 = t0 + u.qb * QB
        qrow = lambda ref, h: ref[pl.ds(pl.multiple_of(g * 64 + h * 16, 16), 16), pl.ds(q0, QB)]
        k0 = (t0 + kt * QB) // 2
        if kt < u.qb:
            parts = []
            if u.h > 0:
                parts.append(jnp.zeros((u.h * 16, QB), U32))
            parts.append(qrow(R.qT, u.h))
            if u.h < HPG - 1:
                parts.append(jnp.zeros(((HPG - 1 - u.h) * 16, QB), U32))
            put(u, kt, _nn(_b16(R.kk[g, pl.ds(k0, QB // 2), :]), _b16(jnp.concatenate(parts, axis=0))))
            return
        if u.h % 2 == 1:
            return
        lane16 = lax.broadcasted_iota(jnp.int32, (16, QB), 1) < HB
        z = jnp.uint32(0)

        def packed(rows, wa, wb):
            parts = []
            if u.h > 0:
                parts.append(jnp.zeros((u.h * 16, QB), U32))
            parts += [jnp.where(lane16, wa, z), jnp.where(lane16, z, wb)]
            if u.h < HPG - 2:
                parts.append(jnp.zeros(((HPG - 2 - u.h) * 16, QB), U32))
            return _nn(_b16(R.kk[g, pl.ds(k0, rows // 2), :]), _b16(jnp.concatenate(parts, axis=0)))

        X = packed(QB, qrow(R.qS, u.h), qrow(R.qT, u.h + 1))
        Y = packed(HB, qrow(R.qT, u.h), qrow(R.qS, u.h + 1)) + tri
        X0, X1 = _vsplit(X[:HB]), _vsplit(X[HB:] + tri)
        Y = _vsplit(Y)
        put(u, kt, jnp.concatenate([jnp.where(lo8, y, swap(x)) for x, y in zip(X0, Y)]
                                   + [jnp.where(lo8, MASKV, swap(x)) for x in X1], axis=0))
        put(tiles[i + 1 + u.qb][0], kt,
            jnp.concatenate([jnp.where(lo8, swap(y), x) for x, y in zip(X0, Y)]
                            + [jnp.where(lo8, MASKV, x) for x in X1], axis=0))

    def pv(i, gg, tag):
        u, kt = tiles[i]
        t0 = u.s * L
        q0 = t0 + u.qb * QB
        buf = R.sb[u.idx % NSB]
        km, kl, ko = ("mf", u.idx, tag), ("l", u.idx, tag), ("o", u.idx, tag)
        if kt == 0:
            st[km] = buf[pl.ds(pl.multiple_of(4 * QB + zero, 8), 8), :]
        m = st[km]
        x = buf[pl.ds(pl.multiple_of(kt * QB + zero, 8), QB), :]
        p = jnp.concatenate([jnp.exp2(v - m) for v in _vsplit(x)], axis=0)
        ls = _tree(jnp.add, _vsplit(p))
        st[kl] = ls if kt == 0 else st[kl] + ls
        vt = _b16(R.vT[pl.ds(pl.multiple_of(gg * 64 + u.h * 16, 16), 16), pl.ds(t0 + kt * QB, QB)])
        ot = _nn(vt, p.astype(BF16))
        st[ko] = ot if kt == 0 else st[ko] + ot
        if kt == u.qb:
            l = jnp.sum(st[kl], axis=0, keepdims=True)
            adot = st[ko] * (1.0 / l)
            gt = R.gs[pl.ds(pl.multiple_of(gg * 128 + u.h * DH, 8), 8), :]
            gt = jnp.concatenate([1.0 - gt] * 4, axis=0)
            o = gt * adot
            if u.s > 0:
                o = R.am[u.s % 2][pl.ds(pl.multiple_of(u.qb * QB + u.h * DH + zero, 8), DH), :] + o
            lst = outs.setdefault((u.s, u.qb, tag), [])
            lst.append(o)
            if len(lst) == HPG:
                oT = jnp.concatenate(lst, axis=0)
                R.ob[gg, pl.ds(q0 // 2, QB // 2), :] = _p32(oT.T)

    def upd(s):
        t0 = s * L
        lhs = _b16(R.vT[pl.ds(pl.multiple_of(g * 64, 64), 64), pl.ds(t0, L)])
        rhs = _b16(R.pk[g, pl.ds(t0 // 2, L // 2), :])
        u_ = jnp.where(bd, _nn(lhs, rhs), 0.0)
        zr = R.zs[pl.ds(pl.multiple_of(g * 8 * NSEG + s * 8, 8), 8), :]
        if s == 0:
            mem["M"], mem["z"] = u_, zr
        else:
            mem["M"], mem["z"] = mem["M"] + u_, mem["z"] + zr

    def nd(s):
        t0 = s * L
        zl = [jnp.where(laneh == h, mem["z"], 0.0) for h in range(HPG)]
        lhs = jnp.concatenate([mem["M"]] + zl, axis=0).astype(BF16)
        for qb in range(L // QB):
            r = _nn(lhs, _b16(R.pqT[pl.ds(pl.multiple_of(g * 64, 64), 64), pl.ds(t0 + qb * QB, QB)]))
            for h in range(HPG):
                den = r[128 + 8 * h:128 + 8 * h + 8] + 1e-6
                gt = R.gs[pl.ds(pl.multiple_of(g * 128 + h * DH, 8), 8), :] * (1.0 / den)
                R.am[s % 2][pl.ds(qb * QB + h * DH, DH), :] = (
                    r[h * DH:(h + 1) * DH] * jnp.concatenate([gt] * 4, axis=0))

    extra = {}
    if do_qk:
        for s in range(NSEG - 1):
            extra.setdefault(40 * s + UPD_AT, []).append(("upd", s))
            extra.setdefault(40 * s + ND_AT, []).append(("nd", s + 1))
    for i in range(len(tiles)):
        if do_qk:
            qk(i)
        for kind, s in extra.get(i, []):
            (upd if kind == "upd" else nd)(s)
        for j in prev.get(i, []):
            pv(j, gp, 0)
        if do_qk:
            for j in now.get(i, []):
                pv(j, g, 1)


def _kernel(x_hbm, wq_hbm, wk_hbm, wv_hbm, wo_hbm, beta_ref, wr_ref, wg_hbm, wu_hbm, wd_hbm,
            out_hbm,
            xin, xw, xn, wall, wo, wo32, wT, wg, wu, wd,
            qT, qS, pqT, vT, kk, pk, ob, xb, zs, gs, rr, tst, wrf, am0, am1, *rest):
    sb = rest[:NSB]
    sem_x, sem_w, sem_d, sem_o = rest[NSB:]
    R = _Refs()
    R.qS = qS
    R.qT, R.pqT, R.vT, R.kk, R.pk, R.ob, R.zs, R.gs = qT, pqT, vT, kk, pk, ob, zs, gs
    R.am, R.sb = (am0, am1), sb
    xo = xin

    def x_copy(i):
        return pltpu.make_async_copy(x_hbm.at[0, pl.ds(i * L, L), :], xin.at[pl.ds(i * L, L), :], sem_x.at[i])

    def w_copy(j):
        half = lambda ref, c: ref.at[pl.ds(0, D), pl.ds(c * (D // 2), D // 2)]
        src = (half(wk_hbm, 0), wq_hbm, wv_hbm, wo_hbm, wg_hbm, wu_hbm, half(wk_hbm, 1))[j]
        dst = (half(wall, 0), wall.at[pl.ds(D, D), :], wall.at[pl.ds(2 * D, D), :], wo, wg, wu, half(wall, 1))[j]
        return pltpu.make_async_copy(src, dst, sem_w.at[j])

    def wd_copy(j):
        return pltpu.make_async_copy(wd_hbm.at[:, pl.ds(j * 128, 128)], wd.at[j], sem_d.at[j])

    def out_copy(i):
        return pltpu.make_async_copy(xo.at[pl.ds(i * L, L), :], out_hbm.at[0, pl.ds(i * L, L), :], sem_o.at[i])

    x_copy(0).start()
    w_copy(0).start()

    b = beta_ref[...].astype(F32).reshape(1, H)
    wrf[...] = jnp.broadcast_to(wr_ref[...].astype(F32).reshape(1, D), (8, D))
    sg = 1.0 / (1.0 + jnp.exp(-b))
    lane = lax.broadcasted_iota(jnp.int32, (1, H), 1)
    for h in range(H):
        gh = jnp.sum(jnp.where(lane == h, sg, 0.0), axis=1, keepdims=True)
        gs[pl.ds(h * DH, DH), :] = jnp.broadcast_to(gh, (DH, 128))
    for buf in sb:
        buf[...] = jnp.zeros(buf.shape, F32)
    am0[...] = jnp.zeros(am0.shape, F32)
    am1[...] = jnp.zeros(am1.shape, F32)
    tst[...] = jnp.zeros(tst.shape, F32)
    rr[...] = jnp.zeros(rr.shape, F32)

    def ln_first(blk, nchain=0):
        deps = {}
        for k in range(L // 16):
            xv = xin[pl.ds(blk * L + k * 16, 16), :].astype(F32)
            m = jnp.sum(xv, axis=-1, keepdims=True) * (1.0 / D)
            if nchain and k >= nchain:
                m = m + deps[k % nchain]
            xc = xv - m
            rstd = lax.rsqrt(jnp.sum(xc * xc, axis=-1, keepdims=True) * (1.0 / D) + 1e-5)
            xn[pl.ds(blk * (L // 2) + k * 8, 8), :] = _p32(xc * rstd)
            if nchain:
                deps[k % nchain] = jnp.minimum(jnp.abs(rstd), 0.0)

    order = ([("w", 6), ("x", 1), ("x", 2), ("x", 3)] + [("w", j) for j in range(1, 6)]
             + [("d", j) for j in range(NG)])

    def issue(i, c):
        for j, (kind, n) in enumerate(order):
            @pl.when(i == j)
            def _():
                {"x": x_copy, "w": w_copy, "d": wd_copy}[kind](n).start()
        return c
    lax.fori_loop(0, len(order), issue, 0)

    x_copy(0).wait()
    ln_first(0)

    def layer(first):

        def kproj_main(s, g0=0, g1=NG):
            r2 = _mul(s * (L // 2), L // 2)
            kf = _nn(_b16(xn[pl.ds(r2, L // 2), :]), wall[pl.ds(0, D), pl.ds(g0 * 128, (g1 - g0) * 128)])
            pf = _phi(kf)
            zrow = jnp.sum(pf, axis=0, keepdims=True)
            for g in range(g0, g1):
                sl = slice((g - g0) * 128, (g - g0 + 1) * 128)
                kk[g, pl.ds(r2, L // 2), :] = _p32(kf[:, sl])
                pk[g, pl.ds(r2, L // 2), :] = _p32(pf[:, sl])
                zs[pl.ds(_mul(g * 8 * NSEG + s * 8, 8), 8), :] = jnp.broadcast_to(zrow[:, sl], (8, 128))

        def transpose_w(j):
            for c_ in range(D // 128):
                rw = j * D + c_ * 128
                wT[:, pl.ds(rw, 128)] = wall[pl.ds(rw, 128), :].T

        def kproj_first(step, c):
            @pl.when(step == 0)
            def _():
                w_copy(0).wait()
                kproj_main(0, 0, NG // 2)

            @pl.when(step == 1)
            def _():
                w_copy(6).wait()
                kproj_main(0, NG // 2, NG)

            @pl.when(step == 2)
            def _():
                x_copy(1).wait()
                ln_first(1)

            @pl.when(step == 3)
            def _():
                x_copy(2).wait()
                ln_first(2, LN_CHAIN)
                kproj_main(1)

            @pl.when(step == 4)
            def _():
                x_copy(3).wait()
                w_copy(1).wait()
                ln_first(3, LN_CHAIN)
                kproj_main(2)
                transpose_w(1)

            @pl.when(step == 5)
            def _():
                w_copy(2).wait()
                kproj_main(3)
                transpose_w(2)
            return c

        def kproj(s, c):
            kproj_main(s)
            return c

        if first:
            lax.fori_loop(0, 6, kproj_first, 0)
        else:
            lax.fori_loop(0, NSEG, kproj, 0)

        if first:
            w_copy(3).wait()

        def qvproj(s, c):
            r = pl.multiple_of(s * L, L)
            r2 = pl.multiple_of(s * (L // 2), L // 2)
            if first:
                wo32[pl.ds(pl.multiple_of(s * (D // 8), D // 8), D // 8), :] = pltpu.bitcast(
                    wo[pl.ds(pl.multiple_of(s * (D // 4), D // 4), D // 4), :], U32)
            xb_ = _b16(xn[pl.ds(r2, L // 2), :])
            qf = _nt(wT[:, pl.ds(D, D)], xb_)
            q16 = _p32(qf * QSCALE)
            qT[:, pl.ds(r, L)] = q16
            for c_ in range(L // QB):
                qS[:, pl.ds(r + c_ * QB, QB)] = pltpu.roll(q16[:, c_ * QB:(c_ + 1) * QB], QB // 2, 1)
            pqT[:, pl.ds(r, L)] = _p32(_phi(qf))
            vf = _nt(wT[:, pl.ds(2 * D, D)], xb_)
            vT[:, pl.ds(r, L)] = _p32(vf)
            return c
        lax.fori_loop(0, NSEG, qvproj, 0)

        def attn(g, c):
            _attn_body(R, g, jnp.maximum(g - 1, 0), g >> 10)
            return c
        lax.fori_loop(0, NG, attn, 0)
        _attn_body(R, NG - 1, NG - 1, 0, do_qk=False)

        def o_dot(r2, j):
            lhs = jnp.concatenate(
                [_b16(ob[g, pl.ds(r2 + j * SUB // 2, SUB // 2), :]) for g in range(NG)], axis=1)
            return _nn(lhs, _b16(wo32[...]))

        STRIP, NCHAIN = O_PACE[first]

        def o_epilogue(t, r0, lane0, racc, deps, cid0, nchain=NCHAIN):
            wr = wrf[pl.ds(0, 1), :]
            lane_i = lax.broadcasted_iota(jnp.int32, (8, 128), 1)
            for k in range(SUB // STRIP):
                rows = pl.ds(r0 + k * STRIP, STRIP)
                rows2 = pl.ds(_mul(r0 // 2 + k * (STRIP // 2), STRIP // 2), STRIP // 2)
                xres = xin[rows, :].astype(F32) if first else xw[rows, :]
                x1 = xres + t[k * STRIP:(k + 1) * STRIP]
                m = jnp.sum(x1, axis=-1, keepdims=True) * (1.0 / D)
                cid = (cid0 + k) % nchain
                if deps.get(cid) is not None:
                    m = m + deps[cid]
                xc = x1 - m
                v = jnp.sum(xc * xc, axis=-1, keepdims=True) * (1.0 / D)
                rstd = lax.rsqrt(v + 1e-5)
                xl = xc * rstd
                rs = jnp.sum(xl * wr, axis=1, keepdims=True)
                for q in range(STRIP // 8):
                    racc = jnp.where(lane_i == lane0 + (k * STRIP) // 8 + q,
                                     jnp.broadcast_to(rs[q * 8:(q + 1) * 8], (8, 128)), racc)
                xb[rows2, :] = _p32(xl)
                if first:
                    xw[rows, :] = x1 + xl
                    c2 = 1.0 + rstd
                    s2 = c2 * lax.rsqrt(v * c2 * c2 + 1e-5)
                    xn[rows2, :] = _p32(xc * s2)
                    deps[cid] = jnp.minimum(jnp.abs(s2), 0.0)
                else:
                    xo[rows, :] = (x1 + xl).astype(BF16)
                    deps[cid] = jnp.minimum(jnp.abs(rstd), 0.0)
            return racc

        nsub = L // SUB
        ninf = jnp.full((8, 128), -jnp.inf, F32)

        def oproj(i, c):
            r = pl.multiple_of(i * L, L)
            r2 = pl.multiple_of(i * (L // 2), L // 2)
            ip = jnp.where(i == 0, NSEG - 1, i - 1)
            rp = pl.multiple_of(ip * L + (nsub - 1) * SUB, SUB)
            rr_prev = pl.ds(pl.multiple_of(jnp.where(i == 0, NSEG, i - 1) * 8, 8), 8)
            deps = {}
            t_prev = o_dot(r2, 0)
            rr[rr_prev, :] = o_epilogue(tst[pl.ds(pl.multiple_of(i >> 10, 8), SUB), :], rp,
                                        ((nsub - 1) * SUB) // 8, rr[rr_prev, :], deps, 0)
            racc = ninf
            for j in range(1, nsub):
                t_cur = o_dot(r2, j)
                racc = o_epilogue(t_prev, r + (j - 1) * SUB, ((j - 1) * SUB) // 8, racc, deps,
                                  j * (SUB // STRIP))
                t_prev = t_cur
            tst[...] = t_prev
            rr[pl.ds(pl.multiple_of(i * 8, 8), 8), :] = racc

            if not first:
                @pl.when(i > 0)
                def _():
                    out_copy(i - 1).start()
            return c
        lax.fori_loop(0, NSEG, oproj, 0)
        rr_last = pl.ds((NSEG - 1) * 8, 8)
        rr[rr_last, :] = o_epilogue(tst[...], (NSEG - 1) * L + (nsub - 1) * SUB,
                                    ((nsub - 1) * SUB) // 8, rr[rr_last, :], {}, 0, nchain=4)
        if not first:
            out_copy(NSEG - 1).start()

        if first:
            w_copy(4).wait()
            w_copy(5).wait()
            for j in range(NG):
                wd_copy(j).wait()

        rv = rr[pl.ds(0, NSEG * 8), :]
        prow = lax.broadcasted_iota(jnp.int32, (NSEG * 8, 128), 0)
        plane = lax.broadcasted_iota(jnp.int32, (NSEG * 8, 128), 1)
        idx = (prow // 8) * L + plane * 8 + prow % 8

        bits = pltpu.bitcast(rv, jnp.int32)
        key = jnp.where(bits < 0, bits ^ 0x7FFFFFFF, bits)
        key = (key & ~(S - 1)) | ((S - 1 - idx) & (S - 1))
        max_all = lambda v: jnp.max(jnp.max(v, axis=0, keepdims=True), axis=1, keepdims=True)
        k1 = max_all(key)
        k2 = max_all(jnp.where(key == k1, jnp.iinfo(jnp.int32).min, key))
        i1 = S - 1 - (k1[0, 0] & (S - 1))
        i2 = S - 1 - (k2[0, 0] & (S - 1))
        g1 = pl.multiple_of((i1 // 16) * 16, 16)
        g2 = pl.multiple_of((i2 // 16) * 16, 16)
        xs = jnp.concatenate([_b16(xb[pl.ds(pl.multiple_of(g1 // 2, 8), 8), :]),
                              _b16(xb[pl.ds(pl.multiple_of(g2 // 2, 8), 8), :])], axis=0)
        gg = _nn(xs, wg[...])
        uu = _nn(xs, wu[...])
        hh = (gg * (1.0 / (1.0 + jnp.exp(-gg))) * uu).astype(BF16)
        yy = jnp.concatenate([_nn(hh, wd[j]) for j in range(NG)], axis=1)
        rsel = jnp.sum(xs.astype(F32) * wrf[pl.ds(0, 1), :], axis=1, keepdims=True)
        yy = yy * (1.0 / (1.0 + jnp.exp(-rsel)))
        riota = lax.broadcasted_iota(jnp.int32, (16, D), 0)
        if not first:
            for i in range(NSEG):
                out_copy(i).wait()
        for j, (ii, gr) in enumerate(((i1, g1), (i2, g2))):
            upd_ = yy[16 * j:16 * (j + 1)]
            if first:
                x2 = xw[pl.ds(gr, 16), :]
                x2 = jnp.where(riota == ii - gr, x2 + upd_, x2)
                xw[pl.ds(gr, 16), :] = x2
                xn[pl.ds(pl.multiple_of(gr // 2, 8), 8), :] = _p32(_ln(x2))
            else:
                x2 = xo[pl.ds(gr, 16), :].astype(F32)
                xo[pl.ds(gr, 16), :] = jnp.where(riota == ii - gr, x2 + upd_, x2).astype(BF16)
        if not first:
            patch = lambda gr, j: pltpu.make_async_copy(
                xo.at[pl.ds(gr, 16), :], out_hbm.at[0, pl.ds(gr, 16), :], sem_o.at[j])
            patch(g1, 0).start()

            @pl.when(g2 != g1)
            def _():
                patch(g2, 1).start()
            patch(g1, 0).wait()

            @pl.when(g2 != g1)
            def _():
                patch(g2, 1).wait()

    layer(True)
    layer(False)


@jax.jit
def pallas_interleave_layers__memory_aug_infini_attn__moe_arch_mod__prompt_kernel(
    A_x: jax.Array,
    A_wq: jax.Array,
    A_wk: jax.Array,
    A_wv: jax.Array,
    A_wo: jax.Array,
    A_beta: jax.Array,
    B_x: jax.Array,
    B_w_r: jax.Array,
    B_w_gate: jax.Array,
    B_w_up: jax.Array,
    B_w_down: jax.Array,
):
    del B_x
    any_spec = pl.BlockSpec(memory_space=pl.ANY)
    small = lambda shape: pl.BlockSpec(shape, lambda: (0,) * len(shape))
    vm = pltpu.VMEM
    scratch = [
        vm((S, D), BF16),
        vm((S, D), F32),
        vm((S // 2, D), U32),
        vm((3 * D, D), BF16),
        vm((D, D), BF16),
        vm((D // 2, D), U32),
        vm((D, 3 * D), BF16),
        vm((D, FF), BF16), vm((D, FF), BF16), vm((NG, FF, 128), BF16),
        vm((D // 2, S), U32), vm((D // 2, S), U32),
        vm((D // 2, S), U32), vm((D // 2, S), U32),
        vm((NG, S // 2, 128), U32), vm((NG, S // 2, 128), U32),
        vm((NG, S // 2, 128), U32),
        vm((S // 2, D), U32),
        vm((NG * NSEG * 8, 128), F32),
        vm((D, 128), F32),
        vm(((NSEG + 1) * 8, 128), F32),
        vm((SUB, D), F32),
        vm((8, D), F32),
        vm((L, QB), F32), vm((L, QB), F32),
    ] + [vm((4 * QB + 8, QB), F32) for _ in range(NSB)] + [
        pltpu.SemaphoreType.DMA((NSEG,)),
        pltpu.SemaphoreType.DMA((7,)),
        pltpu.SemaphoreType.DMA((NG,)),
        pltpu.SemaphoreType.DMA((NSEG,)),
    ]
    return pl.pallas_call(
        _kernel,
        out_shape=jax.ShapeDtypeStruct((1, S, D), BF16),
        in_specs=[any_spec, any_spec, any_spec, any_spec, any_spec,
                  small((H,)), small((D,)), any_spec, any_spec, any_spec],
        out_specs=any_spec,
        scratch_shapes=scratch,
        compiler_params=pltpu.CompilerParams(vmem_limit_bytes=110 * 1024 * 1024),
        name="infini_mod",
    )(A_x, A_wq, A_wk, A_wv, A_wo, A_beta, B_w_r, B_w_gate, B_w_up, B_w_down)
```

```python
import numpy as np
import jax
import jax.numpy as jnp
from jax import lax
import jax.experimental.pallas as pl
import jax.experimental.pallas.tpu as pltpu

F32 = jnp.float32
BF16 = jnp.bfloat16
U32 = jnp.uint32

S, D, H, NSEG, FF = 2048, 1024, 32, 4, 3584
DH = D // H
L = S // NSEG
NG = D // 128
HPG = 128 // DH
QB = 128
SUB = 64
O_PACE = {True: (16, 1), False: (16, 1)}
LN_CHAIN = 4


NSB = 16
LOG2E = float(np.log2(np.e))
SCALE = float(np.asarray(DH ** -0.5, dtype=np.float32).astype(jnp.bfloat16).astype(np.float32))
QSCALE = SCALE * LOG2E
MASKV = -1e9 * LOG2E


def _phi(t):
    return jnp.where(t > 0, t + 1.0, jnp.exp(t))


def _ln(x):
    m = jnp.sum(x, axis=-1, keepdims=True) * (1.0 / D)
    xc = x - m
    v = jnp.sum(xc * xc, axis=-1, keepdims=True) * (1.0 / D)
    return xc * lax.rsqrt(v + 1e-5)


def _nt(a, b):
    return lax.dot_general(a, b, (((1,), (1,)), ((), ())), preferred_element_type=F32)


def _nn(a, b):
    return jnp.dot(a, b, preferred_element_type=F32)


def _b16(x):
    return pltpu.bitcast(x, BF16)


def _p32(x):
    return pltpu.bitcast(x.astype(BF16), U32)


def _mul(i, n):
    return i if isinstance(i, int) else pl.multiple_of(i, n)


def _tree(op, xs):
    xs = list(xs)
    while len(xs) > 1:
        nx = [op(xs[i], xs[i + 1]) for i in range(0, len(xs) - 1, 2)]
        if len(xs) % 2:
            nx.append(xs[-1])
        xs = nx
    return xs[0]


def _vsplit(x):
    return [x[i * 8:(i + 1) * 8] for i in range(x.shape[0] // 8)]


class _Sub:
    def __init__(self, idx, s, qb, h):
        self.idx, self.s, self.qb, self.h = idx, s, qb, h
        self.n = qb + 1


ORDER, OFF, SLOPE, UPD_AT, ND_AT = (0, 1, 2, 3), 16, 0, 10, 30


def _attn_plan(order=ORDER, off=OFF):
    subs = []
    for s in range(NSEG):
        for qb in order:
            for h in range(HPG):
                subs.append(_Sub(len(subs), s, qb, h))
    tiles = [(u, kt) for u in subs for kt in range(u.n)]
    n = len(tiles)
    first = {}
    for i, (u, kt) in enumerate(tiles):
        if kt == 0:
            first[u.idx] = i
    pos = [first[u.idx] + u.n - 1 + off + int(SLOPE * kt) for (u, kt) in tiles]
    deferred = set((u.s, u.qb) for i, (u, kt) in enumerate(tiles) if pos[i] >= n)
    now, prev = {}, {}
    for i, (u, kt) in enumerate(tiles):
        if (u.s, u.qb) in deferred:
            prev.setdefault(max(pos[i] - n, 0), []).append(i)
        else:
            now.setdefault(pos[i], []).append(i)
    return tiles, now, prev


_PLAN = _attn_plan()


class _Refs:
    pass


def _attn_body(R, g, gp, zero, do_qk=True):
    tiles, now, prev = _PLAN
    krow = lax.broadcasted_iota(jnp.int32, (QB, QB), 0)
    qcol = lax.broadcasted_iota(jnp.int32, (QB, QB), 1)
    bd = (krow // DH) == (qcol // DH)
    laneh = lax.broadcasted_iota(jnp.int32, (8, QB), 1) // DH
    st, outs, mem = {}, {}, {}

    HB = QB // 2
    lo8 = lax.broadcasted_iota(jnp.int32, (8, QB), 1) < HB
    tri = jnp.where(krow[:HB] > qcol[:HB] % HB, MASKV, 0.0).astype(F32)
    swap = lambda v: pltpu.roll(v, HB, 1)

    def put(u, kt, x):
        buf = R.sb[u.idx % NSB]
        buf[pl.ds(kt * QB, QB), :] = x
        mx = _tree(jnp.maximum, _vsplit(x))
        key = ("m", u.idx)
        st[key] = jnp.maximum(st[key], mx) if key in st else mx
        if kt == (u.qb if (u.h % 2 == 0 or u.qb == 0) else u.qb - 1):
            buf[pl.ds(4 * QB, 8), :] = jnp.broadcast_to(jnp.max(st[key], axis=0, keepdims=True), (8, QB))

    def qk(i):
        u, kt = tiles[i]
        t0 = u.s * L
        q0 = t0 + u.qb * QB
        qrow = lambda ref, h: ref[pl.ds(pl.multiple_of(g * 64 + h * 16, 16), 16), pl.ds(q0, QB)]
        k0 = (t0 + kt * QB) // 2
        if kt < u.qb:
            parts = []
            if u.h > 0:
                parts.append(jnp.zeros((u.h * 16, QB), U32))
            parts.append(qrow(R.qT, u.h))
            if u.h < HPG - 1:
                parts.append(jnp.zeros(((HPG - 1 - u.h) * 16, QB), U32))
            put(u, kt, _nn(_b16(R.kk[g, pl.ds(k0, QB // 2), :]), _b16(jnp.concatenate(parts, axis=0))))
            return
        if u.h % 2 == 1:
            return
        lane16 = lax.broadcasted_iota(jnp.int32, (16, QB), 1) < HB
        z = jnp.uint32(0)

        def packed(rows, wa, wb):
            parts = []
            if u.h > 0:
                parts.append(jnp.zeros((u.h * 16, QB), U32))
            parts += [jnp.where(lane16, wa, z), jnp.where(lane16, z, wb)]
            if u.h < HPG - 2:
                parts.append(jnp.zeros(((HPG - 2 - u.h) * 16, QB), U32))
            return _nn(_b16(R.kk[g, pl.ds(k0, rows // 2), :]), _b16(jnp.concatenate(parts, axis=0)))

        X = packed(QB, qrow(R.qS, u.h), qrow(R.qT, u.h + 1))
        Y = packed(HB, qrow(R.qT, u.h), qrow(R.qS, u.h + 1)) + tri
        X0, X1 = _vsplit(X[:HB]), _vsplit(X[HB:] + tri)
        Y = _vsplit(Y)
        put(u, kt, jnp.concatenate([jnp.where(lo8, y, swap(x)) for x, y in zip(X0, Y)]
                                   + [jnp.where(lo8, MASKV, swap(x)) for x in X1], axis=0))
        put(tiles[i + 1 + u.qb][0], kt,
            jnp.concatenate([jnp.where(lo8, swap(y), x) for x, y in zip(X0, Y)]
                            + [jnp.where(lo8, MASKV, x) for x in X1], axis=0))

    def pv(i, gg, tag):
        u, kt = tiles[i]
        t0 = u.s * L
        q0 = t0 + u.qb * QB
        buf = R.sb[u.idx % NSB]
        km, kl, ko = ("mf", u.idx, tag), ("l", u.idx, tag), ("o", u.idx, tag)
        if kt == 0:
            st[km] = buf[pl.ds(pl.multiple_of(4 * QB + zero, 8), 8), :]
        m = st[km]
        x = buf[pl.ds(pl.multiple_of(kt * QB + zero, 8), QB), :]
        p = jnp.concatenate([jnp.exp2(v - m) for v in _vsplit(x)], axis=0)
        ls = _tree(jnp.add, _vsplit(p))
        st[kl] = ls if kt == 0 else st[kl] + ls
        vt = _b16(R.vT[pl.ds(pl.multiple_of(gg * 64 + u.h * 16, 16), 16), pl.ds(t0 + kt * QB, QB)])
        ot = _nn(vt, p.astype(BF16))
        st[ko] = ot if kt == 0 else st[ko] + ot
        if kt == u.qb:
            l = jnp.sum(st[kl], axis=0, keepdims=True)
            adot = st[ko] * (1.0 / l)
            gt = R.gs[pl.ds(pl.multiple_of(gg * 128 + u.h * DH, 8), 8), :]
            gt = jnp.concatenate([1.0 - gt] * 4, axis=0)
            o = gt * adot
            if u.s > 0:
                o = R.am[u.s % 2][pl.ds(pl.multiple_of(u.qb * QB + u.h * DH + zero, 8), DH), :] + o
            lst = outs.setdefault((u.s, u.qb, tag), [])
            lst.append(o)
            if len(lst) == HPG:
                oT = jnp.concatenate(lst, axis=0)
                R.ob[gg, pl.ds(q0 // 2, QB // 2), :] = _p32(oT.T)

    def mem_load():
        return (R.macc[pl.ds(pl.multiple_of(zero, 8), QB), :], R.macc[pl.ds(pl.multiple_of(QB + zero, 8), 8), :])

    def upd(s):
        t0 = s * L
        lhs = _b16(R.vT[pl.ds(pl.multiple_of(g * 64, 64), 64), pl.ds(t0, L)])
        rhs = _b16(R.pk[g, pl.ds(t0 // 2, L // 2), :])
        u_ = jnp.where(bd, _nn(lhs, rhs), 0.0)
        zr = R.zs[pl.ds(pl.multiple_of(g * 8 * NSEG + s * 8, 8), 8), :]
        if s > 0:
            M, z = mem_load()
            u_, zr = M + u_, z + zr
        R.macc[pl.ds(0, QB), :] = u_
        R.macc[pl.ds(QB, 8), :] = zr

    def nd(s):
        t0 = s * L
        M, z = mem_load()
        zl = [jnp.where(laneh == h, z, 0.0) for h in range(HPG)]
        lhs = jnp.concatenate([M] + zl, axis=0).astype(BF16)
        for qb in range(L // QB):
            r = _nn(lhs, _b16(R.pqT[pl.ds(pl.multiple_of(g * 64, 64), 64), pl.ds(t0 + qb * QB, QB)]))
            for h in range(HPG):
                den = r[128 + 8 * h:128 + 8 * h + 8] + 1e-6
                gt = R.gs[pl.ds(pl.multiple_of(g * 128 + h * DH, 8), 8), :] * (1.0 / den)
                R.am[s % 2][pl.ds(qb * QB + h * DH, DH), :] = (
                    r[h * DH:(h + 1) * DH] * jnp.concatenate([gt] * 4, axis=0))

    extra = {}
    if do_qk:
        for s in range(NSEG - 1):
            extra.setdefault(40 * s + UPD_AT, []).append(("upd", s))
            extra.setdefault(40 * s + ND_AT, []).append(("nd", s + 1))
    for i in range(len(tiles)):
        if do_qk:
            qk(i)
        for kind, s in extra.get(i, []):
            (upd if kind == "upd" else nd)(s)
        for j in prev.get(i, []):
            pv(j, gp, 0)
        if do_qk:
            for j in now.get(i, []):
                pv(j, g, 1)


def _kernel(x_hbm, wq_hbm, wk_hbm, wv_hbm, wo_hbm, beta_ref, wr_ref, wg_hbm, wu_hbm, wd_hbm,
            out_hbm,
            xin, xw, xn, wall, wo, wo32, wT, wg, wu, wd,
            qT, qS, pqT, vT, kk, pk, ob, xb, zs, gs, rr, tst, wrf, am0, am1, macc, *rest):
    sb = rest[:NSB]
    sem_x, sem_w, sem_d, sem_o = rest[NSB:]
    R = _Refs()
    R.qS = qS
    R.qT, R.pqT, R.vT, R.kk, R.pk, R.ob, R.zs, R.gs = qT, pqT, vT, kk, pk, ob, zs, gs
    R.am, R.sb, R.macc = (am0, am1), sb, macc
    xo = xin

    def x_copy(i):
        return pltpu.make_async_copy(x_hbm.at[0, pl.ds(i * L, L), :], xin.at[pl.ds(i * L, L), :], sem_x.at[i])

    def w_copy(j):
        half = lambda ref, c: ref.at[pl.ds(0, D), pl.ds(c * (D // 2), D // 2)]
        src = (half(wk_hbm, 0), wq_hbm, wv_hbm, wo_hbm, wg_hbm, wu_hbm, half(wk_hbm, 1))[j]
        dst = (half(wall, 0), wall.at[pl.ds(D, D), :], wall.at[pl.ds(2 * D, D), :], wo, wg, wu, half(wall, 1))[j]
        return pltpu.make_async_copy(src, dst, sem_w.at[j])

    def wd_copy(j):
        return pltpu.make_async_copy(wd_hbm.at[:, pl.ds(j * 128, 128)], wd.at[j], sem_d.at[j])

    def out_copy(i):
        return pltpu.make_async_copy(xo.at[pl.ds(i * L, L), :], out_hbm.at[0, pl.ds(i * L, L), :], sem_o.at[i])

    x_copy(0).start()
    w_copy(0).start()

    b = beta_ref[...].astype(F32).reshape(1, H)
    wrf[...] = jnp.broadcast_to(wr_ref[...].astype(F32).reshape(1, D), (8, D))
    sg = 1.0 / (1.0 + jnp.exp(-b))
    lane = lax.broadcasted_iota(jnp.int32, (1, H), 1)
    for h in range(H):
        gh = jnp.sum(jnp.where(lane == h, sg, 0.0), axis=1, keepdims=True)
        gs[pl.ds(h * DH, DH), :] = jnp.broadcast_to(gh, (DH, 128))
    for buf in sb:
        buf[...] = jnp.zeros(buf.shape, F32)
    am0[...] = jnp.zeros(am0.shape, F32)
    am1[...] = jnp.zeros(am1.shape, F32)
    tst[...] = jnp.zeros(tst.shape, F32)
    rr[...] = jnp.zeros(rr.shape, F32)

    def ln_first(blk, nchain=0):
        deps = {}
        for k in range(L // 16):
            xv = xin[pl.ds(blk * L + k * 16, 16), :].astype(F32)
            m = jnp.sum(xv, axis=-1, keepdims=True) * (1.0 / D)
            if nchain and k >= nchain:
                m = m + deps[k % nchain]
            xc = xv - m
            rstd = lax.rsqrt(jnp.sum(xc * xc, axis=-1, keepdims=True) * (1.0 / D) + 1e-5)
            xn[pl.ds(blk * (L // 2) + k * 8, 8), :] = _p32(xc * rstd)
            if nchain:
                deps[k % nchain] = jnp.minimum(jnp.abs(rstd), 0.0)

    order = ([("x", 1), ("w", 6), ("x", 2), ("x", 3)] + [("w", j) for j in range(1, 6)]
             + [("d", j) for j in range(NG)])

    def issue(i, c):
        for j, (kind, n) in enumerate(order):
            @pl.when(i == j)
            def _():
                {"x": x_copy, "w": w_copy, "d": wd_copy}[kind](n).start()
        return c
    lax.fori_loop(0, len(order), issue, 0)

    x_copy(0).wait()
    ln_first(0)

    def layer(first):

        def kproj_main(s, g0=0, g1=NG):
            r2 = _mul(s * (L // 2), L // 2)
            kf = _nn(_b16(xn[pl.ds(r2, L // 2), :]), wall[pl.ds(0, D), pl.ds(g0 * 128, (g1 - g0) * 128)])
            pf = _phi(kf)
            zrow = jnp.sum(pf, axis=0, keepdims=True)
            for g in range(g0, g1):
                sl = slice((g - g0) * 128, (g - g0 + 1) * 128)
                kk[g, pl.ds(r2, L // 2), :] = _p32(kf[:, sl])
                pk[g, pl.ds(r2, L // 2), :] = _p32(pf[:, sl])
                zs[pl.ds(_mul(g * 8 * NSEG + s * 8, 8), 8), :] = jnp.broadcast_to(zrow[:, sl], (8, 128))

        def transpose_w(j):
            for c_ in range(D // 128):
                rw = j * D + c_ * 128
                wT[:, pl.ds(rw, 128)] = wall[pl.ds(rw, 128), :].T

        def kproj_first(step, c):
            @pl.when(step == 0)
            def _():
                w_copy(0).wait()
                kproj_main(0, 0, NG // 2)

            @pl.when(step == 1)
            def _():
                x_copy(1).wait()
                w_copy(6).wait()
                ln_first(1, LN_CHAIN)
                kproj_main(0, NG // 2, NG)

            @pl.when(step == 2)
            def _():
                x_copy(2).wait()
                ln_first(2, LN_CHAIN)
                kproj_main(1)

            @pl.when(step == 3)
            def _():
                x_copy(3).wait()
                w_copy(1).wait()
                ln_first(3, LN_CHAIN)
                kproj_main(2)
                transpose_w(1)

            @pl.when(step == 4)
            def _():
                w_copy(2).wait()
                kproj_main(3)
                transpose_w(2)
            return c

        def qv_main(s):
            r = pl.multiple_of(s * L, L)
            r2 = pl.multiple_of(s * (L // 2), L // 2)
            xb_ = _b16(xn[pl.ds(r2, L // 2), :])
            qf = _nt(wT[:, pl.ds(D, D)], xb_)
            q16 = _p32(qf * QSCALE)
            qT[:, pl.ds(r, L)] = q16
            for c_ in range(L // QB):
                qS[:, pl.ds(r + c_ * QB, QB)] = pltpu.roll(q16[:, c_ * QB:(c_ + 1) * QB], QB // 2, 1)
            pqT[:, pl.ds(r, L)] = _p32(_phi(qf))
            vf = _nt(wT[:, pl.ds(2 * D, D)], xb_)
            vT[:, pl.ds(r, L)] = _p32(vf)

        def qv_first(s, c):
            wo32[pl.ds(pl.multiple_of(s * (D // 8), D // 8), D // 8), :] = pltpu.bitcast(
                wo[pl.ds(pl.multiple_of(s * (D // 4), D // 4), D // 4), :], U32)
            qv_main(s)
            return c

        def kqv(s, c):
            kproj_main(s)
            qv_main(s)
            return c

        if first:
            lax.fori_loop(0, 5, kproj_first, 0)
            w_copy(3).wait()
            lax.fori_loop(0, NSEG, qv_first, 0)
        else:
            lax.fori_loop(0, NSEG, kqv, 0)

        def attn(g, c):
            _attn_body(R, g, jnp.maximum(g - 1, 0), g >> 10)
            return c
        lax.fori_loop(0, NG, attn, 0)
        _attn_body(R, NG - 1, NG - 1, 0, do_qk=False)

        def o_dot(r2, j):
            lhs = jnp.concatenate(
                [_b16(ob[g, pl.ds(r2 + j * SUB // 2, SUB // 2), :]) for g in range(NG)], axis=1)
            return _nn(lhs, _b16(wo32[...]))

        STRIP, NCHAIN = O_PACE[first]

        def o_epilogue(t, r0, lane0, racc, deps, cid0, nchain=NCHAIN):
            wr = wrf[pl.ds(0, 1), :]
            lane_i = lax.broadcasted_iota(jnp.int32, (8, 128), 1)
            for k in range(SUB // STRIP):
                rows = pl.ds(r0 + k * STRIP, STRIP)
                rows2 = pl.ds(_mul(r0 // 2 + k * (STRIP // 2), STRIP // 2), STRIP // 2)
                xres = xin[rows, :].astype(F32) if first else xw[rows, :]
                x1 = xres + t[k * STRIP:(k + 1) * STRIP]
                m = jnp.sum(x1, axis=-1, keepdims=True) * (1.0 / D)
                cid = (cid0 + k) % nchain
                if deps.get(cid) is not None:
                    m = m + deps[cid]
                xc = x1 - m
                v = jnp.sum(xc * xc, axis=-1, keepdims=True) * (1.0 / D)
                rstd = lax.rsqrt(v + 1e-5)
                xl = xc * rstd
                rs = jnp.sum(xl * wr, axis=1, keepdims=True)
                for q in range(STRIP // 8):
                    racc = jnp.where(lane_i == lane0 + (k * STRIP) // 8 + q,
                                     jnp.broadcast_to(rs[q * 8:(q + 1) * 8], (8, 128)), racc)
                xb[rows2, :] = _p32(xl)
                if first:
                    xw[rows, :] = x1 + xl
                    c2 = 1.0 + rstd
                    s2 = c2 * lax.rsqrt(v * c2 * c2 + 1e-5)
                    xn[rows2, :] = _p32(xc * s2)
                    deps[cid] = jnp.minimum(jnp.abs(s2), 0.0)
                else:
                    xo[rows, :] = (x1 + xl).astype(BF16)
                    deps[cid] = jnp.minimum(jnp.abs(rstd), 0.0)
            return racc

        nsub = L // SUB
        ninf = jnp.full((8, 128), -jnp.inf, F32)

        def oproj(i, c):
            r = pl.multiple_of(i * L, L)
            r2 = pl.multiple_of(i * (L // 2), L // 2)
            ip = jnp.where(i == 0, NSEG - 1, i - 1)
            rp = pl.multiple_of(ip * L + (nsub - 1) * SUB, SUB)
            rr_prev = pl.ds(pl.multiple_of(jnp.where(i == 0, NSEG, i - 1) * 8, 8), 8)
            deps = {}
            t_prev = o_dot(r2, 0)
            rr[rr_prev, :] = o_epilogue(tst[pl.ds(pl.multiple_of(i >> 10, 8), SUB), :], rp,
                                        ((nsub - 1) * SUB) // 8, rr[rr_prev, :], deps, 0)
            racc = ninf
            for j in range(1, nsub):
                t_cur = o_dot(r2, j)
                racc = o_epilogue(t_prev, r + (j - 1) * SUB, ((j - 1) * SUB) // 8, racc, deps,
                                  j * (SUB // STRIP))
                t_prev = t_cur
            tst[...] = t_prev
            rr[pl.ds(pl.multiple_of(i * 8, 8), 8), :] = racc

            if not first:
                @pl.when(i > 0)
                def _():
                    out_copy(i - 1).start()
            return c
        lax.fori_loop(0, NSEG, oproj, 0)
        rr_last = pl.ds((NSEG - 1) * 8, 8)
        rr[rr_last, :] = o_epilogue(tst[...], (NSEG - 1) * L + (nsub - 1) * SUB,
                                    ((nsub - 1) * SUB) // 8, rr[rr_last, :], {}, 0, nchain=4)
        if not first:
            out_copy(NSEG - 1).start()

        if first:
            w_copy(4).wait()
            w_copy(5).wait()
            for j in range(NG):
                wd_copy(j).wait()

        rv = rr[pl.ds(0, NSEG * 8), :]
        prow = lax.broadcasted_iota(jnp.int32, (NSEG * 8, 128), 0)
        plane = lax.broadcasted_iota(jnp.int32, (NSEG * 8, 128), 1)
        idx = (prow // 8) * L + plane * 8 + prow % 8

        bits = pltpu.bitcast(rv, jnp.int32)
        key = jnp.where(bits < 0, bits ^ 0x7FFFFFFF, bits)
        key = (key & ~(S - 1)) | ((S - 1 - idx) & (S - 1))
        max_all = lambda v: jnp.max(jnp.max(v, axis=0, keepdims=True), axis=1, keepdims=True)
        k1 = max_all(key)
        k2 = max_all(jnp.where(key == k1, jnp.iinfo(jnp.int32).min, key))
        i1 = S - 1 - (k1[0, 0] & (S - 1))
        i2 = S - 1 - (k2[0, 0] & (S - 1))
        g1 = pl.multiple_of((i1 // 16) * 16, 16)
        g2 = pl.multiple_of((i2 // 16) * 16, 16)
        xs = jnp.concatenate([_b16(xb[pl.ds(pl.multiple_of(g1 // 2, 8), 8), :]),
                              _b16(xb[pl.ds(pl.multiple_of(g2 // 2, 8), 8), :])], axis=0)
        gg = _nn(xs, wg[...])
        uu = _nn(xs, wu[...])
        hh = (gg * (1.0 / (1.0 + jnp.exp(-gg))) * uu).astype(BF16)
        yy = jnp.concatenate([_nn(hh, wd[j]) for j in range(NG)], axis=1)
        rsel = jnp.sum(xs.astype(F32) * wrf[pl.ds(0, 1), :], axis=1, keepdims=True)
        yy = yy * (1.0 / (1.0 + jnp.exp(-rsel)))
        riota = lax.broadcasted_iota(jnp.int32, (16, D), 0)
        if not first:
            for i in range(NSEG):
                out_copy(i).wait()
        for j, (ii, gr) in enumerate(((i1, g1), (i2, g2))):
            upd_ = yy[16 * j:16 * (j + 1)]
            if first:
                x2 = xw[pl.ds(gr, 16), :]
                x2 = jnp.where(riota == ii - gr, x2 + upd_, x2)
                xw[pl.ds(gr, 16), :] = x2
                xn[pl.ds(pl.multiple_of(gr // 2, 8), 8), :] = _p32(_ln(x2))
            else:
                x2 = xo[pl.ds(gr, 16), :].astype(F32)
                xo[pl.ds(gr, 16), :] = jnp.where(riota == ii - gr, x2 + upd_, x2).astype(BF16)
        if not first:
            patch = lambda gr, j: pltpu.make_async_copy(
                xo.at[pl.ds(gr, 16), :], out_hbm.at[0, pl.ds(gr, 16), :], sem_o.at[j])
            patch(g1, 0).start()

            @pl.when(g2 != g1)
            def _():
                patch(g2, 1).start()
            patch(g1, 0).wait()

            @pl.when(g2 != g1)
            def _():
                patch(g2, 1).wait()

    layer(True)
    layer(False)


@jax.jit
def pallas_interleave_layers__memory_aug_infini_attn__moe_arch_mod__prompt_kernel(
    A_x: jax.Array,
    A_wq: jax.Array,
    A_wk: jax.Array,
    A_wv: jax.Array,
    A_wo: jax.Array,
    A_beta: jax.Array,
    B_x: jax.Array,
    B_w_r: jax.Array,
    B_w_gate: jax.Array,
    B_w_up: jax.Array,
    B_w_down: jax.Array,
):
    del B_x
    any_spec = pl.BlockSpec(memory_space=pl.ANY)
    small = lambda shape: pl.BlockSpec(shape, lambda: (0,) * len(shape))
    vm = pltpu.VMEM
    scratch = [
        vm((S, D), BF16),
        vm((S, D), F32),
        vm((S // 2, D), U32),
        vm((3 * D, D), BF16),
        vm((D, D), BF16),
        vm((D // 2, D), U32),
        vm((D, 3 * D), BF16),
        vm((D, FF), BF16), vm((D, FF), BF16), vm((NG, FF, 128), BF16),
        vm((D // 2, S), U32), vm((D // 2, S), U32),
        vm((D // 2, S), U32), vm((D // 2, S), U32),
        vm((NG, S // 2, 128), U32), vm((NG, S // 2, 128), U32),
        vm((NG, S // 2, 128), U32),
        vm((S // 2, D), U32),
        vm((NG * NSEG * 8, 128), F32),
        vm((D, 128), F32),
        vm(((NSEG + 1) * 8, 128), F32),
        vm((SUB, D), F32),
        vm((8, D), F32),
        vm((L, QB), F32), vm((L, QB), F32),
        vm((QB + 8, QB), F32),
    ] + [vm((4 * QB + 8, QB), F32) for _ in range(NSB)] + [
        pltpu.SemaphoreType.DMA((NSEG,)),
        pltpu.SemaphoreType.DMA((7,)),
        pltpu.SemaphoreType.DMA((NG,)),
        pltpu.SemaphoreType.DMA((NSEG,)),
    ]
    return pl.pallas_call(
        _kernel,
        out_shape=jax.ShapeDtypeStruct((1, S, D), BF16),
        in_specs=[any_spec, any_spec, any_spec, any_spec, any_spec,
                  small((H,)), small((D,)), any_spec, any_spec, any_spec],
        out_specs=any_spec,
        scratch_shapes=scratch,
        compiler_params=pltpu.CompilerParams(vmem_limit_bytes=110 * 1024 * 1024),
        name="infini_mod",
    )(A_x, A_wq, A_wk, A_wv, A_wo, A_beta, B_w_r, B_w_gate, B_w_up, B_w_down)
```

```python
import numpy as np
import jax
import jax.numpy as jnp
from jax import lax
import jax.experimental.pallas as pl
import jax.experimental.pallas.tpu as pltpu

F32 = jnp.float32
BF16 = jnp.bfloat16
U32 = jnp.uint32

S, D, H, NSEG, FF = 2048, 1024, 32, 4, 3584
DH = D // H
L = S // NSEG
NG = D // 128
HPG = 128 // DH
QB = 128
SUB = 64
O_PACE = {True: (16, 1), False: (16, 1)}
LN_CHAIN = 4


NSB = 16
LOG2E = float(np.log2(np.e))
SCALE = float(np.asarray(DH ** -0.5, dtype=np.float32).astype(jnp.bfloat16).astype(np.float32))
QSCALE = SCALE * LOG2E
MASKV = -1e9 * LOG2E


def _phi(t):
    return jnp.where(t > 0, t + 1.0, jnp.exp(t))


def _ln(x):
    m = jnp.sum(x, axis=-1, keepdims=True) * (1.0 / D)
    xc = x - m
    v = jnp.sum(xc * xc, axis=-1, keepdims=True) * (1.0 / D)
    return xc * lax.rsqrt(v + 1e-5)


def _nt(a, b):
    return lax.dot_general(a, b, (((1,), (1,)), ((), ())), preferred_element_type=F32)


def _nn(a, b):
    return jnp.dot(a, b, preferred_element_type=F32)


def _b16(x):
    return pltpu.bitcast(x, BF16)


def _p32(x):
    return pltpu.bitcast(x.astype(BF16), U32)


def _mul(i, n):
    return i if isinstance(i, int) else pl.multiple_of(i, n)


def _tree(op, xs):
    xs = list(xs)
    while len(xs) > 1:
        nx = [op(xs[i], xs[i + 1]) for i in range(0, len(xs) - 1, 2)]
        if len(xs) % 2:
            nx.append(xs[-1])
        xs = nx
    return xs[0]


def _vsplit(x):
    return [x[i * 8:(i + 1) * 8] for i in range(x.shape[0] // 8)]


class _Sub:
    def __init__(self, idx, s, qb, h):
        self.idx, self.s, self.qb, self.h = idx, s, qb, h
        self.n = qb + 1


ORDER, OFF, SLOPE, UPD_AT, ND_AT = (0, 1, 2, 3), 16, 0, 10, 30


def _attn_plan(order=ORDER, off=OFF):
    subs = []
    for s in range(NSEG):
        for qb in order:
            for h in range(HPG):
                subs.append(_Sub(len(subs), s, qb, h))
    tiles = [(u, kt) for u in subs for kt in range(u.n)]
    n = len(tiles)
    first = {}
    for i, (u, kt) in enumerate(tiles):
        if kt == 0:
            first[u.idx] = i
    pos = [first[u.idx] + u.n - 1 + off + int(SLOPE * kt) for (u, kt) in tiles]
    deferred = set((u.s, u.qb) for i, (u, kt) in enumerate(tiles) if pos[i] >= n)
    now, prev = {}, {}
    for i, (u, kt) in enumerate(tiles):
        if (u.s, u.qb) in deferred:
            prev.setdefault(max(pos[i] - n, 0), []).append(i)
        else:
            now.setdefault(pos[i], []).append(i)
    return tiles, now, prev


_PLAN = _attn_plan()


class _Refs:
    pass


def _attn_body(R, g, gp, zero, do_qk=True):
    tiles, now, prev = _PLAN
    krow = lax.broadcasted_iota(jnp.int32, (QB, QB), 0)
    qcol = lax.broadcasted_iota(jnp.int32, (QB, QB), 1)
    bd = (krow // DH) == (qcol // DH)
    laneh = lax.broadcasted_iota(jnp.int32, (8, QB), 1) // DH
    st, outs, mem = {}, {}, {}

    HB = QB // 2
    lo8 = lax.broadcasted_iota(jnp.int32, (8, QB), 1) < HB
    tri = jnp.where(krow[:HB] > qcol[:HB] % HB, MASKV, 0.0).astype(F32)
    swap = lambda v: pltpu.roll(v, HB, 1)

    def put(u, kt, x):
        buf = R.sb[u.idx % NSB]
        buf[pl.ds(kt * QB, QB), :] = x
        mx = _tree(jnp.maximum, _vsplit(x))
        key = ("m", u.idx)
        st[key] = jnp.maximum(st[key], mx) if key in st else mx
        if kt == (u.qb if (u.h % 2 == 0 or u.qb == 0) else u.qb - 1):
            buf[pl.ds(4 * QB, 8), :] = jnp.broadcast_to(jnp.max(st[key], axis=0, keepdims=True), (8, QB))

    def qk(i):
        u, kt = tiles[i]
        t0 = u.s * L
        q0 = t0 + u.qb * QB
        qrow = lambda ref, h: ref[pl.ds(pl.multiple_of(g * 64 + h * 16, 16), 16), pl.ds(q0, QB)]
        k0 = (t0 + kt * QB) // 2
        if kt < u.qb:
            parts = []
            if u.h > 0:
                parts.append(jnp.zeros((u.h * 16, QB), U32))
            parts.append(qrow(R.qT, u.h))
            if u.h < HPG - 1:
                parts.append(jnp.zeros(((HPG - 1 - u.h) * 16, QB), U32))
            put(u, kt, _nn(_b16(R.kk[g, pl.ds(k0, QB // 2), :]), _b16(jnp.concatenate(parts, axis=0))))
            return
        if u.h % 2 == 1:
            return
        lane16 = lax.broadcasted_iota(jnp.int32, (16, QB), 1) < HB
        z = jnp.uint32(0)

        def packed(rows, wa, wb):
            parts = []
            if u.h > 0:
                parts.append(jnp.zeros((u.h * 16, QB), U32))
            parts += [jnp.where(lane16, wa, z), jnp.where(lane16, z, wb)]
            if u.h < HPG - 2:
                parts.append(jnp.zeros(((HPG - 2 - u.h) * 16, QB), U32))
            return _nn(_b16(R.kk[g, pl.ds(k0, rows // 2), :]), _b16(jnp.concatenate(parts, axis=0)))

        X = packed(QB, qrow(R.qS, u.h), qrow(R.qT, u.h + 1))
        Y = packed(HB, qrow(R.qT, u.h), qrow(R.qS, u.h + 1)) + tri
        X0, X1 = _vsplit(X[:HB]), _vsplit(X[HB:] + tri)
        Y = _vsplit(Y)
        put(u, kt, jnp.concatenate([jnp.where(lo8, y, swap(x)) for x, y in zip(X0, Y)]
                                   + [jnp.where(lo8, MASKV, swap(x)) for x in X1], axis=0))
        put(tiles[i + 1 + u.qb][0], kt,
            jnp.concatenate([jnp.where(lo8, swap(y), x) for x, y in zip(X0, Y)]
                            + [jnp.where(lo8, MASKV, x) for x in X1], axis=0))

    def pv(i, gg, tag):
        u, kt = tiles[i]
        t0 = u.s * L
        q0 = t0 + u.qb * QB
        buf = R.sb[u.idx % NSB]
        km, kl, ko = ("mf", u.idx, tag), ("l", u.idx, tag), ("o", u.idx, tag)
        if kt == 0:
            st[km] = buf[pl.ds(pl.multiple_of(4 * QB + zero, 8), 8), :]
        m = st[km]
        x = buf[pl.ds(pl.multiple_of(kt * QB + zero, 8), QB), :]
        p = jnp.concatenate([jnp.exp2(v - m) for v in _vsplit(x)], axis=0)
        ls = _tree(jnp.add, _vsplit(p))
        st[kl] = ls if kt == 0 else st[kl] + ls
        vt = _b16(R.vT[pl.ds(pl.multiple_of(gg * 64 + u.h * 16, 16), 16), pl.ds(t0 + kt * QB, QB)])
        ot = _nn(vt, p.astype(BF16))
        st[ko] = ot if kt == 0 else st[ko] + ot
        if kt == u.qb:
            l = jnp.sum(st[kl], axis=0, keepdims=True)
            adot = st[ko] * (1.0 / l)
            gt = R.gs[pl.ds(pl.multiple_of(gg * 128 + u.h * DH, 8), 8), :]
            gt = jnp.concatenate([1.0 - gt] * 4, axis=0)
            o = gt * adot
            if u.s > 0:
                o = R.am[u.s % 2][pl.ds(pl.multiple_of(u.qb * QB + u.h * DH + zero, 8), DH), :] + o
            lst = outs.setdefault((u.s, u.qb, tag), [])
            lst.append(o)
            if len(lst) == HPG:
                oT = jnp.concatenate(lst, axis=0)
                R.ob[gg, pl.ds(q0 // 2, QB // 2), :] = _p32(oT.T)

    def upd(s):
        t0 = s * L
        lhs = _b16(R.vT[pl.ds(pl.multiple_of(g * 64, 64), 64), pl.ds(t0, L)])
        rhs = _b16(R.pk[g, pl.ds(t0 // 2, L // 2), :])
        u_ = jnp.where(bd, _nn(lhs, rhs), 0.0)
        zr = R.zs[pl.ds(pl.multiple_of(g * 8 * NSEG + s * 8, 8), 8), :]
        if s == 0:
            mem["M"], mem["z"] = u_, zr
        else:
            mem["M"], mem["z"] = mem["M"] + u_, mem["z"] + zr

    def nd(s):
        t0 = s * L
        zl = [jnp.where(laneh == h, mem["z"], 0.0) for h in range(HPG)]
        lhs = jnp.concatenate([mem["M"]] + zl, axis=0).astype(BF16)
        for qb in range(L // QB):
            r = _nn(lhs, _b16(R.pqT[pl.ds(pl.multiple_of(g * 64, 64), 64), pl.ds(t0 + qb * QB, QB)]))
            for h in range(HPG):
                den = r[128 + 8 * h:128 + 8 * h + 8] + 1e-6
                gt = R.gs[pl.ds(pl.multiple_of(g * 128 + h * DH, 8), 8), :] * (1.0 / den)
                R.am[s % 2][pl.ds(qb * QB + h * DH, DH), :] = (
                    r[h * DH:(h + 1) * DH] * jnp.concatenate([gt] * 4, axis=0))

    extra = {}
    if do_qk:
        for s in range(NSEG - 1):
            extra.setdefault(40 * s + UPD_AT, []).append(("upd", s))
            extra.setdefault(40 * s + ND_AT, []).append(("nd", s + 1))
    for i in range(len(tiles)):
        if do_qk:
            qk(i)
        for kind, s in extra.get(i, []):
            (upd if kind == "upd" else nd)(s)
        for j in prev.get(i, []):
            pv(j, gp, 0)
        if do_qk:
            for j in now.get(i, []):
                pv(j, g, 1)


def _kernel(x_hbm, wq_hbm, wk_hbm, wv_hbm, wo_hbm, beta_ref, wr_ref, wg_hbm, wu_hbm, wd_hbm,
            out_hbm,
            xin, xw, xn, wall, wo, wo32, wT, wg, wu, wd,
            qT, qS, pqT, vT, kk, pk, ob, xb, zs, gs, rr, tst, wrf, am0, am1, *rest):
    sb = rest[:NSB]
    sem_x, sem_w, sem_d, sem_o = rest[NSB:]
    R = _Refs()
    R.qS = qS
    R.qT, R.pqT, R.vT, R.kk, R.pk, R.ob, R.zs, R.gs = qT, pqT, vT, kk, pk, ob, zs, gs
    R.am, R.sb = (am0, am1), sb
    xo = xin

    def x_copy(i):
        return pltpu.make_async_copy(x_hbm.at[0, pl.ds(i * L, L), :], xin.at[pl.ds(i * L, L), :], sem_x.at[i])

    def w_copy(j):
        half = lambda ref, c: ref.at[pl.ds(0, D), pl.ds(c * (D // 2), D // 2)]
        src = (half(wk_hbm, 0), wq_hbm, wv_hbm, wo_hbm, wg_hbm, wu_hbm, half(wk_hbm, 1))[j]
        dst = (half(wall, 0), wall.at[pl.ds(D, D), :], wall.at[pl.ds(2 * D, D), :], wo, wg, wu, half(wall, 1))[j]
        return pltpu.make_async_copy(src, dst, sem_w.at[j])

    def wd_copy(j):
        return pltpu.make_async_copy(wd_hbm.at[:, pl.ds(j * 128, 128)], wd.at[j], sem_d.at[j])

    def out_copy(i):
        return pltpu.make_async_copy(xo.at[pl.ds(i * L, L), :], out_hbm.at[0, pl.ds(i * L, L), :], sem_o.at[i])

    x_copy(0).start()
    w_copy(0).start()

    b = beta_ref[...].astype(F32).reshape(1, H)
    wrf[...] = jnp.broadcast_to(wr_ref[...].astype(F32).reshape(1, D), (8, D))
    sg = 1.0 / (1.0 + jnp.exp(-b))
    lane = lax.broadcasted_iota(jnp.int32, (1, H), 1)
    for h in range(H):
        gh = jnp.sum(jnp.where(lane == h, sg, 0.0), axis=1, keepdims=True)
        gs[pl.ds(h * DH, DH), :] = jnp.broadcast_to(gh, (DH, 128))
    for j in sorted(set(_PLAN[0][t][0].idx % NSB for ts in _PLAN[2].values() for t in ts)):
        sb[j][...] = jnp.zeros(sb[j].shape, F32)
    (am0, am1)[(NSEG - 1) % 2][...] = jnp.zeros(am1.shape, F32)
    tst[...] = jnp.zeros(tst.shape, F32)
    rr[...] = jnp.zeros(rr.shape, F32)

    def ln_rows(row0, nrows, nchain=0):
        deps = {}
        for k in range(nrows // 16):
            xv = xin[pl.ds(_mul(row0 + k * 16, 16), 16), :].astype(F32)
            m = jnp.sum(xv, axis=-1, keepdims=True) * (1.0 / D)
            if nchain and k >= nchain:
                m = m + deps[k % nchain]
            xc = xv - m
            rstd = lax.rsqrt(jnp.sum(xc * xc, axis=-1, keepdims=True) * (1.0 / D) + 1e-5)
            xn[pl.ds(_mul(row0 // 2 + k * 8, 8), 8), :] = _p32(xc * rstd)
            if nchain:
                deps[k % nchain] = jnp.minimum(jnp.abs(rstd), 0.0)

    def ln_first(blk, nchain):
        ln_rows(blk * L, L, nchain)

    order = ([("x", 1), ("w", 6), ("x", 2), ("x", 3)] + [("w", j) for j in range(1, 6)]
             + [("d", j) for j in range(NG)])

    def issue(i, c):
        for j, (kind, n) in enumerate(order):
            @pl.when(i == j)
            def _():
                {"x": x_copy, "w": w_copy, "d": wd_copy}[kind](n).start()
        return c
    lax.fori_loop(0, len(order), issue, 0)

    x_copy(0).wait()

    def ln0(i, c):
        ln_rows(i * (L // 4), L // 4)
        return c
    lax.fori_loop(0, 4, ln0, 0)

    def layer(first):

        def kproj_main(s, g0=0, g1=NG):
            r2 = _mul(s * (L // 2), L // 2)
            kf = _nn(_b16(xn[pl.ds(r2, L // 2), :]), wall[pl.ds(0, D), pl.ds(g0 * 128, (g1 - g0) * 128)])
            pf = _phi(kf)
            zrow = jnp.sum(pf, axis=0, keepdims=True)
            for g in range(g0, g1):
                sl = slice((g - g0) * 128, (g - g0 + 1) * 128)
                kk[g, pl.ds(r2, L // 2), :] = _p32(kf[:, sl])
                pk[g, pl.ds(r2, L // 2), :] = _p32(pf[:, sl])
                zs[pl.ds(_mul(g * 8 * NSEG + s * 8, 8), 8), :] = jnp.broadcast_to(zrow[:, sl], (8, 128))

        def transpose_w(j):
            for c_ in range(D // 128):
                rw = j * D + c_ * 128
                wT[:, pl.ds(rw, 128)] = wall[pl.ds(rw, 128), :].T

        def kproj_first(step, c):
            @pl.when(step == 0)
            def _():
                w_copy(0).wait()
                kproj_main(0, 0, NG // 2)

            @pl.when(step == 1)
            def _():
                x_copy(1).wait()
                w_copy(6).wait()
                ln_first(1, LN_CHAIN)
                kproj_main(0, NG // 2, NG)

            @pl.when(step == 2)
            def _():
                x_copy(2).wait()
                ln_first(2, LN_CHAIN)
                kproj_main(1)

            @pl.when(step == 3)
            def _():
                x_copy(3).wait()
                w_copy(1).wait()
                ln_first(3, LN_CHAIN)
                kproj_main(2)
                transpose_w(1)

            @pl.when(step == 4)
            def _():
                w_copy(2).wait()
                kproj_main(3)
                transpose_w(2)
            return c

        def qv_main(s):
            r = pl.multiple_of(s * L, L)
            r2 = pl.multiple_of(s * (L // 2), L // 2)
            xb_ = _b16(xn[pl.ds(r2, L // 2), :])
            qf = _nt(wT[:, pl.ds(D, D)], xb_)
            q16 = _p32(qf * QSCALE)
            qT[:, pl.ds(r, L)] = q16
            for c_ in range(L // QB):
                qS[:, pl.ds(r + c_ * QB, QB)] = pltpu.roll(q16[:, c_ * QB:(c_ + 1) * QB], QB // 2, 1)
            pqT[:, pl.ds(r, L)] = _p32(_phi(qf))
            vf = _nt(wT[:, pl.ds(2 * D, D)], xb_)
            vT[:, pl.ds(r, L)] = _p32(vf)

        def qv_first(s, c):
            wo32[pl.ds(pl.multiple_of(s * (D // 8), D // 8), D // 8), :] = pltpu.bitcast(
                wo[pl.ds(pl.multiple_of(s * (D // 4), D // 4), D // 4), :], U32)
            qv_main(s)
            return c

        def kqv(s, c):
            kproj_main(s)
            qv_main(s)
            return c

        if first:
            lax.fori_loop(0, 5, kproj_first, 0)
            w_copy(3).wait()
            lax.fori_loop(0, NSEG, qv_first, 0)
        else:
            lax.fori_loop(0, NSEG, kqv, 0)

        def attn(g, c):
            _attn_body(R, g, jnp.maximum(g - 1, 0), g >> 10)
            return c
        lax.fori_loop(0, NG, attn, 0)
        _attn_body(R, NG - 1, NG - 1, 0, do_qk=False)

        def o_dot(r2, j):
            lhs = jnp.concatenate(
                [_b16(ob[g, pl.ds(r2 + j * SUB // 2, SUB // 2), :]) for g in range(NG)], axis=1)
            return _nn(lhs, _b16(wo32[...]))

        STRIP, NCHAIN = O_PACE[first]

        def o_epilogue(t, r0, lane0, racc, deps, cid0, nchain=NCHAIN):
            wr = wrf[pl.ds(0, 1), :]
            lane_i = lax.broadcasted_iota(jnp.int32, (8, 128), 1)
            for k in range(SUB // STRIP):
                rows = pl.ds(r0 + k * STRIP, STRIP)
                rows2 = pl.ds(_mul(r0 // 2 + k * (STRIP // 2), STRIP // 2), STRIP // 2)
                xres = xin[rows, :].astype(F32) if first else xw[rows, :]
                x1 = xres + t[k * STRIP:(k + 1) * STRIP]
                m = jnp.sum(x1, axis=-1, keepdims=True) * (1.0 / D)
                cid = (cid0 + k) % nchain
                if deps.get(cid) is not None:
                    m = m + deps[cid]
                xc = x1 - m
                v = jnp.sum(xc * xc, axis=-1, keepdims=True) * (1.0 / D)
                rstd = lax.rsqrt(v + 1e-5)
                xl = xc * rstd
                rs = jnp.sum(xl * wr, axis=1, keepdims=True)
                for q in range(STRIP // 8):
                    racc = jnp.where(lane_i == lane0 + (k * STRIP) // 8 + q,
                                     jnp.broadcast_to(rs[q * 8:(q + 1) * 8], (8, 128)), racc)
                xb[rows2, :] = _p32(xl)
                if first:
                    xw[rows, :] = x1 + xl
                    c2 = 1.0 + rstd
                    s2 = c2 * lax.rsqrt(v * c2 * c2 + 1e-5)
                    xn[rows2, :] = _p32(xc * s2)
                    deps[cid] = jnp.minimum(jnp.abs(s2), 0.0)
                else:
                    xo[rows, :] = (x1 + xl).astype(BF16)
                    deps[cid] = jnp.minimum(jnp.abs(rstd), 0.0)
            return racc

        nsub = L // SUB
        ninf = jnp.full((8, 128), -jnp.inf, F32)

        def oproj(i, c):
            r = pl.multiple_of(i * L, L)
            r2 = pl.multiple_of(i * (L // 2), L // 2)
            ip = jnp.where(i == 0, NSEG - 1, i - 1)
            rp = pl.multiple_of(ip * L + (nsub - 1) * SUB, SUB)
            rr_prev = pl.ds(pl.multiple_of(jnp.where(i == 0, NSEG, i - 1) * 8, 8), 8)
            deps = {}
            t_prev = o_dot(r2, 0)
            rr[rr_prev, :] = o_epilogue(tst[pl.ds(pl.multiple_of(i >> 10, 8), SUB), :], rp,
                                        ((nsub - 1) * SUB) // 8, rr[rr_prev, :], deps, 0)
            racc = ninf
            for j in range(1, nsub):
                t_cur = o_dot(r2, j)
                racc = o_epilogue(t_prev, r + (j - 1) * SUB, ((j - 1) * SUB) // 8, racc, deps,
                                  j * (SUB // STRIP))
                t_prev = t_cur
            tst[...] = t_prev
            rr[pl.ds(pl.multiple_of(i * 8, 8), 8), :] = racc

            if not first:
                @pl.when(i > 0)
                def _():
                    out_copy(i - 1).start()
            return c
        lax.fori_loop(0, NSEG, oproj, 0)
        rr_last = pl.ds((NSEG - 1) * 8, 8)
        rr[rr_last, :] = o_epilogue(tst[...], (NSEG - 1) * L + (nsub - 1) * SUB,
                                    ((nsub - 1) * SUB) // 8, rr[rr_last, :], {}, 0, nchain=4)
        if not first:
            out_copy(NSEG - 1).start()

        if first:
            w_copy(4).wait()
            w_copy(5).wait()
            for j in range(NG):
                wd_copy(j).wait()

        rv = rr[pl.ds(0, NSEG * 8), :]
        prow = lax.broadcasted_iota(jnp.int32, (NSEG * 8, 128), 0)
        plane = lax.broadcasted_iota(jnp.int32, (NSEG * 8, 128), 1)
        idx = (prow // 8) * L + plane * 8 + prow % 8

        bits = pltpu.bitcast(rv, jnp.int32)
        key = jnp.where(bits < 0, bits ^ 0x7FFFFFFF, bits)
        key = (key & ~(S - 1)) | ((S - 1 - idx) & (S - 1))
        max_all = lambda v: jnp.max(jnp.max(v, axis=0, keepdims=True), axis=1, keepdims=True)
        k1 = max_all(key)
        k2 = max_all(jnp.where(key == k1, jnp.iinfo(jnp.int32).min, key))
        i1 = S - 1 - (k1[0, 0] & (S - 1))
        i2 = S - 1 - (k2[0, 0] & (S - 1))
        g1 = pl.multiple_of((i1 // 16) * 16, 16)
        g2 = pl.multiple_of((i2 // 16) * 16, 16)
        xs = jnp.concatenate([_b16(xb[pl.ds(pl.multiple_of(g1 // 2, 8), 8), :]),
                              _b16(xb[pl.ds(pl.multiple_of(g2 // 2, 8), 8), :])], axis=0)
        gg = _nn(xs, wg[...])
        uu = _nn(xs, wu[...])
        hh = (gg * (1.0 / (1.0 + jnp.exp(-gg))) * uu).astype(BF16)
        yy = jnp.concatenate([_nn(hh, wd[j]) for j in range(NG)], axis=1)
        rsel = jnp.sum(xs.astype(F32) * wrf[pl.ds(0, 1), :], axis=1, keepdims=True)
        yy = yy * (1.0 / (1.0 + jnp.exp(-rsel)))
        riota = lax.broadcasted_iota(jnp.int32, (16, D), 0)
        if not first:
            for i in range(NSEG):
                out_copy(i).wait()
        for j, (ii, gr) in enumerate(((i1, g1), (i2, g2))):
            upd_ = yy[16 * j:16 * (j + 1)]
            if first:
                x2 = xw[pl.ds(gr, 16), :]
                x2 = jnp.where(riota == ii - gr, x2 + upd_, x2)
                xw[pl.ds(gr, 16), :] = x2
                xn[pl.ds(pl.multiple_of(gr // 2, 8), 8), :] = _p32(_ln(x2))
            else:
                x2 = xo[pl.ds(gr, 16), :].astype(F32)
                xo[pl.ds(gr, 16), :] = jnp.where(riota == ii - gr, x2 + upd_, x2).astype(BF16)
        if not first:
            patch = lambda gr, j: pltpu.make_async_copy(
                xo.at[pl.ds(gr, 16), :], out_hbm.at[0, pl.ds(gr, 16), :], sem_o.at[j])
            patch(g1, 0).start()

            @pl.when(g2 != g1)
            def _():
                patch(g2, 1).start()
            patch(g1, 0).wait()

            @pl.when(g2 != g1)
            def _():
                patch(g2, 1).wait()

    layer(True)
    layer(False)


@jax.jit
def pallas_interleave_layers__memory_aug_infini_attn__moe_arch_mod__prompt_kernel(
    A_x: jax.Array,
    A_wq: jax.Array,
    A_wk: jax.Array,
    A_wv: jax.Array,
    A_wo: jax.Array,
    A_beta: jax.Array,
    B_x: jax.Array,
    B_w_r: jax.Array,
    B_w_gate: jax.Array,
    B_w_up: jax.Array,
    B_w_down: jax.Array,
):
    del B_x
    any_spec = pl.BlockSpec(memory_space=pl.ANY)
    small = lambda shape: pl.BlockSpec(shape, lambda: (0,) * len(shape))
    vm = pltpu.VMEM
    scratch = [
        vm((S, D), BF16),
        vm((S, D), F32),
        vm((S // 2, D), U32),
        vm((3 * D, D), BF16),
        vm((D, D), BF16),
        vm((D // 2, D), U32),
        vm((D, 3 * D), BF16),
        vm((D, FF), BF16), vm((D, FF), BF16), vm((NG, FF, 128), BF16),
        vm((D // 2, S), U32), vm((D // 2, S), U32),
        vm((D // 2, S), U32), vm((D // 2, S), U32),
        vm((NG, S // 2, 128), U32), vm((NG, S // 2, 128), U32),
        vm((NG, S // 2, 128), U32),
        vm((S // 2, D), U32),
        vm((NG * NSEG * 8, 128), F32),
        vm((D, 128), F32),
        vm(((NSEG + 1) * 8, 128), F32),
        vm((SUB, D), F32),
        vm((8, D), F32),
        vm((L, QB), F32), vm((L, QB), F32),
    ] + [vm((4 * QB + 8, QB), F32) for _ in range(NSB)] + [
        pltpu.SemaphoreType.DMA((NSEG,)),
        pltpu.SemaphoreType.DMA((7,)),
        pltpu.SemaphoreType.DMA((NG,)),
        pltpu.SemaphoreType.DMA((NSEG,)),
    ]
    return pl.pallas_call(
        _kernel,
        out_shape=jax.ShapeDtypeStruct((1, S, D), BF16),
        in_specs=[any_spec, any_spec, any_spec, any_spec, any_spec,
                  small((H,)), small((D,)), any_spec, any_spec, any_spec],
        out_specs=any_spec,
        scratch_shapes=scratch,
        compiler_params=pltpu.CompilerParams(vmem_limit_bytes=110 * 1024 * 1024),
        name="infini_mod",
    )(A_x, A_wq, A_wk, A_wv, A_wo, A_beta, B_w_r, B_w_gate, B_w_up, B_w_down)
```

```python
import numpy as np
import jax
import jax.numpy as jnp
from jax import lax
import jax.experimental.pallas as pl
import jax.experimental.pallas.tpu as pltpu

F32 = jnp.float32
BF16 = jnp.bfloat16
U32 = jnp.uint32

S, D, H, NSEG, FF = 2048, 1024, 32, 4, 3584
DH = D // H
L = S // NSEG
NG = D // 128
HPG = 128 // DH
QB = 128
SUB = 64
O_PACE = {True: (16, 1), False: (16, 1)}
LN_CHAIN = 4


NSB = 16
LOG2E = float(np.log2(np.e))
SCALE = float(np.asarray(DH ** -0.5, dtype=np.float32).astype(jnp.bfloat16).astype(np.float32))
QSCALE = SCALE * LOG2E
MASKV = -1e9 * LOG2E


def _phi(t):
    return jnp.where(t > 0, t + 1.0, jnp.exp(t))


def _ln(x):
    m = jnp.sum(x, axis=-1, keepdims=True) * (1.0 / D)
    xc = x - m
    v = jnp.sum(xc * xc, axis=-1, keepdims=True) * (1.0 / D)
    return xc * lax.rsqrt(v + 1e-5)


def _nt(a, b):
    return lax.dot_general(a, b, (((1,), (1,)), ((), ())), preferred_element_type=F32)


def _nn(a, b):
    return jnp.dot(a, b, preferred_element_type=F32)


def _b16(x):
    return pltpu.bitcast(x, BF16)


def _p32(x):
    return pltpu.bitcast(x.astype(BF16), U32)


def _mul(i, n):
    return i if isinstance(i, int) else pl.multiple_of(i, n)


def _tree(op, xs):
    xs = list(xs)
    while len(xs) > 1:
        nx = [op(xs[i], xs[i + 1]) for i in range(0, len(xs) - 1, 2)]
        if len(xs) % 2:
            nx.append(xs[-1])
        xs = nx
    return xs[0]


def _vsplit(x):
    return [x[i * 8:(i + 1) * 8] for i in range(x.shape[0] // 8)]


class _Sub:
    def __init__(self, idx, s, qb, h):
        self.idx, self.s, self.qb, self.h = idx, s, qb, h
        self.n = qb + 1


ORDER, OFF, SLOPE, UPD_AT, ND_AT, ND_STEP = (0, 1, 2, 3), 16, 0, 10, 30, 0


def _attn_plan(order=ORDER, off=OFF):
    subs = []
    for s in range(NSEG):
        for qb in order:
            for h in range(HPG):
                subs.append(_Sub(len(subs), s, qb, h))
    tiles = [(u, kt) for u in subs for kt in range(u.n)]
    n = len(tiles)
    first = {}
    for i, (u, kt) in enumerate(tiles):
        if kt == 0:
            first[u.idx] = i
    pos = [first[u.idx] + u.n - 1 + off + int(SLOPE * kt) for (u, kt) in tiles]
    deferred = set((u.s, u.qb) for i, (u, kt) in enumerate(tiles) if pos[i] >= n)
    now, prev = {}, {}
    for i, (u, kt) in enumerate(tiles):
        if (u.s, u.qb) in deferred:
            prev.setdefault(max(pos[i] - n, 0), []).append(i)
        else:
            now.setdefault(pos[i], []).append(i)
    return tiles, now, prev


_PLAN = _attn_plan()


class _Refs:
    pass


def _attn_body(R, g, gp, zsrc, do_qk=True):
    tiles, now, prev = _PLAN
    krow = lax.broadcasted_iota(jnp.int32, (QB, QB), 0)
    qcol = lax.broadcasted_iota(jnp.int32, (QB, QB), 1)
    bd = (krow // DH) == (qcol // DH)
    st, outs, mem = {}, {}, {}

    HB = QB // 2
    lo8 = lax.broadcasted_iota(jnp.int32, (8, QB), 1) < HB
    tri = jnp.where(krow[:HB] > qcol[:HB] % HB, MASKV, 0.0).astype(F32)
    swap = lambda v: pltpu.roll(v, HB, 1)

    def put(u, kt, x):
        buf = R.sb[u.idx % NSB]
        buf[pl.ds(kt * QB, QB), :] = x
        mx = _tree(jnp.maximum, _vsplit(x))
        key = ("m", u.idx)
        st[key] = jnp.maximum(st[key], mx) if key in st else mx
        if kt == (u.qb if (u.h % 2 == 0 or u.qb == 0) else u.qb - 1):
            buf[pl.ds(4 * QB, 8), :] = jnp.broadcast_to(jnp.max(st[key], axis=0, keepdims=True), (8, QB))

    def qk(i):
        u, kt = tiles[i]
        t0 = u.s * L
        q0 = t0 + u.qb * QB
        qrow = lambda ref, h: ref[pl.ds(pl.multiple_of(g * 64 + h * 16, 16), 16), pl.ds(q0, QB)]
        k0 = (t0 + kt * QB) // 2
        if kt < u.qb:
            parts = []
            if u.h > 0:
                parts.append(jnp.zeros((u.h * 16, QB), U32))
            parts.append(qrow(R.qT, u.h))
            if u.h < HPG - 1:
                parts.append(jnp.zeros(((HPG - 1 - u.h) * 16, QB), U32))
            put(u, kt, _nn(_b16(R.kk[g, pl.ds(k0, QB // 2), :]), _b16(jnp.concatenate(parts, axis=0))))
            return
        if u.h % 2 == 1:
            return
        lane16 = lax.broadcasted_iota(jnp.int32, (16, QB), 1) < HB
        z = jnp.uint32(0)

        def packed(rows, wa, wb):
            parts = []
            if u.h > 0:
                parts.append(jnp.zeros((u.h * 16, QB), U32))
            parts += [jnp.where(lane16, wa, z), jnp.where(lane16, z, wb)]
            if u.h < HPG - 2:
                parts.append(jnp.zeros(((HPG - 2 - u.h) * 16, QB), U32))
            return _nn(_b16(R.kk[g, pl.ds(k0, rows // 2), :]), _b16(jnp.concatenate(parts, axis=0)))

        X = packed(QB, qrow(R.qS, u.h), qrow(R.qT, u.h + 1))
        Y = packed(HB, qrow(R.qT, u.h), qrow(R.qS, u.h + 1)) + tri
        X0, X1 = _vsplit(X[:HB]), _vsplit(X[HB:] + tri)
        Y = _vsplit(Y)
        put(u, kt, jnp.concatenate([jnp.where(lo8, y, swap(x)) for x, y in zip(X0, Y)]
                                   + [jnp.where(lo8, MASKV, swap(x)) for x in X1], axis=0))
        put(tiles[i + 1 + u.qb][0], kt,
            jnp.concatenate([jnp.where(lo8, swap(y), x) for x, y in zip(X0, Y)]
                            + [jnp.where(lo8, MASKV, x) for x in X1], axis=0))

    def pv(i, gg, tag):
        u, kt = tiles[i]
        zero = 0 if isinstance(zsrc, int) else (zsrc + i) >> 12
        t0 = u.s * L
        q0 = t0 + u.qb * QB
        buf = R.sb[u.idx % NSB]
        km, kl, ko = ("mf", u.idx, tag), ("l", u.idx, tag), ("o", u.idx, tag)
        if kt == 0:
            st[km] = buf[pl.ds(pl.multiple_of(4 * QB + zero, 8), 8), :]
        m = st[km]
        x = buf[pl.ds(pl.multiple_of(kt * QB + zero, 8), QB), :]
        p = jnp.concatenate([jnp.exp2(v - m) for v in _vsplit(x)], axis=0)
        ls = _tree(jnp.add, _vsplit(p))
        st[kl] = ls if kt == 0 else st[kl] + ls
        vt = _b16(R.vT[pl.ds(pl.multiple_of(gg * 64 + u.h * 16, 16), 16), pl.ds(t0 + kt * QB, QB)])
        ot = _nn(vt, p.astype(BF16))
        st[ko] = ot if kt == 0 else st[ko] + ot
        if kt == u.qb:
            l = jnp.sum(st[kl], axis=0, keepdims=True)
            adot = st[ko] * (1.0 / l)
            gt = R.gs[pl.ds(pl.multiple_of(gg * 128 + u.h * DH, 8), 8), :]
            gt = jnp.concatenate([1.0 - gt] * 4, axis=0)
            o = gt * adot
            if u.s > 0:
                o = R.am[u.s % 2][pl.ds(pl.multiple_of(u.qb * QB + u.h * DH + zero, 8), DH), :] + o
            lst = outs.setdefault((u.s, u.qb, tag), [])
            lst.append(o)
            if len(lst) == HPG:
                oT = jnp.concatenate(lst, axis=0)
                R.ob[gg, pl.ds(q0 // 2, QB // 2), :] = _p32(oT.T)

    def upd(s):
        t0 = s * L
        lhs = _b16(R.vT[pl.ds(pl.multiple_of(g * 64, 64), 64), pl.ds(t0, L)])
        rhs = _b16(R.pk[g, pl.ds(t0 // 2, L // 2), :])
        u_ = jnp.where(bd, _nn(lhs, rhs), 0.0)
        zr = R.zs[pl.ds(pl.multiple_of(g * 8 * NSEG + s * 8, 8), 8), :]
        if s == 0:
            mem["M"], mem["z"] = u_, zr
        else:
            mem["M"], mem["z"] = mem["M"] + u_, mem["z"] + zr

    def nd(s, qb):
        t0 = s * L
        row16 = lax.broadcasted_iota(jnp.int32, (16, QB), 0)
        lane16h = lax.broadcasted_iota(jnp.int32, (16, QB), 1) // DH
        z16 = jnp.concatenate([mem["z"], mem["z"]], axis=0)
        zl = jnp.where(row16 == lane16h, z16, 0.0)
        lhs = jnp.concatenate([mem["M"], zl], axis=0).astype(BF16)
        r = _nn(lhs, _b16(R.pqT[pl.ds(pl.multiple_of(g * 64, 64), 64), pl.ds(t0 + qb * QB, QB)]))
        rden = 1.0 / (r[128:136] + 1e-6)
        for h in range(HPG):
            gt = (R.gs[pl.ds(pl.multiple_of(g * 128 + h * DH, 8), 8), :]
                  * jnp.broadcast_to(rden[h:h + 1], (8, QB)))
            R.am[s % 2][pl.ds(qb * QB + h * DH, DH), :] = (
                r[h * DH:(h + 1) * DH] * jnp.concatenate([gt] * 4, axis=0))

    extra = {}
    if do_qk:
        for s in range(NSEG - 1):
            extra.setdefault(40 * s + UPD_AT, []).append(("upd", s, 0))
            for qb in range(L // QB):
                extra.setdefault(min(40 * s + ND_AT + ND_STEP * qb, 40 * s + 39), []).append(("nd", s + 1, qb))
    for i in range(len(tiles)):
        if do_qk:
            qk(i)
        for kind, s, qb in extra.get(i, []):
            upd(s) if kind == "upd" else nd(s, qb)
        for j in prev.get(i, []):
            pv(j, gp, 0)
        if do_qk:
            for j in now.get(i, []):
                pv(j, g, 1)


def _kernel(x_hbm, wq_hbm, wk_hbm, wv_hbm, wo_hbm, beta_ref, wr_ref, wg_hbm, wu_hbm, wd_hbm,
            out_hbm,
            xin, xw, xn, wall, wo, wo32, wT, wg, wu, wd,
            qT, qS, pqT, vT, kk, pk, ob, xb, zs, gs, rr, tst, wrf, am0, am1, *rest):
    sb = rest[:NSB]
    sem_x, sem_w, sem_d, sem_o = rest[NSB:]
    R = _Refs()
    R.qS = qS
    R.qT, R.pqT, R.vT, R.kk, R.pk, R.ob, R.zs, R.gs = qT, pqT, vT, kk, pk, ob, zs, gs
    R.am, R.sb = (am0, am1), sb
    xo = xin

    def x_copy(i):
        return pltpu.make_async_copy(x_hbm.at[0, pl.ds(i * L, L), :], xin.at[pl.ds(i * L, L), :], sem_x.at[i])

    def w_copy(j):
        half = lambda ref, c: ref.at[pl.ds(0, D), pl.ds(c * (D // 2), D // 2)]
        src = (half(wk_hbm, 0), wq_hbm, wv_hbm, wo_hbm, wg_hbm, wu_hbm, half(wk_hbm, 1))[j]
        dst = (half(wall, 0), wall.at[pl.ds(D, D), :], wall.at[pl.ds(2 * D, D), :], wo, wg, wu, half(wall, 1))[j]
        return pltpu.make_async_copy(src, dst, sem_w.at[j])

    def wd_copy(j):
        return pltpu.make_async_copy(wd_hbm.at[:, pl.ds(j * 128, 128)], wd.at[j], sem_d.at[j])

    def out_copy(i):
        return pltpu.make_async_copy(xo.at[pl.ds(i * L, L), :], out_hbm.at[0, pl.ds(i * L, L), :], sem_o.at[i])

    x_copy(0).start()
    w_copy(0).start()

    b = beta_ref[...].astype(F32).reshape(1, H)
    wrf[...] = jnp.broadcast_to(wr_ref[...].astype(F32).reshape(1, D), (8, D))
    sg = 1.0 / (1.0 + jnp.exp(-b))
    lane = lax.broadcasted_iota(jnp.int32, (1, H), 1)
    for h in range(H):
        gh = jnp.sum(jnp.where(lane == h, sg, 0.0), axis=1, keepdims=True)
        gs[pl.ds(h * DH, DH), :] = jnp.broadcast_to(gh, (DH, 128))
    for j in sorted(set(_PLAN[0][t][0].idx % NSB for ts in _PLAN[2].values() for t in ts)):
        sb[j][...] = jnp.zeros(sb[j].shape, F32)
    (am0, am1)[(NSEG - 1) % 2][...] = jnp.zeros(am1.shape, F32)
    tst[...] = jnp.zeros(tst.shape, F32)
    rr[...] = jnp.zeros(rr.shape, F32)

    def ln_rows(row0, nrows, nchain=0):
        deps = {}
        for k in range(nrows // 16):
            xv = xin[pl.ds(_mul(row0 + k * 16, 16), 16), :].astype(F32)
            m = jnp.sum(xv, axis=-1, keepdims=True) * (1.0 / D)
            if nchain and k >= nchain:
                m = m + deps[k % nchain]
            xc = xv - m
            rstd = lax.rsqrt(jnp.sum(xc * xc, axis=-1, keepdims=True) * (1.0 / D) + 1e-5)
            xn[pl.ds(_mul(row0 // 2 + k * 8, 8), 8), :] = _p32(xc * rstd)
            if nchain:
                deps[k % nchain] = jnp.minimum(jnp.abs(rstd), 0.0)

    def ln_first(blk, nchain):
        ln_rows(blk * L, L, nchain)

    order = ([("x", 1), ("w", 6), ("x", 2), ("x", 3)] + [("w", j) for j in range(1, 6)]
             + [("d", j) for j in range(NG)])

    def issue(i, c):
        for j, (kind, n) in enumerate(order):
            @pl.when(i == j)
            def _():
                {"x": x_copy, "w": w_copy, "d": wd_copy}[kind](n).start()
        return c
    lax.fori_loop(0, len(order), issue, 0)

    x_copy(0).wait()

    def ln0(i, c):
        ln_rows(i * (L // 4), L // 4)
        return c
    lax.fori_loop(0, 4, ln0, 0)

    def layer(first):

        def kproj_main(s, g0=0, g1=NG):
            r2 = _mul(s * (L // 2), L // 2)
            kf = _nn(_b16(xn[pl.ds(r2, L // 2), :]), wall[pl.ds(0, D), pl.ds(g0 * 128, (g1 - g0) * 128)])
            pf = _phi(kf)
            zrow = jnp.sum(pf, axis=0, keepdims=True)
            for g in range(g0, g1):
                sl = slice((g - g0) * 128, (g - g0 + 1) * 128)
                kk[g, pl.ds(r2, L // 2), :] = _p32(kf[:, sl])
                pk[g, pl.ds(r2, L // 2), :] = _p32(pf[:, sl])
                zs[pl.ds(_mul(g * 8 * NSEG + s * 8, 8), 8), :] = jnp.broadcast_to(zrow[:, sl], (8, 128))

        def transpose_w(j):
            for c_ in range(D // 128):
                rw = j * D + c_ * 128
                wT[:, pl.ds(rw, 128)] = wall[pl.ds(rw, 128), :].T

        def kproj_first(step, c):
            @pl.when(step == 0)
            def _():
                w_copy(0).wait()
                kproj_main(0, 0, NG // 2)

            @pl.when(step == 1)
            def _():
                x_copy(1).wait()
                w_copy(6).wait()
                ln_first(1, LN_CHAIN)
                kproj_main(0, NG // 2, NG)

            @pl.when(step == 2)
            def _():
                x_copy(2).wait()
                ln_first(2, LN_CHAIN)
                kproj_main(1)

            @pl.when(step == 3)
            def _():
                x_copy(3).wait()
                w_copy(1).wait()
                ln_first(3, LN_CHAIN)
                kproj_main(2)
                transpose_w(1)

            @pl.when(step == 4)
            def _():
                w_copy(2).wait()
                kproj_main(3)
                transpose_w(2)
            return c

        def qv_main(s):
            r = pl.multiple_of(s * L, L)
            r2 = pl.multiple_of(s * (L // 2), L // 2)
            xb_ = _b16(xn[pl.ds(r2, L // 2), :])
            qf = _nt(wT[:, pl.ds(D, D)], xb_)
            q16 = _p32(qf * QSCALE)
            qT[:, pl.ds(r, L)] = q16
            for c_ in range(L // QB):
                qS[:, pl.ds(r + c_ * QB, QB)] = pltpu.roll(q16[:, c_ * QB:(c_ + 1) * QB], QB // 2, 1)
            pqT[:, pl.ds(r, L)] = _p32(_phi(qf))
            vf = _nt(wT[:, pl.ds(2 * D, D)], xb_)
            vT[:, pl.ds(r, L)] = _p32(vf)

        def qv_first(s, c):
            wo32[pl.ds(pl.multiple_of(s * (D // 8), D // 8), D // 8), :] = pltpu.bitcast(
                wo[pl.ds(pl.multiple_of(s * (D // 4), D // 4), D // 4), :], U32)
            qv_main(s)
            return c

        def kqv(s, c):
            kproj_main(s)
            qv_main(s)
            return c

        if first:
            lax.fori_loop(0, 5, kproj_first, 0)
            w_copy(3).wait()
            lax.fori_loop(0, NSEG, qv_first, 0)
        else:
            lax.fori_loop(0, NSEG, kqv, 0)

        def attn(g, c):
            _attn_body(R, g, jnp.maximum(g - 1, 0), g)
            return c
        lax.fori_loop(0, NG, attn, 0)
        _attn_body(R, NG - 1, NG - 1, 0, do_qk=False)

        def o_dot(r2, j):
            lhs = jnp.concatenate(
                [_b16(ob[g, pl.ds(r2 + j * SUB // 2, SUB // 2), :]) for g in range(NG)], axis=1)
            return _nn(lhs, _b16(wo32[...]))

        STRIP, NCHAIN = O_PACE[first]

        def o_epilogue(t, r0, lane0, racc, deps, cid0, nchain=NCHAIN):
            wr = wrf[pl.ds(0, 1), :]
            lane_i = lax.broadcasted_iota(jnp.int32, (8, 128), 1)
            for k in range(SUB // STRIP):
                rows = pl.ds(r0 + k * STRIP, STRIP)
                rows2 = pl.ds(_mul(r0 // 2 + k * (STRIP // 2), STRIP // 2), STRIP // 2)
                xres = xin[rows, :].astype(F32) if first else xw[rows, :]
                x1 = xres + t[k * STRIP:(k + 1) * STRIP]
                m = jnp.sum(x1, axis=-1, keepdims=True) * (1.0 / D)
                cid = (cid0 + k) % nchain
                if deps.get(cid) is not None:
                    m = m + deps[cid]
                xc = x1 - m
                v = jnp.sum(xc * xc, axis=-1, keepdims=True) * (1.0 / D)
                rstd = lax.rsqrt(v + 1e-5)
                xl = xc * rstd
                rs = jnp.sum(xl * wr, axis=1, keepdims=True)
                for q in range(STRIP // 8):
                    racc = jnp.where(lane_i == lane0 + (k * STRIP) // 8 + q,
                                     jnp.broadcast_to(rs[q * 8:(q + 1) * 8], (8, 128)), racc)
                xb[rows2, :] = _p32(xl)
                if first:
                    xw[rows, :] = x1 + xl
                    c2 = 1.0 + rstd
                    s2 = c2 * lax.rsqrt(v * c2 * c2 + 1e-5)
                    xn[rows2, :] = _p32(xc * s2)
                    deps[cid] = jnp.minimum(jnp.abs(s2), 0.0)
                else:
                    xo[rows, :] = (x1 + xl).astype(BF16)
                    deps[cid] = jnp.minimum(jnp.abs(rstd), 0.0)
            return racc

        nsub = L // SUB
        ninf = jnp.full((8, 128), -jnp.inf, F32)

        def oproj(i, c):
            r = pl.multiple_of(i * L, L)
            r2 = pl.multiple_of(i * (L // 2), L // 2)
            ip = jnp.where(i == 0, NSEG - 1, i - 1)
            rp = pl.multiple_of(ip * L + (nsub - 1) * SUB, SUB)
            rr_prev = pl.ds(pl.multiple_of(jnp.where(i == 0, NSEG, i - 1) * 8, 8), 8)
            deps = {}
            t_prev = o_dot(r2, 0)
            rr[rr_prev, :] = o_epilogue(tst[pl.ds(pl.multiple_of(i >> 10, 8), SUB), :], rp,
                                        ((nsub - 1) * SUB) // 8, rr[rr_prev, :], deps, 0)
            racc = ninf
            for j in range(1, nsub):
                t_cur = o_dot(r2, j)
                racc = o_epilogue(t_prev, r + (j - 1) * SUB, ((j - 1) * SUB) // 8, racc, deps,
                                  j * (SUB // STRIP))
                t_prev = t_cur
            tst[...] = t_prev
            rr[pl.ds(pl.multiple_of(i * 8, 8), 8), :] = racc

            if not first:
                @pl.when(i > 0)
                def _():
                    out_copy(i - 1).start()
            return c
        lax.fori_loop(0, NSEG, oproj, 0)
        rr_last = pl.ds((NSEG - 1) * 8, 8)
        rr[rr_last, :] = o_epilogue(tst[...], (NSEG - 1) * L + (nsub - 1) * SUB,
                                    ((nsub - 1) * SUB) // 8, rr[rr_last, :], {}, 0, nchain=4)
        if not first:
            out_copy(NSEG - 1).start()

        if first:
            w_copy(4).wait()
            w_copy(5).wait()
            for j in range(NG):
                wd_copy(j).wait()

        rv = rr[pl.ds(0, NSEG * 8), :]
        prow = lax.broadcasted_iota(jnp.int32, (NSEG * 8, 128), 0)
        plane = lax.broadcasted_iota(jnp.int32, (NSEG * 8, 128), 1)
        idx = (prow // 8) * L + plane * 8 + prow % 8

        bits = pltpu.bitcast(rv, jnp.int32)
        key = jnp.where(bits < 0, bits ^ 0x7FFFFFFF, bits)
        key = (key & ~(S - 1)) | ((S - 1 - idx) & (S - 1))
        max_all = lambda v: jnp.max(jnp.max(v, axis=0, keepdims=True), axis=1, keepdims=True)
        k1 = max_all(key)
        k2 = max_all(jnp.where(key == k1, jnp.iinfo(jnp.int32).min, key))
        i1 = S - 1 - (k1[0, 0] & (S - 1))
        i2 = S - 1 - (k2[0, 0] & (S - 1))
        g1 = pl.multiple_of((i1 // 16) * 16, 16)
        g2 = pl.multiple_of((i2 // 16) * 16, 16)
        xs = jnp.concatenate([_b16(xb[pl.ds(pl.multiple_of(g1 // 2, 8), 8), :]),
                              _b16(xb[pl.ds(pl.multiple_of(g2 // 2, 8), 8), :])], axis=0)
        gg = _nn(xs, wg[...])
        uu = _nn(xs, wu[...])
        hh = (gg * (1.0 / (1.0 + jnp.exp(-gg))) * uu).astype(BF16)
        yy = jnp.concatenate([_nn(hh, wd[j]) for j in range(NG)], axis=1)
        rsel = jnp.sum(xs.astype(F32) * wrf[pl.ds(0, 1), :], axis=1, keepdims=True)
        yy = yy * (1.0 / (1.0 + jnp.exp(-rsel)))
        riota = lax.broadcasted_iota(jnp.int32, (16, D), 0)
        if not first:
            for i in range(NSEG):
                out_copy(i).wait()
        for j, (ii, gr) in enumerate(((i1, g1), (i2, g2))):
            upd_ = yy[16 * j:16 * (j + 1)]
            if first:
                x2 = xw[pl.ds(gr, 16), :]
                x2 = jnp.where(riota == ii - gr, x2 + upd_, x2)
                xw[pl.ds(gr, 16), :] = x2
                xn[pl.ds(pl.multiple_of(gr // 2, 8), 8), :] = _p32(_ln(x2))
            else:
                x2 = xo[pl.ds(gr, 16), :].astype(F32)
                xo[pl.ds(gr, 16), :] = jnp.where(riota == ii - gr, x2 + upd_, x2).astype(BF16)
        if not first:
            patch = lambda gr, j: pltpu.make_async_copy(
                xo.at[pl.ds(gr, 16), :], out_hbm.at[0, pl.ds(gr, 16), :], sem_o.at[j])
            patch(g1, 0).start()

            @pl.when(g2 != g1)
            def _():
                patch(g2, 1).start()
            patch(g1, 0).wait()

            @pl.when(g2 != g1)
            def _():
                patch(g2, 1).wait()

    layer(True)
    layer(False)


@jax.jit
def pallas_interleave_layers__memory_aug_infini_attn__moe_arch_mod__prompt_kernel(
    A_x: jax.Array,
    A_wq: jax.Array,
    A_wk: jax.Array,
    A_wv: jax.Array,
    A_wo: jax.Array,
    A_beta: jax.Array,
    B_x: jax.Array,
    B_w_r: jax.Array,
    B_w_gate: jax.Array,
    B_w_up: jax.Array,
    B_w_down: jax.Array,
):
    del B_x
    any_spec = pl.BlockSpec(memory_space=pl.ANY)
    small = lambda shape: pl.BlockSpec(shape, lambda: (0,) * len(shape))
    vm = pltpu.VMEM
    scratch = [
        vm((S, D), BF16),
        vm((S, D), F32),
        vm((S // 2, D), U32),
        vm((3 * D, D), BF16),
        vm((D, D), BF16),
        vm((D // 2, D), U32),
        vm((D, 3 * D), BF16),
        vm((D, FF), BF16), vm((D, FF), BF16), vm((NG, FF, 128), BF16),
        vm((D // 2, S), U32), vm((D // 2, S), U32),
        vm((D // 2, S), U32), vm((D // 2, S), U32),
        vm((NG, S // 2, 128), U32), vm((NG, S // 2, 128), U32),
        vm((NG, S // 2, 128), U32),
        vm((S // 2, D), U32),
        vm((NG * NSEG * 8, 128), F32),
        vm((D, 128), F32),
        vm(((NSEG + 1) * 8, 128), F32),
        vm((SUB, D), F32),
        vm((8, D), F32),
        vm((L, QB), F32), vm((L, QB), F32),
    ] + [vm((4 * QB + 8, QB), F32) for _ in range(NSB)] + [
        pltpu.SemaphoreType.DMA((NSEG,)),
        pltpu.SemaphoreType.DMA((7,)),
        pltpu.SemaphoreType.DMA((NG,)),
        pltpu.SemaphoreType.DMA((NSEG,)),
    ]
    return pl.pallas_call(
        _kernel,
        out_shape=jax.ShapeDtypeStruct((1, S, D), BF16),
        in_specs=[any_spec, any_spec, any_spec, any_spec, any_spec,
                  small((H,)), small((D,)), any_spec, any_spec, any_spec],
        out_specs=any_spec,
        scratch_shapes=scratch,
        compiler_params=pltpu.CompilerParams(vmem_limit_bytes=110 * 1024 * 1024),
        name="infini_mod",
    )(A_x, A_wq, A_wk, A_wv, A_wo, A_beta, B_w_r, B_w_gate, B_w_up, B_w_down)
```

```python
import numpy as np
import jax
import jax.numpy as jnp
from jax import lax
import jax.experimental.pallas as pl
import jax.experimental.pallas.tpu as pltpu

F32 = jnp.float32
BF16 = jnp.bfloat16
U32 = jnp.uint32

S, D, H, NSEG, FF = 2048, 1024, 32, 4, 3584
DH = D // H
L = S // NSEG
NG = D // 128
HPG = 128 // DH
QB = 128
NSB = 16
SUB = 64
STRIP, NCHAIN = 16, 1
LN_CHAIN = 4
PV_LAG = 16
UPD_AT, ND_AT = 10, 30
LOG2E = float(np.log2(np.e))
SCALE = float(np.asarray(DH ** -0.5, dtype=np.float32).astype(jnp.bfloat16).astype(np.float32))
QSCALE = SCALE * LOG2E
MASKV = -1e9 * LOG2E


def _phi(t):
    return jnp.where(t > 0, t + 1.0, jnp.exp(t))


def _ln(x):
    m = jnp.sum(x, axis=-1, keepdims=True) * (1.0 / D)
    xc = x - m
    v = jnp.sum(xc * xc, axis=-1, keepdims=True) * (1.0 / D)
    return xc * lax.rsqrt(v + 1e-5)


def _nt(a, b):
    return lax.dot_general(a, b, (((1,), (1,)), ((), ())), preferred_element_type=F32)


def _nn(a, b):
    return jnp.dot(a, b, preferred_element_type=F32)


def _b16(x):
    return pltpu.bitcast(x, BF16)


def _p32(x):
    return pltpu.bitcast(x.astype(BF16), U32)


def _mul(i, n):
    return i if isinstance(i, int) else pl.multiple_of(i, n)


def _tree(op, xs):
    xs = list(xs)
    while len(xs) > 1:
        nx = [op(xs[i], xs[i + 1]) for i in range(0, len(xs) - 1, 2)]
        if len(xs) % 2:
            nx.append(xs[-1])
        xs = nx
    return xs[0]


def _vsplit(x):
    return [x[i * 8:(i + 1) * 8] for i in range(x.shape[0] // 8)]


class _Sub:
    def __init__(self, idx, s, qb, h):
        self.idx, self.s, self.qb, self.h = idx, s, qb, h
        self.n = qb + 1


def _attn_plan():
    subs = []
    for s in range(NSEG):
        for qb in range(L // QB):
            for h in range(HPG):
                subs.append(_Sub(len(subs), s, qb, h))
    tiles = [(u, kt) for u in subs for kt in range(u.n)]
    n = len(tiles)
    first = {}
    for i, (u, kt) in enumerate(tiles):
        if kt == 0:
            first[u.idx] = i
    pos = [first[u.idx] + u.n - 1 + PV_LAG for (u, kt) in tiles]
    deferred = set((u.s, u.qb) for i, (u, kt) in enumerate(tiles) if pos[i] >= n)
    for u in subs:
        nxt = subs[(u.idx + NSB) % len(subs)]
        wr = first[nxt.idx - nxt.h % 2] + (nxt.qb if nxt.h % 2 else 0) + (n if nxt.idx < u.idx else 0)
        last_read = max(first[v.idx] + v.n - 1 + PV_LAG for v in subs if (v.s, v.qb) == (u.s, u.qb))
        assert wr > max(last_read, n if (u.s, u.qb) in deferred else 0)
    now, prev = {}, {}
    for i, (u, kt) in enumerate(tiles):
        if (u.s, u.qb) in deferred:
            prev.setdefault(max(pos[i] - n, 0), []).append(i)
        else:
            now.setdefault(pos[i], []).append(i)
    return tiles, now, prev


_PLAN = _attn_plan()


class _Refs:
    pass


def _attn_body(R, g, gp, zsrc, do_qk=True):
    tiles, now, prev = _PLAN
    krow = lax.broadcasted_iota(jnp.int32, (QB, QB), 0)
    qcol = lax.broadcasted_iota(jnp.int32, (QB, QB), 1)
    bd = (krow // DH) == (qcol // DH)
    st, outs, mem = {}, {}, {}

    HB = QB // 2
    lo8 = lax.broadcasted_iota(jnp.int32, (8, QB), 1) < HB
    tri = jnp.where(krow[:HB] > qcol[:HB] % HB, MASKV, 0.0).astype(F32)
    swap = lambda v: pltpu.roll(v, HB, 1)

    def put(u, kt, x):
        buf = R.sb[u.idx % NSB]
        buf[pl.ds(kt * QB, QB), :] = x
        mx = _tree(jnp.maximum, _vsplit(x))
        key = ("m", u.idx)
        st[key] = jnp.maximum(st[key], mx) if key in st else mx
        if kt == (u.qb if (u.h % 2 == 0 or u.qb == 0) else u.qb - 1):
            buf[pl.ds(4 * QB, 8), :] = jnp.broadcast_to(jnp.max(st[key], axis=0, keepdims=True), (8, QB))

    def qk(i):
        u, kt = tiles[i]
        t0 = u.s * L
        q0 = t0 + u.qb * QB
        qrow = lambda ref, h: ref[pl.ds(pl.multiple_of(g * 64 + h * 16, 16), 16), pl.ds(q0, QB)]
        k0 = (t0 + kt * QB) // 2
        if kt < u.qb:
            parts = []
            if u.h > 0:
                parts.append(jnp.zeros((u.h * 16, QB), U32))
            parts.append(qrow(R.qT, u.h))
            if u.h < HPG - 1:
                parts.append(jnp.zeros(((HPG - 1 - u.h) * 16, QB), U32))
            put(u, kt, _nn(_b16(R.kk[g, pl.ds(k0, QB // 2), :]), _b16(jnp.concatenate(parts, axis=0))))
            return
        if u.h % 2 == 1:
            return
        lane16 = lax.broadcasted_iota(jnp.int32, (16, QB), 1) < HB
        z = jnp.uint32(0)

        def packed(rows, wa, wb):
            parts = []
            if u.h > 0:
                parts.append(jnp.zeros((u.h * 16, QB), U32))
            parts += [jnp.where(lane16, wa, z), jnp.where(lane16, z, wb)]
            if u.h < HPG - 2:
                parts.append(jnp.zeros(((HPG - 2 - u.h) * 16, QB), U32))
            return _nn(_b16(R.kk[g, pl.ds(k0, rows // 2), :]), _b16(jnp.concatenate(parts, axis=0)))

        X = packed(QB, qrow(R.qS, u.h), qrow(R.qT, u.h + 1))
        Y = packed(HB, qrow(R.qT, u.h), qrow(R.qS, u.h + 1)) + tri
        X0, X1 = _vsplit(X[:HB]), _vsplit(X[HB:] + tri)
        Y = _vsplit(Y)
        put(u, kt, jnp.concatenate([jnp.where(lo8, y, swap(x)) for x, y in zip(X0, Y)]
                                   + [jnp.where(lo8, MASKV, swap(x)) for x in X1], axis=0))
        put(tiles[i + 1 + u.qb][0], kt,
            jnp.concatenate([jnp.where(lo8, swap(y), x) for x, y in zip(X0, Y)]
                            + [jnp.where(lo8, MASKV, x) for x in X1], axis=0))

    def pv(i, gg, tag):
        u, kt = tiles[i]
        zero = 0 if isinstance(zsrc, int) else (zsrc + i) >> 12
        t0 = u.s * L
        q0 = t0 + u.qb * QB
        buf = R.sb[u.idx % NSB]
        km, kl, ko = ("mf", u.idx, tag), ("l", u.idx, tag), ("o", u.idx, tag)
        if kt == 0:
            st[km] = buf[pl.ds(pl.multiple_of(4 * QB + zero, 8), 8), :]
        m = st[km]
        x = buf[pl.ds(pl.multiple_of(kt * QB + zero, 8), QB), :]
        p = jnp.concatenate([jnp.exp2(v - m) for v in _vsplit(x)], axis=0)
        ls = _tree(jnp.add, _vsplit(p))
        st[kl] = ls if kt == 0 else st[kl] + ls
        vt = _b16(R.vT[pl.ds(pl.multiple_of(gg * 64 + u.h * 16, 16), 16), pl.ds(t0 + kt * QB, QB)])
        ot = _nn(vt, p.astype(BF16))
        st[ko] = ot if kt == 0 else st[ko] + ot
        if kt == u.qb:
            l = jnp.sum(st[kl], axis=0, keepdims=True)
            adot = st[ko] * (1.0 / l)
            gt = R.gs[pl.ds(pl.multiple_of(gg * 128 + u.h * DH, 8), 8), :]
            gt = jnp.concatenate([1.0 - gt] * 4, axis=0)
            o = gt * adot
            if u.s > 0:
                o = R.am[u.s % 2][pl.ds(pl.multiple_of(u.qb * QB + u.h * DH + zero, 8), DH), :] + o
            lst = outs.setdefault((u.s, u.qb, tag), [])
            lst.append(o)
            if len(lst) == HPG:
                oT = jnp.concatenate(lst, axis=0)
                R.ob[gg, pl.ds(q0 // 2, QB // 2), :] = _p32(oT.T)

    def upd(s):
        t0 = s * L
        lhs = _b16(R.vT[pl.ds(pl.multiple_of(g * 64, 64), 64), pl.ds(t0, L)])
        rhs = _b16(R.pk[g, pl.ds(t0 // 2, L // 2), :])
        u_ = jnp.where(bd, _nn(lhs, rhs), 0.0)
        zr = R.zs[pl.ds(pl.multiple_of(g * 8 * NSEG + s * 8, 8), 8), :]
        if s == 0:
            mem["M"], mem["z"] = u_, zr
        else:
            mem["M"], mem["z"] = mem["M"] + u_, mem["z"] + zr

    def nd(s, qb):
        t0 = s * L
        row16 = lax.broadcasted_iota(jnp.int32, (16, QB), 0)
        lane16h = lax.broadcasted_iota(jnp.int32, (16, QB), 1) // DH
        z16 = jnp.concatenate([mem["z"], mem["z"]], axis=0)
        zl = jnp.where(row16 == lane16h, z16, 0.0)
        lhs = jnp.concatenate([mem["M"], zl], axis=0).astype(BF16)
        r = _nn(lhs, _b16(R.pqT[pl.ds(pl.multiple_of(g * 64, 64), 64), pl.ds(t0 + qb * QB, QB)]))
        rden = 1.0 / (r[128:136] + 1e-6)
        for h in range(HPG):
            gt = (R.gs[pl.ds(pl.multiple_of(g * 128 + h * DH, 8), 8), :]
                  * jnp.broadcast_to(rden[h:h + 1], (8, QB)))
            R.am[s % 2][pl.ds(qb * QB + h * DH, DH), :] = (
                r[h * DH:(h + 1) * DH] * jnp.concatenate([gt] * 4, axis=0))

    extra = {}
    if do_qk:
        for s in range(NSEG - 1):
            extra.setdefault(40 * s + UPD_AT, []).append(("upd", s, 0))
            for qb in range(L // QB):
                extra.setdefault(40 * s + ND_AT, []).append(("nd", s + 1, qb))
    for i in range(len(tiles)):
        if do_qk:
            qk(i)
        for kind, s, qb in extra.get(i, []):
            upd(s) if kind == "upd" else nd(s, qb)
        for j in prev.get(i, []):
            pv(j, gp, 0)
        if do_qk:
            for j in now.get(i, []):
                pv(j, g, 1)


def _kernel(x_hbm, wq_hbm, wk_hbm, wv_hbm, wo_hbm, beta_ref, wr_ref, wg_hbm, wu_hbm, wd_hbm,
            out_hbm,
            xin, xw, xn, wall, wo, wo32, wT, wg, wu, wd,
            qT, qS, pqT, vT, kk, pk, ob, xb, zs, gs, rr, tst, wrf, am0, am1, *rest):
    sb = rest[:NSB]
    sem_x, sem_w, sem_d, sem_o = rest[NSB:]
    R = _Refs()
    R.qS = qS
    R.qT, R.pqT, R.vT, R.kk, R.pk, R.ob, R.zs, R.gs = qT, pqT, vT, kk, pk, ob, zs, gs
    R.am, R.sb = (am0, am1), sb
    xo = xin

    def x_copy(i):
        return pltpu.make_async_copy(x_hbm.at[0, pl.ds(i * L, L), :], xin.at[pl.ds(i * L, L), :], sem_x.at[i])

    def w_copy(j):
        half = lambda ref, c: ref.at[pl.ds(0, D), pl.ds(c * (D // 2), D // 2)]
        src = (half(wk_hbm, 0), wq_hbm, wv_hbm, wo_hbm, wg_hbm, wu_hbm, half(wk_hbm, 1))[j]
        dst = (half(wall, 0), wall.at[pl.ds(D, D), :], wall.at[pl.ds(2 * D, D), :], wo, wg, wu, half(wall, 1))[j]
        return pltpu.make_async_copy(src, dst, sem_w.at[j])

    def wd_copy(j):
        return pltpu.make_async_copy(wd_hbm.at[:, pl.ds(j * 128, 128)], wd.at[j], sem_d.at[j])

    def out_copy(i):
        return pltpu.make_async_copy(xo.at[pl.ds(i * L, L), :], out_hbm.at[0, pl.ds(i * L, L), :], sem_o.at[i])

    x_copy(0).start()
    w_copy(0).start()

    b = beta_ref[...].astype(F32).reshape(1, H)
    wrf[...] = jnp.broadcast_to(wr_ref[...].astype(F32).reshape(1, D), (8, D))
    sg = 1.0 / (1.0 + jnp.exp(-b))
    lane = lax.broadcasted_iota(jnp.int32, (1, H), 1)
    for h in range(H):
        gh = jnp.sum(jnp.where(lane == h, sg, 0.0), axis=1, keepdims=True)
        gs[pl.ds(h * DH, DH), :] = jnp.broadcast_to(gh, (DH, 128))
    for j in sorted(set(_PLAN[0][t][0].idx % NSB for ts in _PLAN[2].values() for t in ts)):
        sb[j][...] = jnp.zeros(sb[j].shape, F32)
    (am0, am1)[(NSEG - 1) % 2][...] = jnp.zeros(am1.shape, F32)
    tst[...] = jnp.zeros(tst.shape, F32)
    rr[...] = jnp.zeros(rr.shape, F32)

    def ln_rows(row0, nrows, nchain=0):
        deps = {}
        for k in range(nrows // 16):
            xv = xin[pl.ds(_mul(row0 + k * 16, 16), 16), :].astype(F32)
            m = jnp.sum(xv, axis=-1, keepdims=True) * (1.0 / D)
            if nchain and k >= nchain:
                m = m + deps[k % nchain]
            xc = xv - m
            rstd = lax.rsqrt(jnp.sum(xc * xc, axis=-1, keepdims=True) * (1.0 / D) + 1e-5)
            xn[pl.ds(_mul(row0 // 2 + k * 8, 8), 8), :] = _p32(xc * rstd)
            if nchain:
                deps[k % nchain] = jnp.minimum(jnp.abs(rstd), 0.0)

    def ln_first(blk, nchain):
        ln_rows(blk * L, L, nchain)

    order = ([("x", 1), ("w", 6), ("x", 2), ("x", 3)] + [("w", j) for j in range(1, 6)]
             + [("d", j) for j in range(NG)])

    def issue(i, c):
        for j, (kind, n) in enumerate(order):
            @pl.when(i == j)
            def _():
                {"x": x_copy, "w": w_copy, "d": wd_copy}[kind](n).start()
        return c
    lax.fori_loop(0, len(order), issue, 0)

    x_copy(0).wait()

    def ln0(i, c):
        ln_rows(i * (L // 4), L // 4)
        return c
    lax.fori_loop(0, 4, ln0, 0)

    def layer(first):

        def kproj_main(s, g0=0, g1=NG):
            r2 = _mul(s * (L // 2), L // 2)
            kf = _nn(_b16(xn[pl.ds(r2, L // 2), :]), wall[pl.ds(0, D), pl.ds(g0 * 128, (g1 - g0) * 128)])
            pf = _phi(kf)
            zrow = jnp.sum(pf, axis=0, keepdims=True)
            for g in range(g0, g1):
                sl = slice((g - g0) * 128, (g - g0 + 1) * 128)
                kk[g, pl.ds(r2, L // 2), :] = _p32(kf[:, sl])
                pk[g, pl.ds(r2, L // 2), :] = _p32(pf[:, sl])
                zs[pl.ds(_mul(g * 8 * NSEG + s * 8, 8), 8), :] = jnp.broadcast_to(zrow[:, sl], (8, 128))

        def transpose_w(j):
            for c_ in range(D // 128):
                rw = j * D + c_ * 128
                wT[:, pl.ds(rw, 128)] = wall[pl.ds(rw, 128), :].T

        def kproj_first(step, c):
            @pl.when(step == 0)
            def _():
                w_copy(0).wait()
                kproj_main(0, 0, NG // 2)

            @pl.when(step == 1)
            def _():
                x_copy(1).wait()
                w_copy(6).wait()
                ln_first(1, LN_CHAIN)
                kproj_main(0, NG // 2, NG)

            @pl.when(step == 2)
            def _():
                x_copy(2).wait()
                ln_first(2, LN_CHAIN)
                kproj_main(1)

            @pl.when(step == 3)
            def _():
                x_copy(3).wait()
                w_copy(1).wait()
                ln_first(3, LN_CHAIN)
                kproj_main(2)
                transpose_w(1)

            @pl.when(step == 4)
            def _():
                w_copy(2).wait()
                kproj_main(3)
                transpose_w(2)
            return c

        def qv_main(s):
            r = pl.multiple_of(s * L, L)
            r2 = pl.multiple_of(s * (L // 2), L // 2)
            xb_ = _b16(xn[pl.ds(r2, L // 2), :])
            qf = _nt(wT[:, pl.ds(D, D)], xb_)
            q16 = _p32(qf * QSCALE)
            qT[:, pl.ds(r, L)] = q16
            for c_ in range(L // QB):
                qS[:, pl.ds(r + c_ * QB, QB)] = pltpu.roll(q16[:, c_ * QB:(c_ + 1) * QB], QB // 2, 1)
            pqT[:, pl.ds(r, L)] = _p32(_phi(qf))
            vf = _nt(wT[:, pl.ds(2 * D, D)], xb_)
            vT[:, pl.ds(r, L)] = _p32(vf)

        def qv_first(s, c):
            wo32[pl.ds(pl.multiple_of(s * (D // 8), D // 8), D // 8), :] = pltpu.bitcast(
                wo[pl.ds(pl.multiple_of(s * (D // 4), D // 4), D // 4), :], U32)
            qv_main(s)
            return c

        def kqv(s, c):
            kproj_main(s)
            qv_main(s)
            return c

        if first:
            lax.fori_loop(0, 5, kproj_first, 0)
            w_copy(3).wait()
            lax.fori_loop(0, NSEG, qv_first, 0)
        else:
            lax.fori_loop(0, NSEG, kqv, 0)

        def attn(g, c):
            _attn_body(R, g, jnp.maximum(g - 1, 0), g)
            return c
        lax.fori_loop(0, NG, attn, 0)
        _attn_body(R, NG - 1, NG - 1, 0, do_qk=False)

        def o_dot(r2, j):
            lhs = jnp.concatenate(
                [_b16(ob[g, pl.ds(r2 + j * SUB // 2, SUB // 2), :]) for g in range(NG)], axis=1)
            return _nn(lhs, _b16(wo32[...]))

        def o_epilogue(t, r0, lane0, racc, deps, cid0, nchain=NCHAIN):
            wr = wrf[pl.ds(0, 1), :]
            lane_i = lax.broadcasted_iota(jnp.int32, (8, 128), 1)
            for k in range(SUB // STRIP):
                rows = pl.ds(r0 + k * STRIP, STRIP)
                rows2 = pl.ds(_mul(r0 // 2 + k * (STRIP // 2), STRIP // 2), STRIP // 2)
                xres = xin[rows, :].astype(F32) if first else xw[rows, :]
                x1 = xres + t[k * STRIP:(k + 1) * STRIP]
                m = jnp.sum(x1, axis=-1, keepdims=True) * (1.0 / D)
                cid = (cid0 + k) % nchain
                if deps.get(cid) is not None:
                    m = m + deps[cid]
                xc = x1 - m
                v = jnp.sum(xc * xc, axis=-1, keepdims=True) * (1.0 / D)
                rstd = lax.rsqrt(v + 1e-5)
                xl = xc * rstd
                rs = jnp.sum(xl * wr, axis=1, keepdims=True)
                for q in range(STRIP // 8):
                    racc = jnp.where(lane_i == lane0 + (k * STRIP) // 8 + q,
                                     jnp.broadcast_to(rs[q * 8:(q + 1) * 8], (8, 128)), racc)
                xb[rows2, :] = _p32(xl)
                if first:
                    xw[rows, :] = x1 + xl
                    c2 = 1.0 + rstd
                    s2 = c2 * lax.rsqrt(v * c2 * c2 + 1e-5)
                    xn[rows2, :] = _p32(xc * s2)
                    deps[cid] = jnp.minimum(jnp.abs(s2), 0.0)
                else:
                    xo[rows, :] = (x1 + xl).astype(BF16)
                    deps[cid] = jnp.minimum(jnp.abs(rstd), 0.0)
            return racc

        nsub = L // SUB
        ninf = jnp.full((8, 128), -jnp.inf, F32)

        def oproj(i, c):
            r = pl.multiple_of(i * L, L)
            r2 = pl.multiple_of(i * (L // 2), L // 2)
            ip = jnp.where(i == 0, NSEG - 1, i - 1)
            rp = pl.multiple_of(ip * L + (nsub - 1) * SUB, SUB)
            rr_prev = pl.ds(pl.multiple_of(jnp.where(i == 0, NSEG, i - 1) * 8, 8), 8)
            deps = {}
            t_prev = o_dot(r2, 0)
            rr[rr_prev, :] = o_epilogue(tst[pl.ds(pl.multiple_of(i >> 10, 8), SUB), :], rp,
                                        ((nsub - 1) * SUB) // 8, rr[rr_prev, :], deps, 0)
            racc = ninf
            for j in range(1, nsub):
                t_cur = o_dot(r2, j)
                racc = o_epilogue(t_prev, r + (j - 1) * SUB, ((j - 1) * SUB) // 8, racc, deps,
                                  j * (SUB // STRIP))
                t_prev = t_cur
            tst[...] = t_prev
            rr[pl.ds(pl.multiple_of(i * 8, 8), 8), :] = racc

            if not first:
                @pl.when(i > 0)
                def _():
                    out_copy(i - 1).start()
            return c
        lax.fori_loop(0, NSEG, oproj, 0)
        rr_last = pl.ds((NSEG - 1) * 8, 8)
        rr[rr_last, :] = o_epilogue(tst[...], (NSEG - 1) * L + (nsub - 1) * SUB,
                                    ((nsub - 1) * SUB) // 8, rr[rr_last, :], {}, 0, nchain=4)
        if not first:
            out_copy(NSEG - 1).start()

        if first:
            w_copy(4).wait()
            w_copy(5).wait()
            for j in range(NG):
                wd_copy(j).wait()

        rv = rr[pl.ds(0, NSEG * 8), :]
        prow = lax.broadcasted_iota(jnp.int32, (NSEG * 8, 128), 0)
        plane = lax.broadcasted_iota(jnp.int32, (NSEG * 8, 128), 1)
        idx = (prow // 8) * L + plane * 8 + prow % 8

        bits = pltpu.bitcast(rv, jnp.int32)
        key = jnp.where(bits < 0, bits ^ 0x7FFFFFFF, bits)
        key = (key & ~(S - 1)) | ((S - 1 - idx) & (S - 1))
        max_all = lambda v: jnp.max(jnp.max(v, axis=0, keepdims=True), axis=1, keepdims=True)
        k1 = max_all(key)
        k2 = max_all(jnp.where(key == k1, jnp.iinfo(jnp.int32).min, key))
        i1 = S - 1 - (k1[0, 0] & (S - 1))
        i2 = S - 1 - (k2[0, 0] & (S - 1))
        g1 = pl.multiple_of((i1 // 16) * 16, 16)
        g2 = pl.multiple_of((i2 // 16) * 16, 16)
        xs = jnp.concatenate([_b16(xb[pl.ds(pl.multiple_of(g1 // 2, 8), 8), :]),
                              _b16(xb[pl.ds(pl.multiple_of(g2 // 2, 8), 8), :])], axis=0)
        gg = _nn(xs, wg[...])
        uu = _nn(xs, wu[...])
        hh = (gg * (1.0 / (1.0 + jnp.exp(-gg))) * uu).astype(BF16)
        yy = jnp.concatenate([_nn(hh, wd[j]) for j in range(NG)], axis=1)
        rsel = jnp.sum(xs.astype(F32) * wrf[pl.ds(0, 1), :], axis=1, keepdims=True)
        yy = yy * (1.0 / (1.0 + jnp.exp(-rsel)))
        riota = lax.broadcasted_iota(jnp.int32, (16, D), 0)
        if not first:
            for i in range(NSEG):
                out_copy(i).wait()
        for j, (ii, gr) in enumerate(((i1, g1), (i2, g2))):
            upd_ = yy[16 * j:16 * (j + 1)]
            if first:
                x2 = xw[pl.ds(gr, 16), :]
                x2 = jnp.where(riota == ii - gr, x2 + upd_, x2)
                xw[pl.ds(gr, 16), :] = x2
                xn[pl.ds(pl.multiple_of(gr // 2, 8), 8), :] = _p32(_ln(x2))
            else:
                x2 = xo[pl.ds(gr, 16), :].astype(F32)
                xo[pl.ds(gr, 16), :] = jnp.where(riota == ii - gr, x2 + upd_, x2).astype(BF16)
        if not first:
            patch = lambda gr, j: pltpu.make_async_copy(
                xo.at[pl.ds(gr, 16), :], out_hbm.at[0, pl.ds(gr, 16), :], sem_o.at[j])
            patch(g1, 0).start()

            @pl.when(g2 != g1)
            def _():
                patch(g2, 1).start()
            patch(g1, 0).wait()

            @pl.when(g2 != g1)
            def _():
                patch(g2, 1).wait()

    layer(True)
    layer(False)


@jax.jit
def pallas_interleave_layers__memory_aug_infini_attn__moe_arch_mod__prompt_kernel(
    A_x: jax.Array,
    A_wq: jax.Array,
    A_wk: jax.Array,
    A_wv: jax.Array,
    A_wo: jax.Array,
    A_beta: jax.Array,
    B_x: jax.Array,
    B_w_r: jax.Array,
    B_w_gate: jax.Array,
    B_w_up: jax.Array,
    B_w_down: jax.Array,
):
    del B_x
    any_spec = pl.BlockSpec(memory_space=pl.ANY)
    small = lambda shape: pl.BlockSpec(shape, lambda: (0,) * len(shape))
    vm = pltpu.VMEM
    scratch = [
        vm((S, D), BF16),
        vm((S, D), F32),
        vm((S // 2, D), U32),
        vm((3 * D, D), BF16),
        vm((D, D), BF16),
        vm((D // 2, D), U32),
        vm((D, 3 * D), BF16),
        vm((D, FF), BF16), vm((D, FF), BF16), vm((NG, FF, 128), BF16),
        vm((D // 2, S), U32), vm((D // 2, S), U32),
        vm((D // 2, S), U32), vm((D // 2, S), U32),
        vm((NG, S // 2, 128), U32), vm((NG, S // 2, 128), U32),
        vm((NG, S // 2, 128), U32),
        vm((S // 2, D), U32),
        vm((NG * NSEG * 8, 128), F32),
        vm((D, 128), F32),
        vm(((NSEG + 1) * 8, 128), F32),
        vm((SUB, D), F32),
        vm((8, D), F32),
        vm((L, QB), F32), vm((L, QB), F32),
    ] + [vm((4 * QB + 8, QB), F32) for _ in range(NSB)] + [
        pltpu.SemaphoreType.DMA((NSEG,)),
        pltpu.SemaphoreType.DMA((7,)),
        pltpu.SemaphoreType.DMA((NG,)),
        pltpu.SemaphoreType.DMA((NSEG,)),
    ]
    return pl.pallas_call(
        _kernel,
        out_shape=jax.ShapeDtypeStruct((1, S, D), BF16),
        in_specs=[any_spec, any_spec, any_spec, any_spec, any_spec,
                  small((H,)), small((D,)), any_spec, any_spec, any_spec],
        out_specs=any_spec,
        scratch_shapes=scratch,
        compiler_params=pltpu.CompilerParams(vmem_limit_bytes=110 * 1024 * 1024),
        name="infini_mod",
    )(A_x, A_wq, A_wk, A_wv, A_wo, A_beta, B_w_r, B_w_gate, B_w_up, B_w_down)
```

```python
import numpy as np
import jax
import jax.numpy as jnp
from jax import lax
import jax.experimental.pallas as pl
import jax.experimental.pallas.tpu as pltpu

F32 = jnp.float32
BF16 = jnp.bfloat16
U32 = jnp.uint32

S, D, H, NSEG, FF = 2048, 1024, 32, 4, 3584
DH = D // H
L = S // NSEG
NG = D // 128
HPG = 128 // DH
QB = 128
NSB = 16
SUB = 64
STRIP, NCHAIN = 16, 1
LN_CHAIN = 4
PV_LAG = 16
UPD_AT, ND_AT = 10, 30
LOG2E = float(np.log2(np.e))
SCALE = float(np.asarray(DH ** -0.5, dtype=np.float32).astype(jnp.bfloat16).astype(np.float32))
QSCALE = SCALE * LOG2E
MASKV = -1e9 * LOG2E


def _phi(t):
    return jnp.where(t > 0, t + 1.0, jnp.exp(t))


def _ln(x):
    m = jnp.sum(x, axis=-1, keepdims=True) * (1.0 / D)
    xc = x - m
    v = jnp.sum(xc * xc, axis=-1, keepdims=True) * (1.0 / D)
    return xc * lax.rsqrt(v + 1e-5)


def _nt(a, b):
    return lax.dot_general(a, b, (((1,), (1,)), ((), ())), preferred_element_type=F32)


def _nn(a, b):
    return jnp.dot(a, b, preferred_element_type=F32)


def _b16(x):
    return pltpu.bitcast(x, BF16)


def _p32(x):
    return pltpu.bitcast(x.astype(BF16), U32)


def _mul(i, n):
    return i if isinstance(i, int) else pl.multiple_of(i, n)


def _tree(op, xs):
    xs = list(xs)
    while len(xs) > 1:
        nx = [op(xs[i], xs[i + 1]) for i in range(0, len(xs) - 1, 2)]
        if len(xs) % 2:
            nx.append(xs[-1])
        xs = nx
    return xs[0]


def _vsplit(x):
    return [x[i * 8:(i + 1) * 8] for i in range(x.shape[0] // 8)]


class _Sub:
    def __init__(self, idx, s, qb, h):
        self.idx, self.s, self.qb, self.h = idx, s, qb, h
        self.n = qb + 1


def _attn_plan():
    subs = []
    for s in range(NSEG):
        for qb in range(L // QB):
            for h in range(HPG):
                subs.append(_Sub(len(subs), s, qb, h))
    tiles = [(u, kt) for u in subs for kt in range(u.n)]
    n = len(tiles)
    first = {}
    for i, (u, kt) in enumerate(tiles):
        if kt == 0:
            first[u.idx] = i
    pos = [first[u.idx] + u.n - 1 + PV_LAG for (u, kt) in tiles]
    deferred = set((u.s, u.qb) for i, (u, kt) in enumerate(tiles) if pos[i] >= n)
    for u in subs:
        nxt = subs[(u.idx + NSB) % len(subs)]
        wr = first[nxt.idx - nxt.h % 2] + (nxt.qb if nxt.h % 2 else 0) + (n if nxt.idx < u.idx else 0)
        last_read = max(first[v.idx] + v.n - 1 + PV_LAG for v in subs if (v.s, v.qb) == (u.s, u.qb))
        assert wr > max(last_read, n if (u.s, u.qb) in deferred else 0)
    now, prev = {}, {}
    for i, (u, kt) in enumerate(tiles):
        if (u.s, u.qb) in deferred:
            prev.setdefault(max(pos[i] - n, 0), []).append(i)
        else:
            now.setdefault(pos[i], []).append(i)
    return tiles, now, prev


_PLAN = _attn_plan()


class _Refs:
    pass


def _attn_body(R, g, gp, do_qk=True):
    tiles, now, prev = _PLAN
    krow = lax.broadcasted_iota(jnp.int32, (QB, QB), 0)
    qcol = lax.broadcasted_iota(jnp.int32, (QB, QB), 1)
    bd = (krow // DH) == (qcol // DH)
    st, outs, mem = {}, {}, {}

    HB = QB // 2
    lo8 = lax.broadcasted_iota(jnp.int32, (8, QB), 1) < HB
    tri = jnp.where(krow[:HB] > qcol[:HB] % HB, MASKV, 0.0).astype(F32)
    swap = lambda v: pltpu.roll(v, HB, 1)

    def put(u, kt, x):
        buf = R.sb[u.idx % NSB]
        buf[pl.ds(kt * QB, QB), :] = x
        mx = _tree(jnp.maximum, _vsplit(x))
        key = ("m", u.idx)
        st[key] = jnp.maximum(st[key], mx) if key in st else mx
        if kt == (u.qb if (u.h % 2 == 0 or u.qb == 0) else u.qb - 1):
            buf[pl.ds(4 * QB, 8), :] = jnp.broadcast_to(jnp.max(st[key], axis=0, keepdims=True), (8, QB))

    def qk(i):
        u, kt = tiles[i]
        t0 = u.s * L
        q0 = t0 + u.qb * QB
        qrow = lambda ref, h: ref[pl.ds(pl.multiple_of(g * 64 + h * 16, 16), 16), pl.ds(q0, QB)]
        k0 = (t0 + kt * QB) // 2
        if kt < u.qb:
            parts = []
            if u.h > 0:
                parts.append(jnp.zeros((u.h * 16, QB), U32))
            parts.append(qrow(R.qT, u.h))
            if u.h < HPG - 1:
                parts.append(jnp.zeros(((HPG - 1 - u.h) * 16, QB), U32))
            put(u, kt, _nn(_b16(R.kk[g, pl.ds(k0, QB // 2), :]), _b16(jnp.concatenate(parts, axis=0))))
            return
        if u.h % 2 == 1:
            return
        lane16 = lax.broadcasted_iota(jnp.int32, (16, QB), 1) < HB
        z = jnp.uint32(0)

        def packed(rows, wa, wb):
            parts = []
            if u.h > 0:
                parts.append(jnp.zeros((u.h * 16, QB), U32))
            parts += [jnp.where(lane16, wa, z), jnp.where(lane16, z, wb)]
            if u.h < HPG - 2:
                parts.append(jnp.zeros(((HPG - 2 - u.h) * 16, QB), U32))
            return _nn(_b16(R.kk[g, pl.ds(k0, rows // 2), :]), _b16(jnp.concatenate(parts, axis=0)))

        X = packed(QB, qrow(R.qS, u.h), qrow(R.qT, u.h + 1))
        Y = packed(HB, qrow(R.qT, u.h), qrow(R.qS, u.h + 1)) + tri
        X0, X1 = _vsplit(X[:HB]), _vsplit(X[HB:] + tri)
        Y = _vsplit(Y)
        put(u, kt, jnp.concatenate([jnp.where(lo8, y, swap(x)) for x, y in zip(X0, Y)]
                                   + [jnp.where(lo8, MASKV, swap(x)) for x in X1], axis=0))
        put(tiles[i + 1 + u.qb][0], kt,
            jnp.concatenate([jnp.where(lo8, swap(y), x) for x, y in zip(X0, Y)]
                            + [jnp.where(lo8, MASKV, x) for x in X1], axis=0))

    def pv(i, gg, tag):
        u, kt = tiles[i]
        t0 = u.s * L
        q0 = t0 + u.qb * QB
        buf = R.sb[u.idx % NSB]
        km, kl, ko = ("mf", u.idx, tag), ("l", u.idx, tag), ("o", u.idx, tag)
        if kt == 0:
            st[km] = buf[pl.ds(4 * QB, 8), :]
        m = st[km]
        x = buf[pl.ds(kt * QB, QB), :]
        p = jnp.concatenate([jnp.exp2(v - m) for v in _vsplit(x)], axis=0)
        ls = _tree(jnp.add, _vsplit(p))
        st[kl] = ls if kt == 0 else st[kl] + ls
        vt = _b16(R.vT[pl.ds(pl.multiple_of(gg * 64 + u.h * 16, 16), 16), pl.ds(t0 + kt * QB, QB)])
        ot = _nn(vt, p.astype(BF16))
        st[ko] = ot if kt == 0 else st[ko] + ot
        if kt == u.qb:
            l = jnp.sum(st[kl], axis=0, keepdims=True)
            adot = st[ko] * (1.0 / l)
            gt = R.gs[pl.ds(pl.multiple_of(gg * 128 + u.h * DH, 8), 8), :]
            gt = jnp.concatenate([1.0 - gt] * 4, axis=0)
            o = gt * adot
            if u.s > 0:
                o = R.am[u.s % 2][pl.ds(u.qb * QB + u.h * DH, DH), :] + o
            lst = outs.setdefault((u.s, u.qb, tag), [])
            lst.append(o)
            if len(lst) == HPG:
                oT = jnp.concatenate(lst, axis=0)
                R.ob[gg, pl.ds(q0 // 2, QB // 2), :] = _p32(oT.T)

    def upd(s):
        t0 = s * L
        lhs = _b16(R.vT[pl.ds(pl.multiple_of(g * 64, 64), 64), pl.ds(t0, L)])
        rhs = _b16(R.pk[g, pl.ds(t0 // 2, L // 2), :])
        u_ = jnp.where(bd, _nn(lhs, rhs), 0.0)
        zr = R.zs[pl.ds(pl.multiple_of(g * 8 * NSEG + s * 8, 8), 8), :]
        if s == 0:
            mem["M"], mem["z"] = u_, zr
        else:
            mem["M"], mem["z"] = mem["M"] + u_, mem["z"] + zr

    def nd(s, qb):
        t0 = s * L
        row16 = lax.broadcasted_iota(jnp.int32, (16, QB), 0)
        lane16h = lax.broadcasted_iota(jnp.int32, (16, QB), 1) // DH
        z16 = jnp.concatenate([mem["z"], mem["z"]], axis=0)
        zl = jnp.where(row16 == lane16h, z16, 0.0)
        lhs = jnp.concatenate([mem["M"], zl], axis=0).astype(BF16)
        r = _nn(lhs, _b16(R.pqT[pl.ds(pl.multiple_of(g * 64, 64), 64), pl.ds(t0 + qb * QB, QB)]))
        rden = 1.0 / (r[128:136] + 1e-6)
        for h in range(HPG):
            gt = (R.gs[pl.ds(pl.multiple_of(g * 128 + h * DH, 8), 8), :]
                  * jnp.broadcast_to(rden[h:h + 1], (8, QB)))
            R.am[s % 2][pl.ds(qb * QB + h * DH, DH), :] = (
                r[h * DH:(h + 1) * DH] * jnp.concatenate([gt] * 4, axis=0))

    extra = {}
    if do_qk:
        for s in range(NSEG - 1):
            extra.setdefault(40 * s + UPD_AT, []).append(("upd", s, 0))
            for qb in range(L // QB):
                extra.setdefault(40 * s + ND_AT, []).append(("nd", s + 1, qb))
    for i in range(len(tiles)):
        if do_qk:
            qk(i)
        for kind, s, qb in extra.get(i, []):
            upd(s) if kind == "upd" else nd(s, qb)
        for j in prev.get(i, []):
            pv(j, gp, 0)
        if do_qk:
            for j in now.get(i, []):
                pv(j, g, 1)


def _kernel(x_hbm, wq_hbm, wk_hbm, wv_hbm, wo_hbm, beta_ref, wr_ref, wg_hbm, wu_hbm, wd_hbm,
            out_hbm,
            xin, xw, xn, wall, wo, wo32, wT, wg, wu, wd,
            qT, qS, pqT, vT, kk, pk, ob, xb, zs, gs, rr, tst, wrf, am0, am1, *rest):
    sb = rest[:NSB]
    sem_x, sem_w, sem_d, sem_o = rest[NSB:]
    R = _Refs()
    R.qS = qS
    R.qT, R.pqT, R.vT, R.kk, R.pk, R.ob, R.zs, R.gs = qT, pqT, vT, kk, pk, ob, zs, gs
    R.am, R.sb = (am0, am1), sb
    xo = xin

    def x_copy(i):
        return pltpu.make_async_copy(x_hbm.at[0, pl.ds(i * L, L), :], xin.at[pl.ds(i * L, L), :], sem_x.at[i])

    def w_copy(j):
        half = lambda ref, c: ref.at[pl.ds(0, D), pl.ds(c * (D // 2), D // 2)]
        src = (half(wk_hbm, 0), wq_hbm, wv_hbm, wo_hbm, wg_hbm, wu_hbm, half(wk_hbm, 1))[j]
        dst = (half(wall, 0), wall.at[pl.ds(D, D), :], wall.at[pl.ds(2 * D, D), :], wo, wg, wu, half(wall, 1))[j]
        return pltpu.make_async_copy(src, dst, sem_w.at[j])

    def wd_copy(j):
        return pltpu.make_async_copy(wd_hbm.at[:, pl.ds(j * 128, 128)], wd.at[j], sem_d.at[j])

    def out_copy(i):
        return pltpu.make_async_copy(xo.at[pl.ds(i * L, L), :], out_hbm.at[0, pl.ds(i * L, L), :], sem_o.at[i])

    x_copy(0).start()
    w_copy(0).start()

    b = beta_ref[...].astype(F32).reshape(1, H)
    wrf[...] = jnp.broadcast_to(wr_ref[...].astype(F32).reshape(1, D), (8, D))
    sg = 1.0 / (1.0 + jnp.exp(-b))
    lane = lax.broadcasted_iota(jnp.int32, (1, H), 1)
    for h in range(H):
        gh = jnp.sum(jnp.where(lane == h, sg, 0.0), axis=1, keepdims=True)
        gs[pl.ds(h * DH, DH), :] = jnp.broadcast_to(gh, (DH, 128))
    for j in sorted(set(_PLAN[0][t][0].idx % NSB for ts in _PLAN[2].values() for t in ts)):
        sb[j][...] = jnp.zeros(sb[j].shape, F32)
    (am0, am1)[(NSEG - 1) % 2][...] = jnp.zeros(am1.shape, F32)
    tst[...] = jnp.zeros(tst.shape, F32)
    rr[...] = jnp.zeros(rr.shape, F32)

    def ln_rows(row0, nrows, nchain=0):
        deps = {}
        for k in range(nrows // 16):
            xv = xin[pl.ds(_mul(row0 + k * 16, 16), 16), :].astype(F32)
            m = jnp.sum(xv, axis=-1, keepdims=True) * (1.0 / D)
            if nchain and k >= nchain:
                m = m + deps[k % nchain]
            xc = xv - m
            rstd = lax.rsqrt(jnp.sum(xc * xc, axis=-1, keepdims=True) * (1.0 / D) + 1e-5)
            xn[pl.ds(_mul(row0 // 2 + k * 8, 8), 8), :] = _p32(xc * rstd)
            if nchain:
                deps[k % nchain] = jnp.minimum(jnp.abs(rstd), 0.0)

    def ln_first(blk, nchain):
        ln_rows(blk * L, L, nchain)

    order = ([("x", 1), ("w", 6), ("x", 2), ("x", 3)] + [("w", j) for j in range(1, 6)]
             + [("d", j) for j in range(NG)])

    def issue(i, c):
        for j, (kind, n) in enumerate(order):
            @pl.when(i == j)
            def _():
                {"x": x_copy, "w": w_copy, "d": wd_copy}[kind](n).start()
        return c
    lax.fori_loop(0, len(order), issue, 0)

    x_copy(0).wait()

    def ln0(i, c):
        ln_rows(i * (L // 4), L // 4)
        return c
    lax.fori_loop(0, 4, ln0, 0)

    def layer(first):

        def kproj_main(s, g0=0, g1=NG):
            r2 = _mul(s * (L // 2), L // 2)
            kf = _nn(_b16(xn[pl.ds(r2, L // 2), :]), wall[pl.ds(0, D), pl.ds(g0 * 128, (g1 - g0) * 128)])
            pf = _phi(kf)
            zrow = jnp.sum(pf, axis=0, keepdims=True)
            for g in range(g0, g1):
                sl = slice((g - g0) * 128, (g - g0 + 1) * 128)
                kk[g, pl.ds(r2, L // 2), :] = _p32(kf[:, sl])
                pk[g, pl.ds(r2, L // 2), :] = _p32(pf[:, sl])
                zs[pl.ds(_mul(g * 8 * NSEG + s * 8, 8), 8), :] = jnp.broadcast_to(zrow[:, sl], (8, 128))

        def transpose_w(j):
            for c_ in range(D // 128):
                rw = j * D + c_ * 128
                wT[:, pl.ds(rw, 128)] = wall[pl.ds(rw, 128), :].T

        def kproj_first(step, c):
            @pl.when(step == 0)
            def _():
                w_copy(0).wait()
                kproj_main(0, 0, NG // 2)

            @pl.when(step == 1)
            def _():
                x_copy(1).wait()
                w_copy(6).wait()
                ln_first(1, LN_CHAIN)
                kproj_main(0, NG // 2, NG)

            @pl.when(step == 2)
            def _():
                x_copy(2).wait()
                ln_first(2, LN_CHAIN)
                kproj_main(1)

            @pl.when(step == 3)
            def _():
                x_copy(3).wait()
                w_copy(1).wait()
                ln_first(3, LN_CHAIN)
                kproj_main(2)
                transpose_w(1)

            @pl.when(step == 4)
            def _():
                w_copy(2).wait()
                kproj_main(3)
                transpose_w(2)
            return c

        def qv_main(s):
            r = pl.multiple_of(s * L, L)
            r2 = pl.multiple_of(s * (L // 2), L // 2)
            xb_ = _b16(xn[pl.ds(r2, L // 2), :])
            qf = _nt(wT[:, pl.ds(D, D)], xb_)
            q16 = _p32(qf * QSCALE)
            qT[:, pl.ds(r, L)] = q16
            for c_ in range(L // QB):
                qS[:, pl.ds(r + c_ * QB, QB)] = pltpu.roll(q16[:, c_ * QB:(c_ + 1) * QB], QB // 2, 1)
            pqT[:, pl.ds(r, L)] = _p32(_phi(qf))
            vf = _nt(wT[:, pl.ds(2 * D, D)], xb_)
            vT[:, pl.ds(r, L)] = _p32(vf)

        def qv_first(s, c):
            wo32[pl.ds(pl.multiple_of(s * (D // 8), D // 8), D // 8), :] = pltpu.bitcast(
                wo[pl.ds(pl.multiple_of(s * (D // 4), D // 4), D // 4), :], U32)
            qv_main(s)
            return c

        def kqv(s, c):
            kproj_main(s)
            qv_main(s)
            return c

        if first:
            lax.fori_loop(0, 5, kproj_first, 0)
            w_copy(3).wait()
            lax.fori_loop(0, NSEG, qv_first, 0)
        else:
            lax.fori_loop(0, NSEG, kqv, 0)

        def attn(g, c):
            _attn_body(R, g, jnp.maximum(g - 1, 0))
            return c
        lax.fori_loop(0, NG, attn, 0)
        _attn_body(R, NG - 1, NG - 1, do_qk=False)

        def o_dot(r2, j):
            lhs = jnp.concatenate(
                [_b16(ob[g, pl.ds(r2 + j * SUB // 2, SUB // 2), :]) for g in range(NG)], axis=1)
            return _nn(lhs, _b16(wo32[...]))

        def o_epilogue(t, r0, lane0, racc, deps, cid0, nchain=NCHAIN):
            wr = wrf[pl.ds(0, 1), :]
            lane_i = lax.broadcasted_iota(jnp.int32, (8, 128), 1)
            for k in range(SUB // STRIP):
                rows = pl.ds(r0 + k * STRIP, STRIP)
                rows2 = pl.ds(_mul(r0 // 2 + k * (STRIP // 2), STRIP // 2), STRIP // 2)
                xres = xin[rows, :].astype(F32) if first else xw[rows, :]
                x1 = xres + t[k * STRIP:(k + 1) * STRIP]
                m = jnp.sum(x1, axis=-1, keepdims=True) * (1.0 / D)
                cid = (cid0 + k) % nchain
                if deps.get(cid) is not None:
                    m = m + deps[cid]
                xc = x1 - m
                v = jnp.sum(xc * xc, axis=-1, keepdims=True) * (1.0 / D)
                rstd = lax.rsqrt(v + 1e-5)
                xl = xc * rstd
                rs = jnp.sum(xl * wr, axis=1, keepdims=True)
                for q in range(STRIP // 8):
                    racc = jnp.where(lane_i == lane0 + (k * STRIP) // 8 + q,
                                     jnp.broadcast_to(rs[q * 8:(q + 1) * 8], (8, 128)), racc)
                xb[rows2, :] = _p32(xl)
                if first:
                    xw[rows, :] = x1 + xl
                    c2 = 1.0 + rstd
                    s2 = c2 * lax.rsqrt(v * c2 * c2 + 1e-5)
                    xn[rows2, :] = _p32(xc * s2)
                    deps[cid] = jnp.minimum(jnp.abs(s2), 0.0)
                else:
                    xo[rows, :] = (x1 + xl).astype(BF16)
                    deps[cid] = jnp.minimum(jnp.abs(rstd), 0.0)
            return racc

        nsub = L // SUB
        ninf = jnp.full((8, 128), -jnp.inf, F32)

        def oproj(i, c):
            r = pl.multiple_of(i * L, L)
            r2 = pl.multiple_of(i * (L // 2), L // 2)
            ip = jnp.where(i == 0, NSEG - 1, i - 1)
            rp = pl.multiple_of(ip * L + (nsub - 1) * SUB, SUB)
            rr_prev = pl.ds(pl.multiple_of(jnp.where(i == 0, NSEG, i - 1) * 8, 8), 8)
            deps = {}
            t_prev = o_dot(r2, 0)
            rr[rr_prev, :] = o_epilogue(tst[...], rp,
                                        ((nsub - 1) * SUB) // 8, rr[rr_prev, :], deps, 0)
            racc = ninf
            for j in range(1, nsub):
                t_cur = o_dot(r2, j)
                racc = o_epilogue(t_prev, r + (j - 1) * SUB, ((j - 1) * SUB) // 8, racc, deps,
                                  j * (SUB // STRIP))
                t_prev = t_cur
            tst[...] = t_prev
            rr[pl.ds(pl.multiple_of(i * 8, 8), 8), :] = racc

            if not first:
                @pl.when(i > 0)
                def _():
                    out_copy(i - 1).start()
            return c
        lax.fori_loop(0, NSEG, oproj, 0)
        rr_last = pl.ds((NSEG - 1) * 8, 8)
        rr[rr_last, :] = o_epilogue(tst[...], (NSEG - 1) * L + (nsub - 1) * SUB,
                                    ((nsub - 1) * SUB) // 8, rr[rr_last, :], {}, 0, nchain=4)
        if not first:
            out_copy(NSEG - 1).start()

        if first:
            w_copy(4).wait()
            w_copy(5).wait()
            for j in range(NG):
                wd_copy(j).wait()

        rv = rr[pl.ds(0, NSEG * 8), :]
        prow = lax.broadcasted_iota(jnp.int32, (NSEG * 8, 128), 0)
        plane = lax.broadcasted_iota(jnp.int32, (NSEG * 8, 128), 1)
        idx = (prow // 8) * L + plane * 8 + prow % 8

        bits = pltpu.bitcast(rv, jnp.int32)
        key = jnp.where(bits < 0, bits ^ 0x7FFFFFFF, bits)
        key = (key & ~(S - 1)) | ((S - 1 - idx) & (S - 1))
        max_all = lambda v: jnp.max(jnp.max(v, axis=0, keepdims=True), axis=1, keepdims=True)
        k1 = max_all(key)
        k2 = max_all(jnp.where(key == k1, jnp.iinfo(jnp.int32).min, key))
        i1 = S - 1 - (k1[0, 0] & (S - 1))
        i2 = S - 1 - (k2[0, 0] & (S - 1))
        g1 = pl.multiple_of((i1 // 16) * 16, 16)
        g2 = pl.multiple_of((i2 // 16) * 16, 16)
        xs = jnp.concatenate([_b16(xb[pl.ds(pl.multiple_of(g1 // 2, 8), 8), :]),
                              _b16(xb[pl.ds(pl.multiple_of(g2 // 2, 8), 8), :])], axis=0)
        gg = _nn(xs, wg[...])
        uu = _nn(xs, wu[...])
        hh = (gg * (1.0 / (1.0 + jnp.exp(-gg))) * uu).astype(BF16)
        yy = jnp.concatenate([_nn(hh, wd[j]) for j in range(NG)], axis=1)
        rsel = jnp.sum(xs.astype(F32) * wrf[pl.ds(0, 1), :], axis=1, keepdims=True)
        yy = yy * (1.0 / (1.0 + jnp.exp(-rsel)))
        riota = lax.broadcasted_iota(jnp.int32, (16, D), 0)
        if not first:
            for i in range(NSEG):
                out_copy(i).wait()
        for j, (ii, gr) in enumerate(((i1, g1), (i2, g2))):
            upd_ = yy[16 * j:16 * (j + 1)]
            if first:
                x2 = xw[pl.ds(gr, 16), :]
                x2 = jnp.where(riota == ii - gr, x2 + upd_, x2)
                xw[pl.ds(gr, 16), :] = x2
                xn[pl.ds(pl.multiple_of(gr // 2, 8), 8), :] = _p32(_ln(x2))
            else:
                x2 = xo[pl.ds(gr, 16), :].astype(F32)
                xo[pl.ds(gr, 16), :] = jnp.where(riota == ii - gr, x2 + upd_, x2).astype(BF16)
        if not first:
            patch = lambda gr, j: pltpu.make_async_copy(
                xo.at[pl.ds(gr, 16), :], out_hbm.at[0, pl.ds(gr, 16), :], sem_o.at[j])
            patch(g1, 0).start()

            @pl.when(g2 != g1)
            def _():
                patch(g2, 1).start()
            patch(g1, 0).wait()

            @pl.when(g2 != g1)
            def _():
                patch(g2, 1).wait()

    layer(True)
    layer(False)


@jax.jit
def pallas_interleave_layers__memory_aug_infini_attn__moe_arch_mod__prompt_kernel(
    A_x: jax.Array,
    A_wq: jax.Array,
    A_wk: jax.Array,
    A_wv: jax.Array,
    A_wo: jax.Array,
    A_beta: jax.Array,
    B_x: jax.Array,
    B_w_r: jax.Array,
    B_w_gate: jax.Array,
    B_w_up: jax.Array,
    B_w_down: jax.Array,
):
    del B_x
    any_spec = pl.BlockSpec(memory_space=pl.ANY)
    small = lambda shape: pl.BlockSpec(shape, lambda: (0,) * len(shape))
    vm = pltpu.VMEM
    scratch = [
        vm((S, D), BF16),
        vm((S, D), F32),
        vm((S // 2, D), U32),
        vm((3 * D, D), BF16),
        vm((D, D), BF16),
        vm((D // 2, D), U32),
        vm((D, 3 * D), BF16),
        vm((D, FF), BF16), vm((D, FF), BF16), vm((NG, FF, 128), BF16),
        vm((D // 2, S), U32), vm((D // 2, S), U32),
        vm((D // 2, S), U32), vm((D // 2, S), U32),
        vm((NG, S // 2, 128), U32), vm((NG, S // 2, 128), U32),
        vm((NG, S // 2, 128), U32),
        vm((S // 2, D), U32),
        vm((NG * NSEG * 8, 128), F32),
        vm((D, 128), F32),
        vm(((NSEG + 1) * 8, 128), F32),
        vm((SUB, D), F32),
        vm((8, D), F32),
        vm((L, QB), F32), vm((L, QB), F32),
    ] + [vm((4 * QB + 8, QB), F32) for _ in range(NSB)] + [
        pltpu.SemaphoreType.DMA((NSEG,)),
        pltpu.SemaphoreType.DMA((7,)),
        pltpu.SemaphoreType.DMA((NG,)),
        pltpu.SemaphoreType.DMA((NSEG,)),
    ]
    return pl.pallas_call(
        _kernel,
        out_shape=jax.ShapeDtypeStruct((1, S, D), BF16),
        in_specs=[any_spec, any_spec, any_spec, any_spec, any_spec,
                  small((H,)), small((D,)), any_spec, any_spec, any_spec],
        out_specs=any_spec,
        scratch_shapes=scratch,
        compiler_params=pltpu.CompilerParams(vmem_limit_bytes=110 * 1024 * 1024),
        name="infini_mod",
    )(A_x, A_wq, A_wk, A_wv, A_wo, A_beta, B_w_r, B_w_gate, B_w_up, B_w_down)
```
